```python
import jax
import jax.numpy as jnp

def _softmax(x, axis=-1):
    return jax.nn.softmax(x, axis=axis)

def _gelu(x):
    return jax.nn.gelu(x, approximate=True)

def _silu(x):
    return jax.nn.silu(x)

def _sigmoid(x):
    return jax.nn.sigmoid(x)

def _layernorm(x, axis=-1, eps=1e-05):
    m = jnp.mean(x, axis=axis, keepdims=True)
    v = jnp.var(x, axis=axis, keepdims=True)
    return (x - m) / jnp.sqrt(v + eps)

def _scatter_add(tgt, idx, src, axis=0):
    return tgt.at[idx].add(src)

def _segment_sum(src, seg, n):
    return jax.ops.segment_sum(src, seg, n)

class _Rng:

    def __init__(self, key):
        self._k = key

    def _next(self):
        self._k, sub = jax.random.split(self._k)
        return sub

    def normal(self, shape):
        return jax.random.normal(self._next(), shape, dtype=jnp.bfloat16)

    def randint(self, lo, hi, shape):
        return jax.random.randint(self._next(), shape, lo, hi, dtype=jnp.int32)

    def uniform(self, shape, lo=0.0, hi=1.0):
        return jax.random.uniform(self._next(), shape, jnp.bfloat16, lo, hi)

    def permutation(self, n):
        return jax.random.permutation(self._next(), n)
kernel_name = 'adaLN_cond__memory_aug_recurrent_mem_tr__glu_gated_swiglu__prompt'

def setup_inputs():
    _rng = _Rng(jax.random.key(int.from_bytes(__import__("os").urandom(4), "little")))
    _w = lambda a: (lambda t: t.astype(jnp.bfloat16) if jnp.issubdtype(t.dtype, jnp.floating) else t)(jnp.asarray(a))

    def _A_setup():
        B, S, Dm = (1, 2048, 1024)
        H, Dh = (32, 128)
        M, seg = (8, 32)
        seg = min(seg, S)
        S = S // seg * seg
        return {'x': _w((lambda *s: _rng.normal(s) * 0.05)(B, S, Dm)), 'mem0': _w((lambda *s: _rng.normal(s) * 0.05)(B, M, Dm)), 'Wq': _w((lambda *s: _rng.normal(s) * 0.05)(Dm, H, Dh) * Dm ** (-0.5)), 'Wk': _w((lambda *s: _rng.normal(s) * 0.05)(Dm, H, Dh) * Dm ** (-0.5)), 'Wv': _w((lambda *s: _rng.normal(s) * 0.05)(Dm, H, Dh) * Dm ** (-0.5)), 'Wo': _w((lambda *s: _rng.normal(s) * 0.05)(H, Dh, Dm) * (H * Dh) ** (-0.5)), 'seg_len': seg}
    _A_in = _A_setup()

    def _B_setup():
        B, S, D, F = (1, 2048, 1024, 3584)
        return {'x': _w((lambda *s: _rng.normal(s) * 0.05)(B, S, D)), 'w1': _w((lambda *s: _rng.normal(s) * 0.05)(D, F) * (2.0 / D) ** 0.5), 'w3': _w((lambda *s: _rng.normal(s) * 0.05)(D, F) * (2.0 / D) ** 0.5), 'w2': _w((lambda *s: _rng.normal(s) * 0.05)(F, D) * (2.0 / F) ** 0.5)}
    _B_in = _B_setup()
    return {'A_x': _A_in['x'], 'A_mem0': _A_in['mem0'], 'A_Wq': _A_in['Wq'], 'A_Wk': _A_in['Wk'], 'A_Wv': _A_in['Wv'], 'A_Wo': _A_in['Wo'], 'A_seg_len': _A_in['seg_len'], 'B_x': _B_in['x'], 'B_w1': _B_in['w1'], 'B_w3': _B_in['w3'], 'B_w2': _B_in['w2'], 'c': _w((lambda *s: _rng.normal(s) * 0.05)(1, 1024)), 'w_mod': _w((lambda *s: _rng.normal(s) * 0.05)(1024, 6 * 1024) * 1024 ** (-0.5))}

def reference(A_x, A_mem0, A_Wq, A_Wk, A_Wv, A_Wo, A_seg_len, B_x, B_w1, B_w3, B_w2, c, w_mod):

    def _A_ref(x, mem0, Wq, Wk, Wv, Wo, seg_len):
        B, S, Dm = x.shape
        H, Dh = (Wq.shape[1], Wq.shape[2])
        M = mem0.shape[1]
        scale = Dh ** (-0.5)
        n_seg = S // seg_len
        L = M + seg_len
        idx = jnp.arange(L)
        mask = (idx[:, None] < M) | (idx[:, None] >= idx[None, :])
        mem = mem0
        outs = []
        for s in range(n_seg):
            xs = x[:, s * seg_len:(s + 1) * seg_len, :].copy()
            h = jnp.concatenate([mem, xs], axis=1)
            q = jnp.einsum('btd,dhe->bhte', h, Wq)
            k = jnp.einsum('btd,dhe->bhte', h, Wk)
            v = jnp.einsum('btd,dhe->bhte', h, Wv)
            scores = jnp.einsum('bhqe,bhke->bhqk', q, k) * scale
            scores = jnp.where(mask[None, None], scores, -1000000000.0)
            p = _softmax(scores, axis=-1)
            o = jnp.einsum('bhqk,bhke->bhqe', p, v)
            o = jnp.einsum('bhte,hed->btd', o, Wo)
            mem = o[:, :M, :].copy()
            outs.append(o[:, M:, :])
        return jnp.concatenate(outs, axis=1)

    def _B_ref(x, w1, w3, w2):
        gate = jnp.einsum('bsd,df->bsf', x, w1)
        up = jnp.einsum('bsd,df->bsf', x, w3)
        h = _silu(gate) * up
        out = jnp.einsum('bsf,fd->bsd', h, w2)
        return out
    x = A_x
    mod = (_silu(c) @ w_mod).reshape(c.shape[0], 6, 1, -1)
    sa, ca, ga, sb, cb, gb = (mod[:, 0].copy(), mod[:, 1].copy(), mod[:, 2].copy(), mod[:, 3].copy(), mod[:, 4].copy(), mod[:, 5].copy())
    h = _layernorm(x, axis=-1) * (1 + ca) + sa
    x = x + ga * _A_ref(h, A_mem0, A_Wq, A_Wk, A_Wv, A_Wo, A_seg_len)
    h = _layernorm(x, axis=-1) * (1 + cb) + sb
    x = x + gb * _B_ref(h, B_w1, B_w3, B_w2)
    return x
```

```python
import functools

import jax
import jax.numpy as jnp
from jax import lax
import jax.experimental.pallas as pl
import jax.experimental.pallas.tpu as pltpu

F32 = jnp.float32
BF16 = jnp.bfloat16
U32 = jnp.uint32
LANE = 128
PRE = 8
HG = 4
MB = 128
PAIRS_PER_IT = 2


def _layernorm(x):
    m = jnp.mean(x, axis=-1, keepdims=True)
    d = x - m
    v = jnp.mean(d * d, axis=-1, keepdims=True)
    return d * lax.rsqrt(v + 1e-5)


def _silu(x):
    return x / (1.0 + jnp.exp(-x))


def _w(tile_u32):
    return pltpu.bitcast(tile_u32, BF16)


def _dot(a, b):
    return lax.dot_general(a, b, (((1,), (0,)), ((), ())), preferred_element_type=F32)


def _dot_nt(a, b):
    return lax.dot_general(a, b, (((1,), (1,)), ((), ())), preferred_element_type=F32)


def _kernel(c_ref, mem_ref, x_hbm, wq_hbm, wk_hbm, wv_hbm, wo_hbm, w1_hbm, w3_hbm, w2_hbm,
            wmod_hbm, out_hbm,
            stage, wqkv, wo, w1, w3, w2, pre, xp, hp, xs, attn, lhs, obuf, mod, h2, act, res,
            sems, *, seg, n_seg, n_mem, n_head, d_model, d_ff):
    D, H, M = d_model, n_head, n_mem
    KH = D // 2
    DT = D // LANE
    FT = d_ff // LANE
    L = M + seg
    CUR = seg - PRE
    CP = 8
    n_chunk = 3 * H // (2 * CP)
    slot_rows = D * CP
    stage2 = stage.reshape(3 * slot_rows, LANE)
    (S_XP, S_X, S_WO, S_F1, S_F3, S_F2, S_OUT, S_ST) = range(8)

    def chunk_copy(ci):
        src = (wq_hbm, wk_hbm, wv_hbm)[ci // (n_chunk // 3)].bitcast(U32)
        g = ci % (n_chunk // 3)
        return pltpu.make_async_copy(src.at[:, pl.ds(g * CP, CP), :], stage.at[ci % 3],
                                     sems.at[S_ST + ci % 3])

    def wmod_copies(part, slot):
        src = wmod_hbm.bitcast(U32)
        return [pltpu.make_async_copy(
            src.at[:, pl.ds((part * 2 * DT + j) * LANE, LANE)],
            stage2.at[pl.ds(slot * slot_rows + j * KH, KH), :], sems.at[S_ST + slot])
            for j in range(2 * DT)]

    def tile_copies(src_hbm, dst, sem):
        src = src_hbm.bitcast(U32)
        return [pltpu.make_async_copy(src.at[:, pl.ds(j * LANE, LANE)], dst.at[j], sems.at[sem])
                for j in range(dst.shape[0])]

    def start(cps):
        for cp in cps:
            cp.start()

    def wait(cps):
        for cp in cps:
            cp.wait()

    xp_copy = pltpu.make_async_copy(x_hbm.at[:, pl.ds(CUR, PRE), :], xp, sems.at[S_XP])
    x_copy = pltpu.make_async_copy(x_hbm, xs, sems.at[S_X])

    def modulation(part, slot):
        sc = jnp.broadcast_to(_silu(c_ref[...].astype(F32)), (8, D))
        for j in range(2 * DT):
            r = _dot(sc, _w(stage2[pl.ds(slot * slot_rows + j * KH, KH), :]))
            mod[2 * part + j // DT, :, pl.ds((j % DT) * LANE, LANE)] = r

    def modrow(i):
        return mod[i, 0:1, :]

    xp_copy.start()
    start(wmod_copies(0, 2))
    chunk_copy(0).start()
    xp_copy.wait()
    xn = _layernorm(xp[...].astype(F32).reshape(n_seg * PRE, D))
    wait(wmod_copies(0, 2))
    chunk_copy(1).start()
    modulation(0, 2)
    chunk_copy(2).start()
    hp[...] = (xn * (1.0 + modrow(1)) + modrow(0)).astype(BF16)

    def retile(p):
        base = ((p // CP) % 3) * slot_rows + p % CP
        a = stage2[pl.ds(base, KH, stride=2 * CP), :]
        b = stage2[pl.ds(base + CP, KH, stride=2 * CP), :]
        wqkv[2 * p] = (a & jnp.uint32(0xFFFF)) | (b << 16)
        wqkv[2 * p + 1] = (a >> 16) | (b & jnp.uint32(0xFFFF0000))

    def project_pre(p):
        for t in range(2):
            pre[2 * p + t] = _dot(hp[...], _w(wqkv[2 * p + t]))

    chunk_copy(0).wait()
    for t in range(PAIRS_PER_IT):
        retile(t)
    n_it = n_chunk * CP // PAIRS_PER_IT
    it_per_chunk = CP // PAIRS_PER_IT

    def pro_body(i, carry):
        for ci in range(1, n_chunk):
            @pl.when(i == ci * it_per_chunk - 1)
            def _():
                chunk_copy(ci).wait()
                if ci + 2 < n_chunk:
                    chunk_copy(ci + 2).start()
                if ci == n_chunk - 2:
                    x_copy.start()
                    start(tile_copies(wo_hbm, wo, S_WO))
        for t in range(PAIRS_PER_IT):
            project_pre(i * PAIRS_PER_IT + t)
        for t in range(PAIRS_PER_IT):
            retile((i + 1) * PAIRS_PER_IT + t)
        return carry

    lax.fori_loop(0, n_it - 1, pro_body, 0)
    start(wmod_copies(1, 0))
    start(wmod_copies(2, 1))
    start(tile_copies(w1_hbm, w1, S_F1))
    start(tile_copies(w3_hbm, w3, S_F3))
    start(tile_copies(w2_hbm, w2, S_F2))
    for t in range(PAIRS_PER_IT):
        project_pre((n_it - 1) * PAIRS_PER_IT + t)
    x_copy.wait()
    wait(tile_copies(wo_hbm, wo, S_WO))

    def seg_rows(s):
        xn = _layernorm(xs[s].astype(F32)[0:CUR])
        return xn * (1.0 + modrow(1)) + modrow(0)

    lhs[...] = jnp.concatenate([mem_ref[...].astype(F32), seg_rows(0)], axis=0).astype(BF16)
    scale = float(LANE) ** -0.5
    NG = H // HG

    def chain_body(s, carry):
        row = lax.broadcasted_iota(jnp.int32, (L, L), 0)
        col = lax.broadcasted_iota(jnp.int32, (L, L), 1)
        mask = (row < M) | (row >= col)
        r0 = pl.multiple_of(s * PRE, PRE)
        qkv, sc = {}, {}

        def proj(g):
            for h in range(g * HG, (g + 1) * HG):
                qkv[h] = [jnp.concatenate([_dot(lhs[...], _w(wqkv[m * H + h])),
                                           pre[m * H + h, pl.ds(r0, PRE), :]], axis=0)
                          for m in range(3)]

        def scores(g):
            for h in range(g * HG, (g + 1) * HG):
                q, k, _ = qkv[h]
                sc[h] = _dot_nt(q, k.astype(BF16))

        def values(g):
            for h in range(g * HG, (g + 1) * HG):
                z = jnp.where(mask, sc[h] * scale, -1e9)
                p = jnp.exp(z - jnp.max(z, axis=-1, keepdims=True))
                inv = 1.0 / jnp.sum(p, axis=-1, keepdims=True)
                obuf[:, pl.ds(h * LANE, LANE)] = _dot(p, qkv[h][2].astype(BF16)) * inv

        def out_proj(h0, h1):
            o = obuf[:, pl.ds(h0 * LANE, (h1 - h0) * LANE)]
            return [_dot(o, _w(wo[j, pl.ds(h0 * LANE // 2, (h1 - h0) * LANE // 2), :]))
                    for j in range(DT)]

        for g in range(NG):
            proj(g)
            if g >= 2:
                values(g - 2)
            if g >= 1:
                scores(g - 1)
        nxt = seg_rows(jnp.minimum(s + 1, n_seg - 1))
        ha, hb = (NG - 2) * HG // 2, (NG - 2) * HG
        o1 = out_proj(0, ha)
        values(NG - 2)
        scores(NG - 1)
        o2 = out_proj(ha, hb)
        values(NG - 1)
        o3 = out_proj(hb, hb + HG)
        o4 = out_proj(hb + HG, H)
        o = jnp.concatenate([(a + b) + (c + d) for a, b, c, d in zip(o1, o2, o3, o4)], axis=1)
        attn[s] = o[M:].astype(BF16)
        lhs[...] = jnp.concatenate([o[:M], nxt], axis=0).astype(BF16)
        return carry

    lax.fori_loop(0, n_seg, chain_body, 0)

    wait(wmod_copies(1, 0))
    wait(wmod_copies(2, 1))
    modulation(1, 0)
    modulation(2, 1)
    wait(tile_copies(w1_hbm, w1, S_F1))
    wait(tile_copies(w3_hbm, w3, S_F3))
    wait(tile_copies(w2_hbm, w2, S_F2))
    SB = MB // seg
    n_blk = n_seg // SB

    def resid(i):
        sl = pl.ds(i * SB, SB)
        return (xs[sl].astype(F32).reshape(MB, D)
                + modrow(2) * attn[sl].astype(F32).reshape(MB, D))

    def ffn_in(i):
        return (_layernorm(resid(i)) * (1.0 + modrow(4)) + modrow(3)).astype(BF16)

    def out_copy(i):
        sl = pl.ds(pl.multiple_of(i * MB, MB), MB)
        return pltpu.make_async_copy(res.at[sl, :], out_hbm.at[sl, :], sems.at[S_OUT])

    h2[...] = ffn_in(0)

    def ffn_body(i, carry):
        for j in range(FT):
            g = _dot(h2[...], _w(w1[j]))
            u = _dot(h2[...], _w(w3[j]))
            act[:, pl.ds(j * LANE, LANE)] = (_silu(g) * u).astype(BF16)
        h2[...] = ffn_in(jnp.minimum(i + 1, n_blk - 1))
        y = jnp.concatenate([_dot(act[...], _w(w2[j])) for j in range(DT)], axis=1)
        res[pl.ds(pl.multiple_of(i * MB, MB), MB), :] = (resid(i) + modrow(5) * y).astype(BF16)
        out_copy(i).start()
        return carry

    lax.fori_loop(0, n_blk, ffn_body, 0)
    pltpu.make_async_copy(res, out_hbm, sems.at[S_OUT]).wait()


@functools.partial(jax.jit, static_argnames=("A_seg_len",))
def pallas_adaLN_cond__memory_aug_recurrent_mem_tr__glu_gated_swiglu__prompt_kernel(
    A_x, A_mem0, A_Wq, A_Wk, A_Wv, A_Wo, A_seg_len, B_x, B_w1, B_w3, B_w2, c, w_mod,
):
    del B_x
    B, S, D = A_x.shape
    _, H, Dh = A_Wq.shape
    M = A_mem0.shape[1]
    F = B_w1.shape[1]
    seg = int(A_seg_len)
    n_seg = S // seg
    assert B == 1 and Dh == LANE and S % seg == 0 and S % MB == 0 and MB % seg == 0
    kern = functools.partial(_kernel, seg=seg, n_seg=n_seg, n_mem=M, n_head=H, d_model=D, d_ff=F)
    hbm = pl.BlockSpec(memory_space=pl.ANY)
    vmem = pl.BlockSpec(memory_space=pltpu.VMEM)
    out = pl.pallas_call(
        kern,
        out_shape=jax.ShapeDtypeStruct((S, D), A_x.dtype),
        in_specs=[vmem, vmem] + [hbm] * 9,
        out_specs=hbm,
        scratch_shapes=[
            pltpu.VMEM((3, D, 8, LANE), U32),
            pltpu.VMEM((3 * H, D // 2, LANE), U32),
            pltpu.VMEM((D // LANE, H * Dh // 2, LANE), U32),
            pltpu.VMEM((F // LANE, D // 2, LANE), U32),
            pltpu.VMEM((F // LANE, D // 2, LANE), U32),
            pltpu.VMEM((D // LANE, F // 2, LANE), U32),
            pltpu.VMEM((3 * H, n_seg * PRE, LANE), F32),
            pltpu.VMEM((n_seg, PRE, D), BF16),
            pltpu.VMEM((n_seg * PRE, D), BF16),
            pltpu.VMEM((n_seg, seg, D), BF16),
            pltpu.VMEM((n_seg, seg, D), BF16),
            pltpu.VMEM((M + seg - PRE, D), BF16),
            pltpu.VMEM((M + seg, H * Dh), F32),
            pltpu.VMEM((6, 8, D), F32),
            pltpu.VMEM((MB, D), BF16),
            pltpu.VMEM((MB, F), BF16),
            pltpu.VMEM((S, D), BF16),
            pltpu.SemaphoreType.DMA((10,)),
        ],
        compiler_params=pltpu.CompilerParams(vmem_limit_bytes=124 * 1024 * 1024),
    )(c, A_mem0.reshape(M, D), A_x.reshape(n_seg, seg, D), A_Wq, A_Wk, A_Wv,
      A_Wo.reshape(H * Dh, D), B_w1, B_w3, B_w2, w_mod)
    return out.reshape(B, S, D)
```

```python
import functools

import jax
import jax.numpy as jnp
from jax import lax
import jax.experimental.pallas as pl
import jax.experimental.pallas.tpu as pltpu

F32 = jnp.float32
BF16 = jnp.bfloat16
U32 = jnp.uint32
LANE = 128
PRE = 8
HG = 4
SPLIT = 8
AHEAD = 3
MB = 128
PAIRS_PER_IT = 2


def _layernorm(x):
    m = jnp.mean(x, axis=-1, keepdims=True)
    d = x - m
    v = jnp.mean(d * d, axis=-1, keepdims=True)
    return d * lax.rsqrt(v + 1e-5)


def _silu(x):
    return x / (1.0 + jnp.exp(-x))


def _w(tile_u32):
    return pltpu.bitcast(tile_u32, BF16)


def _dot(a, b):
    return lax.dot_general(a, b, (((1,), (0,)), ((), ())), preferred_element_type=F32)


def _dot_nt(a, b):
    return lax.dot_general(a, b, (((1,), (1,)), ((), ())), preferred_element_type=F32)


def _kernel(c_ref, mem_ref, x_hbm, wq_hbm, wk_hbm, wv_hbm, wo_hbm, w1_hbm, w3_hbm, w2_hbm,
            wmod_hbm, out_hbm,
            stage, wqkv, wo, w1, w3, w2, pre, xp, hp, xs, attn, lhs, mod, h2, act, res,
            sems, *, seg, n_seg, n_mem, n_head, d_model, d_ff):
    D, H, M = d_model, n_head, n_mem
    DT = D // LANE
    FT = d_ff // LANE
    L = M + seg
    CUR = seg - PRE
    PP = PAIRS_PER_IT
    n_it = 3 * H // (2 * PP)
    it_per_mat = n_it // 3
    (S_XP, S_X, S_WO, S_F1, S_F3, S_F2, S_OUT, S_MOD, S_ST) = range(9)

    def pair_copies(w_hbm, i):
        src = w_hbm.bitcast(U32)
        return [pltpu.make_async_copy(
            src.at[:, (i % it_per_mat) * PP + t + par * (H // 2), :],
            wqkv.at[(i * PP + t) * 2 + par], sems.at[S_ST + i])
            for t in range(PP) for par in range(2)]

    def wmod_copies(part):
        src = wmod_hbm.bitcast(U32)
        return [pltpu.make_async_copy(
            src.at[:, pl.ds((part * 2 * DT + j) * LANE, LANE)],
            stage.at[(part % 2) * 2 * DT + j], sems.at[S_MOD])
            for j in range(2 * DT)]

    def tile_copies(src_hbm, dst, sem):
        src = src_hbm.bitcast(U32)
        return [pltpu.make_async_copy(src.at[:, pl.ds(j * LANE, LANE)], dst.at[j], sems.at[sem])
                for j in range(dst.shape[0])]

    def start(cps):
        for cp in cps:
            cp.start()

    def wait(cps):
        for cp in cps:
            cp.wait()

    xp_copy = pltpu.make_async_copy(x_hbm.at[:, pl.ds(CUR, PRE), :], xp, sems.at[S_XP])
    x_copy = pltpu.make_async_copy(x_hbm, xs, sems.at[S_X])

    def modulation(part):
        sc = jnp.broadcast_to(_silu(c_ref[...].astype(F32)), (8, D))
        for j in range(2 * DT):
            r = _dot(sc, _w(stage[(part % 2) * 2 * DT + j]))
            mod[2 * part + j // DT, :, pl.ds((j % DT) * LANE, LANE)] = r

    def modrow(i):
        return mod[i, 0:1, :]

    xp_copy.start()
    start(wmod_copies(0))
    start(pair_copies(wq_hbm, 0))
    xp_copy.wait()
    xn = _layernorm(xp[...].astype(F32).reshape(n_seg * PRE, D))
    wait(wmod_copies(0))
    for i in range(1, AHEAD):
        start(pair_copies(wq_hbm, i))
    modulation(0)
    hp[...] = (xn * (1.0 + modrow(1)) + modrow(0)).astype(BF16)
    wo_copies = tile_copies(wo_hbm, wo, S_WO)

    def pro_body(w_next, i, carry):
        wait(pair_copies(wq_hbm, i))
        for t in range(PP):
            a = wqkv[(i * PP + t) * 2]
            b = wqkv[(i * PP + t) * 2 + 1]
            heads = ((a & jnp.uint32(0xFFFF)) | (b << 16), (a >> 16) | (b & jnp.uint32(0xFFFF0000)))
            for par in range(2):
                wqkv[(i * PP + t) * 2 + par] = heads[par]
            if t == PP - 1 and w_next is not None:
                start(pair_copies(w_next, i + AHEAD))
            for par in range(2):
                pre[(i * PP + t) * 2 + par] = _dot(hp[...], _w(heads[par]))
        return carry

    for m, w_hbm in enumerate((wq_hbm, wk_hbm, wv_hbm)):
        lax.fori_loop(max(m * it_per_mat - AHEAD, 0), (m + 1) * it_per_mat - AHEAD,
                      functools.partial(pro_body, w_hbm), 0)
        if m == 0:
            x_copy.start()
        if m == 1:
            start(wo_copies)
    lax.fori_loop(n_it - AHEAD, n_it, functools.partial(pro_body, None), 0)
    start(wmod_copies(1))
    start(wmod_copies(2))
    start(tile_copies(w1_hbm, w1, S_F1))
    start(tile_copies(w3_hbm, w3, S_F3))
    start(tile_copies(w2_hbm, w2, S_F2))
    x_copy.wait()
    wait(wo_copies)

    def seg_rows(s):
        xn = _layernorm(xs[s].astype(F32)[0:CUR])
        return xn * (1.0 + modrow(1)) + modrow(0)

    lhs[...] = jnp.concatenate([mem_ref[...].astype(F32), seg_rows(0)], axis=0).astype(BF16)
    scale = float(LANE) ** -0.5
    NG = H // HG

    def chain_body(s, carry):
        row = lax.broadcasted_iota(jnp.int32, (L, L), 0)
        col = lax.broadcasted_iota(jnp.int32, (L, L), 1)
        mask = (row < M) | (row >= col)
        r0 = pl.multiple_of(s * PRE, PRE)
        q, k, v, p, inv, ov = {}, {}, {}, {}, {}, {}

        def heads(g):
            return range(g * HG, (g + 1) * HG)

        def proj(m, h):
            return jnp.concatenate([_dot(lhs[...], _w(wqkv[m * H + h])),
                                    pre[m * H + h, pl.ds(r0, PRE), :]], axis=0)

        def probs(g):
            for h in heads(g):
                z = jnp.where(mask, _dot_nt(q[h], k[h]) * scale, -1e9)
                p[h] = jnp.exp(z - jnp.max(z, axis=-1, keepdims=True))
                inv[h] = 1.0 / jnp.sum(p[h], axis=-1, keepdims=True)

        def values(g):
            for h in heads(g):
                ov[h] = _dot(p[h], v[h]) * inv[h]

        def out_proj(h0, h1):
            o = jnp.concatenate([ov[h] for h in range(h0, h1)], axis=1)
            return jnp.concatenate(
                [_dot(o, _w(wo[j, pl.ds(h0 * LANE // 2, (h1 - h0) * LANE // 2), :]))
                 for j in range(DT)], axis=1)

        for g in range(NG):
            for h in heads(g):
                q[h] = proj(0, h)
                k[h] = proj(1, h).astype(BF16)
            if g >= 1:
                probs(g - 1)
        for g in range(NG):
            for h in heads(g):
                v[h] = proj(2, h).astype(BF16)
            if g == 0:
                probs(NG - 1)
            else:
                values(g - 1)
        nxt = seg_rows(jnp.minimum(s + 1, n_seg - 1))
        o = out_proj(0, SPLIT)
        values(NG - 1)
        o = o + out_proj(SPLIT, H)
        attn[s] = o[M:].astype(BF16)
        lhs[...] = jnp.concatenate([o[:M], nxt], axis=0).astype(BF16)
        return carry

    lax.fori_loop(0, n_seg, chain_body, 0)

    wait(wmod_copies(1))
    wait(wmod_copies(2))
    modulation(1)
    modulation(2)
    wait(tile_copies(w1_hbm, w1, S_F1))
    wait(tile_copies(w3_hbm, w3, S_F3))
    wait(tile_copies(w2_hbm, w2, S_F2))
    SB = MB // seg
    n_blk = n_seg // SB

    def resid(i):
        sl = pl.ds(i * SB, SB)
        return (xs[sl].astype(F32).reshape(MB, D)
                + modrow(2) * attn[sl].astype(F32).reshape(MB, D))

    def ffn_in(i):
        return (_layernorm(resid(i)) * (1.0 + modrow(4)) + modrow(3)).astype(BF16)

    def out_copy(i):
        sl = pl.ds(pl.multiple_of(i * MB, MB), MB)
        return pltpu.make_async_copy(res.at[sl, :], out_hbm.at[sl, :], sems.at[S_OUT])

    h2[...] = ffn_in(0)

    def ffn_body(i, carry):
        for j in range(FT):
            g = _dot(h2[...], _w(w1[j]))
            u = _dot(h2[...], _w(w3[j]))
            act[:, pl.ds(j * LANE, LANE)] = (_silu(g) * u).astype(BF16)
        h2[...] = ffn_in(jnp.minimum(i + 1, n_blk - 1))
        y = jnp.concatenate([_dot(act[...], _w(w2[j])) for j in range(DT)], axis=1)
        res[pl.ds(pl.multiple_of(i * MB, MB), MB), :] = (resid(i) + modrow(5) * y).astype(BF16)
        out_copy(i).start()
        return carry

    lax.fori_loop(0, n_blk, ffn_body, 0)
    pltpu.make_async_copy(res, out_hbm, sems.at[S_OUT]).wait()


@functools.partial(jax.jit, static_argnames=("A_seg_len",))
def pallas_adaLN_cond__memory_aug_recurrent_mem_tr__glu_gated_swiglu__prompt_kernel(
    A_x, A_mem0, A_Wq, A_Wk, A_Wv, A_Wo, A_seg_len, B_x, B_w1, B_w3, B_w2, c, w_mod,
):
    del B_x
    B, S, D = A_x.shape
    _, H, Dh = A_Wq.shape
    M = A_mem0.shape[1]
    F = B_w1.shape[1]
    seg = int(A_seg_len)
    n_seg = S // seg
    assert B == 1 and Dh == LANE and S % seg == 0 and S % MB == 0 and MB % seg == 0
    kern = functools.partial(_kernel, seg=seg, n_seg=n_seg, n_mem=M, n_head=H, d_model=D, d_ff=F)
    hbm = pl.BlockSpec(memory_space=pl.ANY)
    vmem = pl.BlockSpec(memory_space=pltpu.VMEM)
    out = pl.pallas_call(
        kern,
        out_shape=jax.ShapeDtypeStruct((S, D), A_x.dtype),
        in_specs=[vmem, vmem] + [hbm] * 9,
        out_specs=hbm,
        scratch_shapes=[
            pltpu.VMEM((4 * D // LANE, D // 2, LANE), U32),
            pltpu.VMEM((3 * H, D // 2, LANE), U32),
            pltpu.VMEM((D // LANE, H * Dh // 2, LANE), U32),
            pltpu.VMEM((F // LANE, D // 2, LANE), U32),
            pltpu.VMEM((F // LANE, D // 2, LANE), U32),
            pltpu.VMEM((D // LANE, F // 2, LANE), U32),
            pltpu.VMEM((3 * H, n_seg * PRE, LANE), F32),
            pltpu.VMEM((n_seg, PRE, D), BF16),
            pltpu.VMEM((n_seg * PRE, D), BF16),
            pltpu.VMEM((n_seg, seg, D), BF16),
            pltpu.VMEM((n_seg, seg, D), BF16),
            pltpu.VMEM((M + seg - PRE, D), BF16),
            pltpu.VMEM((6, 8, D), F32),
            pltpu.VMEM((MB, D), BF16),
            pltpu.VMEM((MB, F), BF16),
            pltpu.VMEM((S, D), BF16),
            pltpu.SemaphoreType.DMA((8 + 3 * H // (2 * PAIRS_PER_IT),)),
        ],
        compiler_params=pltpu.CompilerParams(vmem_limit_bytes=124 * 1024 * 1024),
    )(c, A_mem0.reshape(M, D), A_x.reshape(n_seg, seg, D),
      A_Wq.reshape(D // 2, 2 * H, Dh), A_Wk.reshape(D // 2, 2 * H, Dh),
      A_Wv.reshape(D // 2, 2 * H, Dh),
      A_Wo.reshape(H * Dh, D), B_w1, B_w3, B_w2, w_mod)
    return out.reshape(B, S, D)
```

```python
import functools

import jax
import jax.numpy as jnp
from jax import lax
import jax.experimental.pallas as pl
import jax.experimental.pallas.tpu as pltpu

F32 = jnp.float32
BF16 = jnp.bfloat16
U32 = jnp.uint32
LANE = 128
PRE = 8
HG = 4
SPLIT = 8
AHEAD = 3
CROWS = 8
MB = 128
PAIRS_PER_IT = 2


def _layernorm(x):
    m = jnp.mean(x, axis=-1, keepdims=True)
    d = x - m
    v = jnp.mean(d * d, axis=-1, keepdims=True)
    return d * lax.rsqrt(v + 1e-5)


def _silu(x):
    return x / (1.0 + jnp.exp(-x))


def _w(tile_u32):
    return pltpu.bitcast(tile_u32, BF16)


def _dot(a, b):
    return lax.dot_general(a, b, (((1,), (0,)), ((), ())), preferred_element_type=F32)


def _dot_nt(a, b):
    return lax.dot_general(a, b, (((1,), (1,)), ((), ())), preferred_element_type=F32)


def _strassen_lhs(a11, a12, a21, a22):
    return [t.astype(BF16) for t in
            (a11 + a22, a21 + a22, a11, a22, a11 + a12, a21 - a11, a12 - a22)]


def _strassen_rhs(b11, b12, b21, b22):
    b11, b12, b21, b22 = (t.astype(F32) for t in (b11, b12, b21, b22))
    return [t.astype(BF16) for t in (b11 + b22, b12 - b22, b21 - b11, b11 + b12, b21 + b22)]


def _strassen_out(prod):
    m0, m1, m2, m3, m4 = (prod(i) for i in range(5))
    c12 = m2 + m4
    c21 = m1 + m3
    c22 = (m0 - m1) + m2 + prod(5)
    c11 = (m0 + m3) - m4 + prod(6)
    return c11, c12, c21, c22


def _kernel(c_ref, mem_ref, x_hbm, wq_hbm, wk_hbm, wv_hbm, wo_hbm, w1_hbm, w3_hbm, w2_hbm,
            wmod_hbm, out_hbm,
            stage, wqkv, wo, wf, pre, xp, hp, xs, attn, lhs, mod, h2, act, res,
            sems, *, seg, n_seg, n_mem, n_head, d_model, d_ff):
    D, H, M = d_model, n_head, n_mem
    DT = D // LANE
    FT = d_ff // LANE
    L = M + seg
    CUR = seg - PRE
    PP = PAIRS_PER_IT
    n_it = 3 * H // (2 * PP)
    it_per_mat = n_it // 3
    (S_XP, S_X, S_WO, S_FF, S_OUT, S_MOD, S_ST) = range(7)

    def pair_copies(w_hbm, i):
        src = w_hbm.bitcast(U32)
        return [pltpu.make_async_copy(
            src.at[:, (i % it_per_mat) * PP + t + par * (H // 2), :],
            wqkv.at[(i * PP + t) * 2 + par], sems.at[S_ST + i])
            for t in range(PP) for par in range(2)]

    def wmod_copies(part):
        src = wmod_hbm.bitcast(U32)
        return [pltpu.make_async_copy(
            src.at[:, pl.ds((part * 2 * DT + j) * LANE, LANE)],
            stage.at[(part % 2) * 2 * DT + j], sems.at[S_MOD])
            for j in range(2 * DT)]

    def lane_tile(j):
        return pl.ds(pl.multiple_of(j * LANE, LANE), LANE)

    def wo_copy(j):
        return pltpu.make_async_copy(wo_hbm.bitcast(U32).at[:, lane_tile(j)], wo.at[j],
                                     sems.at[S_WO])

    def x_copy(j):
        sl = pl.ds(j * (n_seg // it_per_mat), n_seg // it_per_mat)
        return pltpu.make_async_copy(x_hbm.at[sl], xs.at[sl], sems.at[S_X])

    UP, DN = D // 4, d_ff // 4
    FH, DH = FT // 2, DT // 2

    def ffn_copies():
        cps = []
        for w_hbm, rows, half, base in ((w1_hbm, UP, FH, 0), (w3_hbm, UP, FH, FH * UP),
                                        (w2_hbm, DN, DH, 2 * FH * UP)):
            src = w_hbm.bitcast(U32)
            for j in range(half):
                for kh in range(2):
                    for nh in range(2):
                        cps.append(pltpu.make_async_copy(
                            src.at[pl.ds(kh * rows, rows), pl.ds((j + nh * half) * LANE, LANE)],
                            wf.at[1 + 2 * kh + nh, pl.ds(base + j * rows, rows), :],
                            sems.at[S_FF]))
        return cps

    def start(cps):
        for cp in cps:
            cp.start()

    def wait(cps):
        for cp in cps:
            cp.wait()

    xp_copy = pltpu.make_async_copy(x_hbm.at[:, pl.ds(CUR, PRE), :], xp, sems.at[S_XP])

    def modulation(part):
        sc = jnp.broadcast_to(_silu(c_ref[...].astype(F32)), (8, D))
        for j in range(2 * DT):
            r = _dot(sc, _w(stage[(part % 2) * 2 * DT + j]))
            mod[2 * part + j // DT, :, pl.ds((j % DT) * LANE, LANE)] = r

    def modrow(i):
        return mod[i, 0:1, :]

    xp_copy.start()
    start(wmod_copies(0))
    start(pair_copies(wq_hbm, 0))
    xp_copy.wait()
    xn = _layernorm(xp[...].astype(F32).reshape(n_seg * PRE, D))
    wait(wmod_copies(0))
    for i in range(1, AHEAD):
        start(pair_copies(wq_hbm, i))
    modulation(0)
    hp[...] = (xn * (1.0 + modrow(1)) + modrow(0)).astype(BF16)

    def pro_body(w_next, extra, i, carry):
        wait(pair_copies(wq_hbm, i))
        for t in range(PP):
            a = wqkv[(i * PP + t) * 2]
            b = wqkv[(i * PP + t) * 2 + 1]
            heads = ((a & jnp.uint32(0xFFFF)) | (b << 16), (a >> 16) | (b & jnp.uint32(0xFFFF0000)))
            for par in range(2):
                wqkv[(i * PP + t) * 2 + par] = heads[par]
            if t == PP - 1 and w_next is not None:
                start(pair_copies(w_next, i + AHEAD))
                if extra is not None:
                    extra((i + AHEAD) % it_per_mat).start()
            for par in range(2):
                pre[(i * PP + t) * 2 + par] = _dot(hp[...], _w(heads[par]))
        return carry

    for m, (w_hbm, extra) in enumerate(((wq_hbm, None), (wk_hbm, wo_copy), (wv_hbm, x_copy))):
        lax.fori_loop(max(m * it_per_mat - AHEAD, 0), (m + 1) * it_per_mat - AHEAD,
                      functools.partial(pro_body, w_hbm, extra), 0)
    lax.fori_loop(n_it - AHEAD, n_it, functools.partial(pro_body, None, None), 0)
    wait([wo_copy(j) for j in range(DT)])
    wait([x_copy(j) for j in range(it_per_mat)])
    start(ffn_copies())
    start(wmod_copies(1))
    start(wmod_copies(2))

    def seg_rows(s):
        xn = _layernorm(xs[s].astype(F32)[0:CUR])
        return xn * (1.0 + modrow(1)) + modrow(0)

    lhs[...] = jnp.concatenate([mem_ref[...].astype(F32), seg_rows(0)], axis=0).astype(BF16)
    scale = float(LANE) ** -0.5
    NG = H // HG

    def chain_body(combine, s, carry):
        row = lax.broadcasted_iota(jnp.int32, (L, L), 0)
        col = lax.broadcasted_iota(jnp.int32, (L, L), 1)
        mask = (row < M) | (row >= col)
        r0 = pl.multiple_of(s * PRE, PRE)
        q, k, v, p, inv, ov = {}, {}, {}, {}, {}, {}

        def heads(g):
            return range(g * HG, (g + 1) * HG)

        def proj(m, h):
            return jnp.concatenate([_dot(lhs[...], _w(wqkv[m * H + h])),
                                    pre[m * H + h, pl.ds(r0, PRE), :]], axis=0)

        def probs(g):
            for h in heads(g):
                z = jnp.where(mask, _dot_nt(q[h], k[h]) * scale, -1e9)
                p[h] = jnp.exp(z - jnp.max(z, axis=-1, keepdims=True))
                inv[h] = 1.0 / jnp.sum(p[h], axis=-1, keepdims=True)

        def values(g):
            for h in heads(g):
                ov[h] = _dot(p[h], v[h]) * inv[h]

        def out_proj(h0, h1):
            o = jnp.concatenate([ov[h] for h in range(h0, h1)], axis=1)
            return jnp.concatenate(
                [_dot(o, _w(wo[j, pl.ds(h0 * LANE // 2, (h1 - h0) * LANE // 2), :]))
                 for j in range(DT)], axis=1)

        def combine_weights(part):
            nr = wf.shape[1] // (n_seg - n_seg // 2)
            for r in range(part * CROWS, nr, H * CROWS) if combine else ():
                rows = pl.ds(pl.multiple_of((s - n_seg // 2) * nr + r, CROWS), CROWS)
                sums = _strassen_rhs(*(_w(wf[i, rows, :]) for i in (1, 2, 3, 4)))
                for i, t in zip((0, 2, 3, 5, 6), sums):
                    wf[i, rows, :] = pltpu.bitcast(t, U32)

        for g in range(NG):
            for h in heads(g):
                combine_weights(h)
                q[h] = proj(0, h)
                k[h] = proj(1, h).astype(BF16)
            if g >= 1:
                probs(g - 1)
        for g in range(NG):
            for h in heads(g):
                v[h] = proj(2, h).astype(BF16)
            if g == 0:
                probs(NG - 1)
            else:
                values(g - 1)
        nxt = seg_rows(jnp.minimum(s + 1, n_seg - 1))
        o = out_proj(0, SPLIT)
        values(NG - 1)
        o = o + out_proj(SPLIT, H)
        attn[s] = o[M:].astype(BF16)
        lhs[...] = jnp.concatenate([o[:M], nxt], axis=0).astype(BF16)
        return carry

    lax.fori_loop(0, n_seg // 2, functools.partial(chain_body, False), 0)
    wait(ffn_copies())
    lax.fori_loop(n_seg // 2, n_seg, functools.partial(chain_body, True), 0)

    wait(wmod_copies(1))
    wait(wmod_copies(2))
    modulation(1)
    modulation(2)
    SB = MB // seg
    n_blk = n_seg // SB

    def resid(i):
        sl = pl.ds(i * SB, SB)
        return (xs[sl].astype(F32).reshape(MB, D)
                + modrow(2) * attn[sl].astype(F32).reshape(MB, D))

    def ffn_in(i):
        h = _layernorm(resid(i)) * (1.0 + modrow(4)) + modrow(3)
        r, k = MB // 2, D // 2
        for n, t in enumerate(_strassen_lhs(h[:r, :k], h[:r, k:], h[r:, :k], h[r:, k:])):
            h2[n] = t

    def out_copy(i):
        sl = pl.ds(pl.multiple_of(i * MB, MB), MB)
        return pltpu.make_async_copy(res.at[sl, :], out_hbm.at[sl, :], sems.at[S_OUT])

    ffn_in(0)

    def ffn_body(i, carry):
        for j in range(FH):
            g = _strassen_out(lambda n: _dot(h2[n], _w(wf[n, pl.ds(j * UP, UP), :])))
            u = _strassen_out(lambda n: _dot(h2[n], _w(wf[n, pl.ds((FH + j) * UP, UP), :])))
            for n, t in enumerate(_strassen_lhs(*(_silu(a) * b for a, b in zip(g, u)))):
                act[n, :, pl.ds(j * LANE, LANE)] = t
        ffn_in(jnp.minimum(i + 1, n_blk - 1))
        c = [_strassen_out(lambda n: _dot(act[n], _w(wf[n, pl.ds(2 * FH * UP + j * DN, DN), :])))
             for j in range(DH)]
        y = jnp.concatenate(
            [jnp.concatenate([t[2 * r] for t in c] + [t[2 * r + 1] for t in c], axis=1)
             for r in range(2)], axis=0)
        res[pl.ds(pl.multiple_of(i * MB, MB), MB), :] = (resid(i) + modrow(5) * y).astype(BF16)
        out_copy(i).start()
        return carry

    lax.fori_loop(0, n_blk, ffn_body, 0)
    pltpu.make_async_copy(res, out_hbm, sems.at[S_OUT]).wait()


@functools.partial(jax.jit, static_argnames=("A_seg_len",))
def pallas_adaLN_cond__memory_aug_recurrent_mem_tr__glu_gated_swiglu__prompt_kernel(
    A_x, A_mem0, A_Wq, A_Wk, A_Wv, A_Wo, A_seg_len, B_x, B_w1, B_w3, B_w2, c, w_mod,
):
    del B_x
    B, S, D = A_x.shape
    _, H, Dh = A_Wq.shape
    M = A_mem0.shape[1]
    F = B_w1.shape[1]
    seg = int(A_seg_len)
    n_seg = S // seg
    assert B == 1 and Dh == LANE and S % seg == 0 and S % MB == 0 and MB % seg == 0
    kern = functools.partial(_kernel, seg=seg, n_seg=n_seg, n_mem=M, n_head=H, d_model=D, d_ff=F)
    hbm = pl.BlockSpec(memory_space=pl.ANY)
    vmem = pl.BlockSpec(memory_space=pltpu.VMEM)
    out = pl.pallas_call(
        kern,
        out_shape=jax.ShapeDtypeStruct((S, D), A_x.dtype),
        in_specs=[vmem, vmem] + [hbm] * 9,
        out_specs=hbm,
        scratch_shapes=[
            pltpu.VMEM((4 * D // LANE, D // 2, LANE), U32),
            pltpu.VMEM((3 * H, D // 2, LANE), U32),
            pltpu.VMEM((D // LANE, H * Dh // 2, LANE), U32),
            pltpu.VMEM((7, 3 * D * F // (8 * LANE), LANE), U32),
            pltpu.VMEM((3 * H, n_seg * PRE, LANE), F32),
            pltpu.VMEM((n_seg, PRE, D), BF16),
            pltpu.VMEM((n_seg * PRE, D), BF16),
            pltpu.VMEM((n_seg, seg, D), BF16),
            pltpu.VMEM((n_seg, seg, D), BF16),
            pltpu.VMEM((M + seg - PRE, D), BF16),
            pltpu.VMEM((6, 8, D), F32),
            pltpu.VMEM((7, MB // 2, D // 2), BF16),
            pltpu.VMEM((7, MB // 2, F // 2), BF16),
            pltpu.VMEM((S, D), BF16),
            pltpu.SemaphoreType.DMA((6 + 3 * H // (2 * PAIRS_PER_IT),)),
        ],
        compiler_params=pltpu.CompilerParams(vmem_limit_bytes=127 * 1024 * 1024),
    )(c, A_mem0.reshape(M, D), A_x.reshape(n_seg, seg, D),
      A_Wq.reshape(D // 2, 2 * H, Dh), A_Wk.reshape(D // 2, 2 * H, Dh),
      A_Wv.reshape(D // 2, 2 * H, Dh),
      A_Wo.reshape(H * Dh, D), B_w1, B_w3, B_w2, w_mod)
    return out.reshape(B, S, D)
```

```python
import functools

import jax
import jax.numpy as jnp
from jax import lax
import jax.experimental.pallas as pl
import jax.experimental.pallas.tpu as pltpu

F32 = jnp.float32
BF16 = jnp.bfloat16
U32 = jnp.uint32
LANE = 128
PRE = 8
HG = 4
SPLIT = 8
AHEAD = 3
CROWS = 8
MB = 128
PAIRS_PER_IT = 2


def _layernorm(x):
    m = jnp.mean(x, axis=-1, keepdims=True)
    d = x - m
    v = jnp.mean(d * d, axis=-1, keepdims=True)
    return d * lax.rsqrt(v + 1e-5)


def _silu(x):
    return x / (1.0 + jnp.exp(-x))


def _w(tile_u32):
    return pltpu.bitcast(tile_u32, BF16)


def _dot(a, b):
    return lax.dot_general(a, b, (((1,), (0,)), ((), ())), preferred_element_type=F32)


def _dot_nt(a, b):
    return lax.dot_general(a, b, (((1,), (1,)), ((), ())), preferred_element_type=F32)


def _strassen_lhs(a11, a12, a21, a22):
    return [t.astype(BF16) for t in
            (a11 + a22, a21 + a22, a11, a22, a11 + a12, a21 - a11, a12 - a22)]


def _strassen_rhs(b11, b12, b21, b22):
    b11, b12, b21, b22 = (t.astype(F32) for t in (b11, b12, b21, b22))
    return [t.astype(BF16) for t in (b11 + b22, b12 - b22, b21 - b11, b11 + b12, b21 + b22)]


def _strassen_out(prod):
    m0, m1, m2, m3, m4 = (prod(i) for i in range(5))
    c12 = m2 + m4
    c21 = m1 + m3
    c22 = (m0 - m1) + m2 + prod(5)
    c11 = (m0 + m3) - m4 + prod(6)
    return c11, c12, c21, c22


def _kernel(c_ref, mem_ref, x_hbm, wq_hbm, wk_hbm, wv_hbm, wo_hbm, w1_hbm, w3_hbm, w2_hbm,
            wmod_hbm, out_hbm,
            wqkv, wo, wraw, aux, xp, hp, xs, attn, lhs, mod, act,
            sems, *, seg, n_seg, n_mem, n_head, d_model, d_ff):
    D, H, M = d_model, n_head, n_mem
    DT = D // LANE
    FT = d_ff // LANE
    L = M + seg
    CUR = seg - PRE
    PP = PAIRS_PER_IT
    n_it = 3 * H // (2 * PP)
    it_per_mat = n_it // 3
    (S_XP, S_X, S_WO, S_FF, S_OUT, S_MOD, S_ST) = range(7)

    WR = wraw.shape[1]
    NP = n_seg * PRE

    def aux_rows(start, size):
        return pl.ds(start if isinstance(start, int) else pl.multiple_of(start, 8), size)

    def pair_copies(w_hbm, i):
        src = w_hbm.bitcast(U32)
        return [pltpu.make_async_copy(
            src.at[:, (i % it_per_mat) * PP + t + par * (H // 2), :],
            wqkv.at[(i * PP + t) * 2 + par], sems.at[S_ST + i])
            for t in range(PP) for par in range(2)]

    def wmod_copies(part):
        src = wmod_hbm.bitcast(U32)
        return [pltpu.make_async_copy(
            src.at[:, pl.ds((part * 2 * DT + j) * LANE, LANE)],
            aux.at[pl.ds(part * WR + j * (D // 2), D // 2), :], sems.at[S_MOD])
            for j in range(2 * DT)]

    def lane_tile(j):
        return pl.ds(pl.multiple_of(j * LANE, LANE), LANE)

    def wo_copy(j):
        return pltpu.make_async_copy(wo_hbm.bitcast(U32).at[:, lane_tile(j)], wo.at[j],
                                     sems.at[S_WO])

    def x_copy(j):
        sl = pl.ds(j * (n_seg // it_per_mat), n_seg // it_per_mat)
        return pltpu.make_async_copy(x_hbm.at[sl], xs.at[sl], sems.at[S_X])

    UP, DN = D // 4, d_ff // 4
    FH, DH = FT // 2, DT // 2

    def ffn_copies():
        cps = []
        for w_hbm, rows, half, base in ((w1_hbm, UP, FH, 0), (w3_hbm, UP, FH, FH * UP),
                                        (w2_hbm, DN, DH, 2 * FH * UP)):
            src = w_hbm.bitcast(U32)
            for j in range(half):
                for kh in range(2):
                    for nh in range(2):
                        cps.append(pltpu.make_async_copy(
                            src.at[pl.ds(kh * rows, rows), pl.ds((j + nh * half) * LANE, LANE)],
                            wraw.at[2 * kh + nh, pl.ds(base + j * rows, rows), :],
                            sems.at[S_FF]))
        return cps

    def start(cps):
        for cp in cps:
            cp.start()

    def wait(cps):
        for cp in cps:
            cp.wait()

    xp_copy = pltpu.make_async_copy(x_hbm.at[:, pl.ds(CUR, PRE), :], xp, sems.at[S_XP])

    def modulation(part):
        sc = jnp.broadcast_to(_silu(c_ref[...].astype(F32)), (8, D))
        for j in range(2 * DT):
            r = _dot(sc, _w(aux[pl.ds(part * WR + j * (D // 2), D // 2), :]))
            mod[2 * part + j // DT, :, pl.ds((j % DT) * LANE, LANE)] = r

    def modrow(i):
        return mod[i, 0:1, :]

    xp_copy.start()
    start(wmod_copies(0))
    start(pair_copies(wq_hbm, 0))
    xp_copy.wait()
    xn = _layernorm(xp[...].astype(F32).reshape(n_seg * PRE, D))
    wait(wmod_copies(0))
    for i in range(1, AHEAD):
        start(pair_copies(wq_hbm, i))
    modulation(0)
    hn = xn * (1.0 + modrow(1)) + modrow(0)
    r, k = NP // 2, D // 2
    for n, t in enumerate(_strassen_lhs(hn[:r, :k], hn[:r, k:], hn[r:, :k], hn[r:, k:])):
        hp[n] = t

    def pro_body(w_next, extra, i, carry):
        wait(pair_copies(wq_hbm, i))
        for t in range(PP):
            a = wqkv[(i * PP + t) * 2]
            b = wqkv[(i * PP + t) * 2 + 1]
            heads = ((a & jnp.uint32(0xFFFF)) | (b << 16), (a >> 16) | (b & jnp.uint32(0xFFFF0000)))
            for par in range(2):
                wqkv[(i * PP + t) * 2 + par] = heads[par]
            if t == PP - 1 and w_next is not None:
                start(pair_copies(w_next, i + AHEAD))
                if extra is not None:
                    extra((i + AHEAD) % it_per_mat).start()
            blocks = [_w(heads[par][kh * (D // 4):(kh + 1) * (D // 4)])
                      for kh in range(2) for par in range(2)]
            sums = _strassen_rhs(*blocks)
            rhs = (sums[0], blocks[0], sums[1], sums[2], blocks[3], sums[3], sums[4])
            c = _strassen_out(lambda n: _dot(hp[n], rhs[n]))
            for n in (1, 2, 3, 0):
                r0 = 5 * WR + ((i * PP + t) * 2 + n % 2) * NP + (n // 2) * (NP // 2)
                aux[aux_rows(r0, NP // 2), :] = pltpu.bitcast(c[n], U32)
        return carry

    for m, (w_hbm, extra) in enumerate(((wq_hbm, None), (wk_hbm, wo_copy), (wv_hbm, x_copy))):
        lax.fori_loop(max(m * it_per_mat - AHEAD, 0), (m + 1) * it_per_mat - AHEAD,
                      functools.partial(pro_body, w_hbm, extra), 0)
    lax.fori_loop(n_it - AHEAD, n_it, functools.partial(pro_body, None, None), 0)
    wait([wo_copy(j) for j in range(DT)])
    wait([x_copy(j) for j in range(it_per_mat)])
    start(ffn_copies())
    start(wmod_copies(1))
    start(wmod_copies(2))

    def seg_rows(s):
        xn = _layernorm(xs[s].astype(F32)[0:CUR])
        return xn * (1.0 + modrow(1)) + modrow(0)

    lhs[...] = jnp.concatenate([mem_ref[...].astype(F32), seg_rows(0)], axis=0).astype(BF16)
    scale = float(LANE) ** -0.5
    NG = H // HG

    def chain_body(combine, s, carry):
        row = lax.broadcasted_iota(jnp.int32, (L, L), 0)
        col = lax.broadcasted_iota(jnp.int32, (L, L), 1)
        mask = (row < M) | (row >= col)
        q, k, v, p, inv, ov = {}, {}, {}, {}, {}, {}

        def heads(g):
            return range(g * HG, (g + 1) * HG)

        def proj(m, h):
            done = aux[aux_rows(5 * WR + (m * H + h) * NP + s * PRE, PRE), :]
            return jnp.concatenate([_dot(lhs[...], _w(wqkv[m * H + h])),
                                    pltpu.bitcast(done, F32)], axis=0)

        def probs(g):
            for h in heads(g):
                z = jnp.where(mask, _dot_nt(q[h], k[h]) * scale, -1e9)
                p[h] = jnp.exp(z - jnp.max(z, axis=-1, keepdims=True))
                inv[h] = 1.0 / jnp.sum(p[h], axis=-1, keepdims=True)

        def values(g):
            for h in heads(g):
                ov[h] = _dot(p[h], v[h]) * inv[h]

        def out_proj(h0, h1):
            o = jnp.concatenate([ov[h] for h in range(h0, h1)], axis=1)
            return jnp.concatenate(
                [_dot(o, _w(wo[j, pl.ds(h0 * LANE // 2, (h1 - h0) * LANE // 2), :]))
                 for j in range(DT)], axis=1)

        def combine_weights(part):
            nr = WR // (n_seg - n_seg // 2)
            for r in range(part * CROWS, nr, 2 * H * CROWS) if combine else ():
                r0 = (s - n_seg // 2) * nr + r
                blocks = (_w(wraw[i, aux_rows(r0, CROWS), :]) for i in range(4))
                for i, t in enumerate(_strassen_rhs(*blocks)):
                    aux[aux_rows(i * WR + r0, CROWS), :] = pltpu.bitcast(t, U32)

        for g in range(NG):
            for h in heads(g):
                combine_weights(h)
                q[h] = proj(0, h)
                k[h] = proj(1, h).astype(BF16)
            if g >= 1:
                probs(g - 1)
        for g in range(NG):
            for h in heads(g):
                combine_weights(H + h)
                v[h] = proj(2, h).astype(BF16)
            if g == 0:
                probs(NG - 1)
            else:
                values(g - 1)
        nxt = seg_rows(jnp.minimum(s + 1, n_seg - 1))
        o = out_proj(0, SPLIT)
        values(NG - 1)
        o = o + out_proj(SPLIT, H)
        attn[s] = o[M:].astype(BF16)
        lhs[...] = jnp.concatenate([o[:M], nxt], axis=0).astype(BF16)
        return carry

    lax.fori_loop(0, n_seg // 2, functools.partial(chain_body, False), 0)
    wait(ffn_copies())
    wait(wmod_copies(1))
    wait(wmod_copies(2))
    modulation(1)
    modulation(2)
    lax.fori_loop(n_seg // 2, n_seg, functools.partial(chain_body, True), 0)

    SB = MB // seg
    n_blk = n_seg // SB

    def resid(sg, n, cols=slice(None)):
        sl = pl.ds(sg, n)
        r = xs[sl, :, cols].astype(F32) + mod[2, 0:1, cols] * attn[sl, :, cols].astype(F32)
        return r.reshape(n * seg, r.shape[2])

    def ffn_in(i):
        h = _layernorm(resid(i * SB, SB)) * (1.0 + modrow(4)) + modrow(3)
        r, k = MB // 2, D // 2
        for n, t in enumerate(_strassen_lhs(h[:r, :k], h[:r, k:], h[r:, :k], h[r:, k:])):
            act[n, :, pl.ds(d_ff // 2, k)] = t

    def product(col0, row0, rows, n):
        if n in (1, 4):
            w = wraw[0 if n == 1 else 3, pl.ds(row0, rows), :]
        else:
            w = aux[pl.ds((0, 2, 3, 5, 6).index(n) * WR + row0, rows), :]
        return _dot(act[n, :, pl.ds(col0, 2 * rows)], _w(w))

    ffn_in(0)

    def ffn_body(i, carry):
        for j in range(FH):
            g = _strassen_out(functools.partial(product, d_ff // 2, j * UP, UP))
            u = _strassen_out(functools.partial(product, d_ff // 2, (FH + j) * UP, UP))
            for n, t in enumerate(_strassen_lhs(*(_silu(a) * b for a, b in zip(g, u)))):
                act[n, :, pl.ds(j * LANE, LANE)] = t
        ffn_in(jnp.minimum(i + 1, n_blk - 1))
        for j in range(DH):
            c = _strassen_out(functools.partial(product, 0, 2 * FH * UP + j * DN, DN))
            for n in (1, 2, 3, 0):
                sg = i * SB + (n // 2) * (SB // 2)
                cols = slice((j + (n % 2) * DH) * LANE, (j + (n % 2) * DH + 1) * LANE)
                y = resid(sg, SB // 2, cols) + mod[5, 0:1, cols] * c[n]
                attn[pl.ds(sg, SB // 2), :, cols] = y.reshape(SB // 2, seg, LANE).astype(BF16)
        sl = pl.ds(i * SB, SB)
        pltpu.make_async_copy(attn.at[sl], out_hbm.at[sl], sems.at[S_OUT]).start()
        return carry

    lax.fori_loop(0, n_blk, ffn_body, 0)
    pltpu.make_async_copy(attn, out_hbm, sems.at[S_OUT]).wait()


@functools.partial(jax.jit, static_argnames=("A_seg_len",))
def pallas_adaLN_cond__memory_aug_recurrent_mem_tr__glu_gated_swiglu__prompt_kernel(
    A_x, A_mem0, A_Wq, A_Wk, A_Wv, A_Wo, A_seg_len, B_x, B_w1, B_w3, B_w2, c, w_mod,
):
    del B_x
    B, S, D = A_x.shape
    _, H, Dh = A_Wq.shape
    M = A_mem0.shape[1]
    F = B_w1.shape[1]
    seg = int(A_seg_len)
    n_seg = S // seg
    assert B == 1 and Dh == LANE and S % seg == 0 and S % MB == 0 and MB % seg == 0
    kern = functools.partial(_kernel, seg=seg, n_seg=n_seg, n_mem=M, n_head=H, d_model=D, d_ff=F)
    hbm = pl.BlockSpec(memory_space=pl.ANY)
    vmem = pl.BlockSpec(memory_space=pltpu.VMEM)
    out = pl.pallas_call(
        kern,
        out_shape=jax.ShapeDtypeStruct((n_seg, seg, D), A_x.dtype),
        in_specs=[vmem, vmem] + [hbm] * 9,
        out_specs=hbm,
        scratch_shapes=[
            pltpu.VMEM((3 * H, D // 2, LANE), U32),
            pltpu.VMEM((D // LANE, H * Dh // 2, LANE), U32),
            pltpu.VMEM((4, 3 * D * F // (8 * LANE), LANE), U32),
            pltpu.VMEM((5 * 3 * D * F // (8 * LANE) + 3 * H * n_seg * PRE, LANE), U32),
            pltpu.VMEM((n_seg, PRE, D), BF16),
            pltpu.VMEM((7, n_seg * PRE // 2, D // 2), BF16),
            pltpu.VMEM((n_seg, seg, D), BF16),
            pltpu.VMEM((n_seg, seg, D), BF16),
            pltpu.VMEM((M + seg - PRE, D), BF16),
            pltpu.VMEM((6, 8, D), F32),
            pltpu.VMEM((7, MB // 2, (F + D) // 2), BF16),
            pltpu.SemaphoreType.DMA((6 + 3 * H // (2 * PAIRS_PER_IT),)),
        ],
        compiler_params=pltpu.CompilerParams(vmem_limit_bytes=127 * 1024 * 1024),
    )(c, A_mem0.reshape(M, D), A_x.reshape(n_seg, seg, D),
      A_Wq.reshape(D // 2, 2 * H, Dh), A_Wk.reshape(D // 2, 2 * H, Dh),
      A_Wv.reshape(D // 2, 2 * H, Dh),
      A_Wo.reshape(H * Dh, D), B_w1, B_w3, B_w2, w_mod)
    return out.reshape(B, S, D)
```

```python
import functools

import jax
import jax.numpy as jnp
from jax import lax
import jax.experimental.pallas as pl
import jax.experimental.pallas.tpu as pltpu

F32 = jnp.float32
BF16 = jnp.bfloat16
U32 = jnp.uint32
LANE = 128
PRE = 8
HG = 4
SPLIT = 8
AHEAD = 3
CROWS = 8
MB = 128
PAIRS_PER_IT = 2


def _layernorm(x):
    m = jnp.mean(x, axis=-1, keepdims=True)
    d = x - m
    v = jnp.mean(d * d, axis=-1, keepdims=True)
    return d * lax.rsqrt(v + 1e-5)


def _silu(x):
    return x / (1.0 + jnp.exp(-x))


def _w(tile_u32):
    return pltpu.bitcast(tile_u32, BF16)


def _dot(a, b):
    return lax.dot_general(a, b, (((1,), (0,)), ((), ())), preferred_element_type=F32)


def _dot_nt(a, b):
    return lax.dot_general(a, b, (((1,), (1,)), ((), ())), preferred_element_type=F32)


def _strassen_lhs(a11, a12, a21, a22):
    return [t.astype(BF16) for t in
            (a11 + a22, a21 + a22, a11, a22, a11 + a12, a21 - a11, a12 - a22)]


def _strassen_rhs(b11, b12, b21, b22):
    b11, b12, b21, b22 = (t.astype(F32) for t in (b11, b12, b21, b22))
    return [t.astype(BF16) for t in (b11 + b22, b12 - b22, b21 - b11, b11 + b12, b21 + b22)]


def _strassen_out(prod):
    m1, m4, m2, m3, m0 = (prod(i) for i in (1, 4, 2, 3, 0))
    c12 = m2 + m4
    c21 = m1 + m3
    c22 = (m0 - m1) + m2 + prod(5)
    c11 = (m0 + m3) - m4 + prod(6)
    return c11, c12, c21, c22


def _kernel(c_ref, mem_ref, x_hbm, wq_hbm, wk_hbm, wv_hbm, wo_hbm, w1_hbm, w3_hbm, w2_hbm,
            wmod_hbm, out_hbm,
            wqkv, wo, wraw, aux, xp, hp, xs, attn, lhs, mod, act,
            sems, *, seg, n_seg, n_mem, n_head, d_model, d_ff):
    D, H, M = d_model, n_head, n_mem
    DT = D // LANE
    FT = d_ff // LANE
    L = M + seg
    CUR = seg - PRE
    PP = PAIRS_PER_IT
    n_it = 3 * H // (2 * PP)
    it_per_mat = n_it // 3
    (S_XP, S_X, S_WO, S_FF, S_OUT, S_MOD, S_ST) = range(7)

    WR = wraw.shape[1]
    NP = n_seg * PRE

    def aux_rows(start, size):
        return pl.ds(start if isinstance(start, int) else pl.multiple_of(start, 8), size)

    def landing(i, t, par):
        return i % 4, aux_rows((((i // 4) % 2 * PP + t) * 2 + par) * (D // 2), D // 2)

    def pair_copies(w_hbm, i):
        src = w_hbm.bitcast(U32)
        return [pltpu.make_async_copy(
            src.at[:, (i % it_per_mat) * PP + t + par * (H // 2), :],
            wraw.at[landing(i, t, par)], sems.at[S_ST + i % 8])
            for t in range(PP) for par in range(2)]

    def lane_tile(j):
        return pl.ds(j * LANE if isinstance(j, int) else pl.multiple_of(j * LANE, LANE), LANE)

    def wmod_copy(part, j):
        return pltpu.make_async_copy(
            wmod_hbm.bitcast(U32).at[:, lane_tile(part * 2 * DT + j)],
            aux.at[aux_rows(part * WR + j * (D // 2), D // 2), :], sems.at[S_MOD])

    def wmod_copies(part):
        return [wmod_copy(part, j) for j in range(2 * DT)]

    def wo_copy(j):
        return pltpu.make_async_copy(wo_hbm.bitcast(U32).at[:, lane_tile(j)], wo.at[j],
                                     sems.at[S_WO])

    def x_copy(j):
        sl = pl.ds(j * (n_seg // it_per_mat), n_seg // it_per_mat)
        return pltpu.make_async_copy(x_hbm.at[sl], xs.at[sl], sems.at[S_X])

    UP, DN = D // 4, d_ff // 4
    FH, DH = FT // 2, DT // 2

    def ffn_copy(w_hbm, rows, half, base, kh, j):
        return pltpu.make_async_copy(
            w_hbm.bitcast(U32).at[aux_rows(kh * rows, rows), lane_tile(j)],
            wraw.at[2 * kh + j // half, aux_rows(base + (j % half) * rows, rows), :],
            sems.at[S_FF])

    def prefetch_ffn(s):
        @pl.when(s < FT)
        def _():
            for kh in range(2):
                ffn_copy(w1_hbm, UP, FH, 0, kh, s).start()
                ffn_copy(w3_hbm, UP, FH, FH * UP, kh, s).start()

        @pl.when(s < 2 * DT)
        def _():
            ffn_copy(w2_hbm, DN, DH, 2 * FH * UP, s // DT, s % DT).start()
            wmod_copy(1, s).start()
            wmod_copy(2, s).start()

    def start(cps):
        for cp in cps:
            cp.start()

    def wait(cps):
        for cp in cps:
            cp.wait()

    xp_copy = pltpu.make_async_copy(x_hbm.at[:, pl.ds(CUR, PRE), :], xp, sems.at[S_XP])

    def modulation(part):
        sc = jnp.broadcast_to(_silu(c_ref[...].astype(F32)), (8, D))
        for j in range(2 * DT):
            r = _dot(sc, _w(aux[pl.ds(part * WR + j * (D // 2), D // 2), :]))
            mod[2 * part + j // DT, :, pl.ds((j % DT) * LANE, LANE)] = r

    def modrow(i):
        return mod[i, 0:1, :]

    xp_copy.start()
    start(wmod_copies(0))
    start(pair_copies(wq_hbm, 0))
    xp_copy.wait()
    xn = _layernorm(xp[...].astype(F32).reshape(n_seg * PRE, D))
    wait(wmod_copies(0))
    for i in range(1, AHEAD):
        start(pair_copies(wq_hbm, i))
    modulation(0)
    hn = xn * (1.0 + modrow(1)) + modrow(0)
    r, k = NP // 2, D // 2
    for n, t in enumerate(_strassen_lhs(hn[:r, :k], hn[:r, k:], hn[r:, :k], hn[r:, k:])):
        hp[n] = t

    def pro_body(w_next, extra, i, carry):
        wait(pair_copies(wq_hbm, i))
        for t in range(PP):
            a = wraw[landing(i, t, 0)]
            b = wraw[landing(i, t, 1)]
            heads = ((a & jnp.uint32(0xFFFF)) | (b << 16), (a >> 16) | (b & jnp.uint32(0xFFFF0000)))
            for par in range(2):
                wqkv[(i * PP + t) * 2 + par] = heads[par]
            if t == PP - 1 and w_next is not None:
                start(pair_copies(w_next, i + AHEAD))
                if extra is not None:
                    extra((i + AHEAD) % it_per_mat).start()
            blocks = [_w(heads[par][kh * (D // 4):(kh + 1) * (D // 4)])
                      for kh in range(2) for par in range(2)]
            sums = _strassen_rhs(*blocks)
            rhs = (sums[0], blocks[0], sums[1], sums[2], blocks[3], sums[3], sums[4])
            c = _strassen_out(lambda n: _dot(hp[n], rhs[n]))
            for n in (1, 2, 3, 0):
                r0 = 5 * WR + ((i * PP + t) * 2 + n % 2) * NP + (n // 2) * (NP // 2)
                aux[aux_rows(r0, NP // 2), :] = pltpu.bitcast(c[n], U32)
        return carry

    for m, (w_hbm, extra) in enumerate(((wq_hbm, None), (wk_hbm, wo_copy), (wv_hbm, x_copy))):
        lax.fori_loop(max(m * it_per_mat - AHEAD, 0), (m + 1) * it_per_mat - AHEAD,
                      functools.partial(pro_body, w_hbm, extra), 0)
    lax.fori_loop(n_it - AHEAD, n_it, functools.partial(pro_body, None, None), 0)
    wait([wo_copy(j) for j in range(DT)])
    wait([x_copy(j) for j in range(it_per_mat)])

    def seg_rows(s):
        xn = _layernorm(xs[s].astype(F32)[0:CUR])
        return xn * (1.0 + modrow(1)) + modrow(0)

    lhs[...] = jnp.concatenate([mem_ref[...].astype(F32), seg_rows(0)], axis=0).astype(BF16)
    scale = float(LANE) ** -0.5
    NG = H // HG

    def chain_body(combine, s, carry):
        if not combine:
            prefetch_ffn(s)
        row = lax.broadcasted_iota(jnp.int32, (L, L), 0)
        col = lax.broadcasted_iota(jnp.int32, (L, L), 1)
        mask = (row < M) | (row >= col)
        q, k, v, p, inv, ov = {}, {}, {}, {}, {}, {}

        def heads(g):
            return range(g * HG, (g + 1) * HG)

        def proj(m, h):
            done = aux[aux_rows(5 * WR + (m * H + h) * NP + s * PRE, PRE), :]
            return jnp.concatenate([_dot(lhs[...], _w(wqkv[m * H + h])),
                                    pltpu.bitcast(done, F32)], axis=0)

        def probs(g):
            for h in heads(g):
                z = jnp.where(mask, _dot_nt(q[h], k[h]) * scale, -1e9)
                p[h] = jnp.exp(z - jnp.max(z, axis=-1, keepdims=True))
                inv[h] = 1.0 / jnp.sum(p[h], axis=-1, keepdims=True)

        def values(g):
            for h in heads(g):
                ov[h] = _dot(p[h], v[h]) * inv[h]

        def out_proj(h0, h1):
            o = jnp.concatenate([ov[h] for h in range(h0, h1)], axis=1)
            return jnp.concatenate(
                [_dot(o, _w(wo[j, pl.ds(h0 * LANE // 2, (h1 - h0) * LANE // 2), :]))
                 for j in range(DT)], axis=1)

        def combine_weights(part):
            nr = WR // (n_seg - n_seg // 2)
            for r in range(part * CROWS, nr, 2 * H * CROWS) if combine else ():
                r0 = (s - n_seg // 2) * nr + r
                blocks = (_w(wraw[i, aux_rows(r0, CROWS), :]) for i in range(4))
                for i, t in enumerate(_strassen_rhs(*blocks)):
                    aux[aux_rows(i * WR + r0, CROWS), :] = pltpu.bitcast(t, U32)

        for g in range(NG):
            for h in heads(g):
                combine_weights(h)
                q[h] = proj(0, h)
                k[h] = proj(1, h).astype(BF16)
            if g >= 1:
                probs(g - 1)
        for g in range(NG):
            for h in heads(g):
                combine_weights(H + h)
                v[h] = proj(2, h).astype(BF16)
            if g == 0:
                probs(NG - 1)
            else:
                values(g - 1)
        nxt = seg_rows(jnp.minimum(s + 1, n_seg - 1))
        o = out_proj(0, SPLIT)
        values(NG - 1)
        o = o + out_proj(SPLIT, H)
        attn[s] = o[M:].astype(BF16)
        lhs[...] = jnp.concatenate([o[:M], nxt], axis=0).astype(BF16)
        return carry

    lax.fori_loop(0, n_seg // 2, functools.partial(chain_body, False), 0)
    pltpu.make_async_copy(wraw, wraw, sems.at[S_FF]).wait()
    wait(wmod_copies(1))
    wait(wmod_copies(2))
    modulation(1)
    modulation(2)
    lax.fori_loop(n_seg // 2, n_seg, functools.partial(chain_body, True), 0)

    SB = MB // seg
    n_blk = n_seg // SB

    def resid(sg, n, cols=slice(None)):
        sl = pl.ds(sg, n)
        r = xs[sl, :, cols].astype(F32) + mod[2, 0:1, cols] * attn[sl, :, cols].astype(F32)
        return r.reshape(n * seg, r.shape[2])

    def ffn_in(i):
        h = _layernorm(resid(i * SB, SB)) * (1.0 + modrow(4)) + modrow(3)
        r, k = MB // 2, D // 2
        for n, t in enumerate(_strassen_lhs(h[:r, :k], h[:r, k:], h[r:, :k], h[r:, k:])):
            act[n, :, pl.ds(d_ff // 2, k)] = t

    def product(col0, row0, rows, n):
        if n in (1, 4):
            w = wraw[0 if n == 1 else 3, pl.ds(row0, rows), :]
        else:
            w = aux[pl.ds((0, 2, 3, 5, 6).index(n) * WR + row0, rows), :]
        return _dot(act[n, :, pl.ds(col0, 2 * rows)], _w(w))

    ffn_in(0)

    def ffn_body(i, carry):
        for j in range(FH):
            g = _strassen_out(functools.partial(product, d_ff // 2, j * UP, UP))
            u = _strassen_out(functools.partial(product, d_ff // 2, (FH + j) * UP, UP))
            for n, t in enumerate(_strassen_lhs(*(_silu(a) * b for a, b in zip(g, u)))):
                act[n, :, pl.ds(j * LANE, LANE)] = t
        ffn_in(jnp.minimum(i + 1, n_blk - 1))
        for j in range(DH):
            c = _strassen_out(functools.partial(product, 0, 2 * FH * UP + j * DN, DN))
            for n in (1, 2, 3, 0):
                sg = i * SB + (n // 2) * (SB // 2)
                cols = slice((j + (n % 2) * DH) * LANE, (j + (n % 2) * DH + 1) * LANE)
                y = resid(sg, SB // 2, cols) + mod[5, 0:1, cols] * c[n]
                attn[pl.ds(sg, SB // 2), :, cols] = y.reshape(SB // 2, seg, LANE).astype(BF16)
        sl = pl.ds(i * SB, SB)
        pltpu.make_async_copy(attn.at[sl], out_hbm.at[sl], sems.at[S_OUT]).start()
        return carry

    lax.fori_loop(0, n_blk, ffn_body, 0)
    pltpu.make_async_copy(attn, out_hbm, sems.at[S_OUT]).wait()


@functools.partial(jax.jit, static_argnames=("A_seg_len",))
def pallas_adaLN_cond__memory_aug_recurrent_mem_tr__glu_gated_swiglu__prompt_kernel(
    A_x, A_mem0, A_Wq, A_Wk, A_Wv, A_Wo, A_seg_len, B_x, B_w1, B_w3, B_w2, c, w_mod,
):
    del B_x
    B, S, D = A_x.shape
    _, H, Dh = A_Wq.shape
    M = A_mem0.shape[1]
    F = B_w1.shape[1]
    seg = int(A_seg_len)
    n_seg = S // seg
    assert max(F, 2 * D) // LANE <= n_seg // 2 and AHEAD < 8
    assert B == 1 and Dh == LANE and S % seg == 0 and S % MB == 0 and MB % seg == 0
    kern = functools.partial(_kernel, seg=seg, n_seg=n_seg, n_mem=M, n_head=H, d_model=D, d_ff=F)
    hbm = pl.BlockSpec(memory_space=pl.ANY)
    vmem = pl.BlockSpec(memory_space=pltpu.VMEM)
    out = pl.pallas_call(
        kern,
        out_shape=jax.ShapeDtypeStruct((n_seg, seg, D), A_x.dtype),
        in_specs=[vmem, vmem] + [hbm] * 9,
        out_specs=hbm,
        scratch_shapes=[
            pltpu.VMEM((3 * H, D // 2, LANE), U32),
            pltpu.VMEM((D // LANE, H * Dh // 2, LANE), U32),
            pltpu.VMEM((4, 3 * D * F // (8 * LANE), LANE), U32),
            pltpu.VMEM((5 * 3 * D * F // (8 * LANE) + 3 * H * n_seg * PRE, LANE), U32),
            pltpu.VMEM((n_seg, PRE, D), BF16),
            pltpu.VMEM((7, n_seg * PRE // 2, D // 2), BF16),
            pltpu.VMEM((n_seg, seg, D), BF16),
            pltpu.VMEM((n_seg, seg, D), BF16),
            pltpu.VMEM((M + seg - PRE, D), BF16),
            pltpu.VMEM((6, 8, D), F32),
            pltpu.VMEM((7, MB // 2, (F + D) // 2), BF16),
            pltpu.SemaphoreType.DMA((6 + 8,)),
        ],
        compiler_params=pltpu.CompilerParams(vmem_limit_bytes=127 * 1024 * 1024),
    )(c, A_mem0.reshape(M, D), A_x.reshape(n_seg, seg, D),
      A_Wq.reshape(D // 2, 2 * H, Dh), A_Wk.reshape(D // 2, 2 * H, Dh),
      A_Wv.reshape(D // 2, 2 * H, Dh),
      A_Wo.reshape(H * Dh, D), B_w1, B_w3, B_w2, w_mod)
    return out.reshape(B, S, D)
```

```python
import functools

import jax
import jax.numpy as jnp
from jax import lax
import jax.experimental.pallas as pl
import jax.experimental.pallas.tpu as pltpu

F32 = jnp.float32
BF16 = jnp.bfloat16
U32 = jnp.uint32
LANE = 128
PRE = 8
HG = 4
SPLIT = 8
AHEAD = 3
CROWS = 8
UNROLL = 1
MB = 128
PAIRS_PER_IT = 2


def _layernorm(x):
    m = jnp.mean(x, axis=-1, keepdims=True)
    d = x - m
    v = jnp.mean(d * d, axis=-1, keepdims=True)
    return d * lax.rsqrt(v + 1e-5)


def _silu(x):
    return x / (1.0 + jnp.exp(-x))


def _w(tile_u32):
    return pltpu.bitcast(tile_u32, BF16)


def _dot(a, b):
    return lax.dot_general(a, b, (((1,), (0,)), ((), ())), preferred_element_type=F32)


def _dot_nt(a, b):
    return lax.dot_general(a, b, (((1,), (1,)), ((), ())), preferred_element_type=F32)


def _strassen_lhs(a11, a12, a21, a22):
    return [t.astype(BF16) for t in
            (a11 + a22, a21 + a22, a11, a22, a11 + a12, a21 - a11, a12 - a22)]


def _strassen_rhs(b11, b12, b21, b22):
    b11, b12, b21, b22 = (t.astype(F32) for t in (b11, b12, b21, b22))
    return [t.astype(BF16) for t in (b11 + b22, b12 - b22, b21 - b11, b11 + b12, b21 + b22)]


def _strassen_out(prod):
    m1, m4, m2, m3, m0 = (prod(i) for i in (1, 4, 2, 3, 0))
    c12 = m2 + m4
    c21 = m1 + m3
    c22 = (m0 - m1) + m2 + prod(5)
    c11 = (m0 + m3) - m4 + prod(6)
    return c11, c12, c21, c22


def _kernel(c_ref, mem_ref, x_hbm, wq_hbm, wk_hbm, wv_hbm, wo_hbm, w1_hbm, w3_hbm, w2_hbm,
            wmod_hbm, out_hbm,
            wqkv, wo, wraw, aux, xp, hp, xs, attn, lhs, mod, act,
            sems, *, seg, n_seg, n_mem, n_head, d_model, d_ff):
    D, H, M = d_model, n_head, n_mem
    DT = D // LANE
    FT = d_ff // LANE
    L = M + seg
    CUR = seg - PRE
    PP = PAIRS_PER_IT
    n_it = 3 * H // (2 * PP)
    it_per_mat = n_it // 3
    (S_XP, S_X, S_WO, S_FF, S_OUT, S_MOD, S_ST) = range(7)

    WR = wraw.shape[1]
    NP = n_seg * PRE

    def aux_rows(start, size):
        return pl.ds(start if isinstance(start, int) else pl.multiple_of(start, 8), size)

    def landing(i, t, par):
        return i % 4, aux_rows((((i // 4) % 2 * PP + t) * 2 + par) * (D // 2), D // 2)

    def pair_copies(w_hbm, i):
        src = w_hbm.bitcast(U32)
        return [pltpu.make_async_copy(
            src.at[:, (i % it_per_mat) * PP + t + par * (H // 2), :],
            wraw.at[landing(i, t, par)], sems.at[S_ST + i % 8])
            for t in range(PP) for par in range(2)]

    def lane_tile(j):
        return pl.ds(j * LANE if isinstance(j, int) else pl.multiple_of(j * LANE, LANE), LANE)

    def wmod_copy(part, j):
        return pltpu.make_async_copy(
            wmod_hbm.bitcast(U32).at[:, lane_tile(part * 2 * DT + j)],
            aux.at[aux_rows(part * WR + j * (D // 2), D // 2), :], sems.at[S_MOD])

    def wmod_copies(part):
        return [wmod_copy(part, j) for j in range(2 * DT)]

    def wo_copy(j):
        return pltpu.make_async_copy(wo_hbm.bitcast(U32).at[:, lane_tile(j)], wo.at[j],
                                     sems.at[S_WO])

    def x_copy(j):
        sl = pl.ds(j * (n_seg // it_per_mat), n_seg // it_per_mat)
        return pltpu.make_async_copy(x_hbm.at[sl], xs.at[sl], sems.at[S_X])

    UP, DN = D // 4, d_ff // 4
    FH, DH = FT // 2, DT // 2

    def ffn_copy(w_hbm, rows, half, base, kh, j):
        nh = (j >= half).astype(jnp.int32)
        return pltpu.make_async_copy(
            w_hbm.bitcast(U32).at[pl.ds(kh * rows, rows), lane_tile(j)],
            wraw.at[2 * nh + kh, aux_rows(base + (j - nh * half) * rows, rows), :],
            sems.at[S_FF])

    def prefetch_ffn(s, kh):
        @pl.when(s < FT)
        def _():
            ffn_copy(w1_hbm, UP, FH, 0, kh, s).start()
            ffn_copy(w3_hbm, UP, FH, FH * UP, kh, s).start()

        @pl.when(s < DT)
        def _():
            ffn_copy(w2_hbm, DN, DH, 2 * FH * UP, kh, s).start()

        @pl.when(s < 2 * DT)
        def _():
            wmod_copy(1 + kh, s).start()

    def start(cps):
        for cp in cps:
            cp.start()

    def wait(cps):
        for cp in cps:
            cp.wait()

    xp_copy = pltpu.make_async_copy(x_hbm.at[:, pl.ds(CUR, PRE), :], xp, sems.at[S_XP])

    def modulation(part):
        sc = jnp.broadcast_to(_silu(c_ref[...].astype(F32)), (8, D))
        for j in range(2 * DT):
            r = _dot(sc, _w(aux[pl.ds(part * WR + j * (D // 2), D // 2), :]))
            mod[2 * part + j // DT, :, pl.ds((j % DT) * LANE, LANE)] = r

    def modrow(i):
        return mod[i, 0:1, :]

    xp_copy.start()
    start(wmod_copies(0))
    start(pair_copies(wq_hbm, 0))
    xp_copy.wait()
    xn = _layernorm(xp[...].astype(F32).reshape(n_seg * PRE, D))
    wait(wmod_copies(0))
    for i in range(1, AHEAD):
        start(pair_copies(wq_hbm, i))
    modulation(0)
    hn = xn * (1.0 + modrow(1)) + modrow(0)
    r, k = NP // 2, D // 2
    for n, t in enumerate(_strassen_lhs(hn[:r, :k], hn[:r, k:], hn[r:, :k], hn[r:, k:])):
        hp[n] = t

    def pro_body(w_next, extra, i, carry):
        wait(pair_copies(wq_hbm, i))
        for t in range(PP):
            a = wraw[landing(i, t, 0)]
            b = wraw[landing(i, t, 1)]
            heads = ((a & jnp.uint32(0xFFFF)) | (b << 16), (a >> 16) | (b & jnp.uint32(0xFFFF0000)))
            for par in range(2):
                wqkv[(i * PP + t) * 2 + par] = heads[par]
            if t == PP - 1 and w_next is not None:
                start(pair_copies(w_next, i + AHEAD))
                if extra is not None:
                    extra((i + AHEAD) % it_per_mat).start()
            blocks = [_w(heads[par][kh * (D // 4):(kh + 1) * (D // 4)])
                      for kh in range(2) for par in range(2)]
            sums = _strassen_rhs(*blocks)
            rhs = (sums[0], blocks[0], sums[1], sums[2], blocks[3], sums[3], sums[4])
            c = _strassen_out(lambda n: _dot(hp[n], rhs[n]))
            for n in (1, 2, 3, 0):
                r0 = 5 * WR + ((i * PP + t) * 2 + n % 2) * NP + (n // 2) * (NP // 2)
                aux[aux_rows(r0, NP // 2), :] = pltpu.bitcast(c[n], U32)
        return carry

    for m, (w_hbm, extra) in enumerate(((wq_hbm, None), (wk_hbm, wo_copy), (wv_hbm, x_copy))):
        lax.fori_loop(max(m * it_per_mat - AHEAD, 0), (m + 1) * it_per_mat - AHEAD,
                      functools.partial(pro_body, w_hbm, extra), 0)
    lax.fori_loop(n_it - AHEAD, n_it, functools.partial(pro_body, None, None), 0)
    wait([wo_copy(j) for j in range(DT)])
    wait([x_copy(j) for j in range(it_per_mat)])

    def seg_rows(s):
        xn = _layernorm(xs[s].astype(F32)[0:CUR])
        return xn * (1.0 + modrow(1)) + modrow(0)

    lhs[...] = jnp.concatenate([mem_ref[...].astype(F32), seg_rows(0)], axis=0).astype(BF16)
    scale = float(LANE) ** -0.5
    NG = H // HG

    def chain_body(combine, s, carry):
        row = lax.broadcasted_iota(jnp.int32, (L, L), 0)
        col = lax.broadcasted_iota(jnp.int32, (L, L), 1)
        mask = (row < M) | (row >= col)
        q, k, v, p, ov = {}, {}, {}, {}, {}

        def heads(g):
            return range(g * HG, (g + 1) * HG)

        def proj(m, h):
            done = aux[aux_rows(5 * WR + (m * H + h) * NP + s * PRE, PRE), :]
            return jnp.concatenate([_dot(lhs[...], _w(wqkv[m * H + h])),
                                    pltpu.bitcast(done, F32)], axis=0)

        def probs(g):
            for h in heads(g):
                z = jnp.where(mask, _dot_nt(q[h], k[h]) * scale, -1e9)
                e = jnp.exp(z - jnp.max(z, axis=-1, keepdims=True))
                p[h] = e / jnp.sum(e, axis=-1, keepdims=True)

        def values(g):
            for h in heads(g):
                ov[h] = _dot(p[h], v[h])

        def out_proj(h0, h1):
            o = jnp.concatenate([ov[h] for h in range(h0, h1)], axis=1)
            return jnp.concatenate(
                [_dot(o, _w(wo[j, pl.ds(h0 * LANE // 2, (h1 - h0) * LANE // 2), :]))
                 for j in range(DT)], axis=1)

        def combine_weights(part):
            nr = WR // (n_seg - n_seg // 2)
            for r in range(part * CROWS, nr, 2 * H * CROWS) if combine else ():
                r0 = (s - n_seg // 2) * nr + r
                blocks = (_w(wraw[i, aux_rows(r0, CROWS), :]) for i in (0, 2, 1, 3))
                for i, t in enumerate(_strassen_rhs(*blocks)):
                    aux[aux_rows(i * WR + r0, CROWS), :] = pltpu.bitcast(t, U32)

        for g in range(NG):
            for h in heads(g):
                combine_weights(h)
                q[h] = proj(0, h)
                k[h] = proj(1, h).astype(BF16)
            if g >= 1:
                probs(g - 1)
            if not combine and g in (2, 4):
                prefetch_ffn(s, g // 2 - 1)
        for g in range(NG):
            for h in heads(g):
                combine_weights(H + h)
                v[h] = proj(2, h).astype(BF16)
            if g == 0:
                probs(NG - 1)
            else:
                values(g - 1)
        nxt = seg_rows(jnp.minimum(s + 1, n_seg - 1))
        o = out_proj(0, SPLIT)
        values(NG - 1)
        o = o + out_proj(SPLIT, H)
        attn[s] = o[M:].astype(BF16)
        lhs[...] = jnp.concatenate([o[:M], nxt], axis=0).astype(BF16)
        return carry

    lax.fori_loop(0, n_seg // 2, functools.partial(chain_body, False), 0, unroll=UNROLL)
    pltpu.make_async_copy(wraw, wraw, sems.at[S_FF]).wait()
    wait(wmod_copies(1))
    wait(wmod_copies(2))
    modulation(1)
    modulation(2)
    lax.fori_loop(n_seg // 2, n_seg, functools.partial(chain_body, True), 0, unroll=UNROLL)

    SB = MB // seg
    n_blk = n_seg // SB

    def resid(sg, n, cols=slice(None)):
        sl = pl.ds(sg, n)
        r = xs[sl, :, cols].astype(F32) + mod[2, 0:1, cols] * attn[sl, :, cols].astype(F32)
        return r.reshape(n * seg, r.shape[2])

    def ffn_in(i):
        h = _layernorm(resid(i * SB, SB)) * (1.0 + modrow(4)) + modrow(3)
        r, k = MB // 2, D // 2
        for n, t in enumerate(_strassen_lhs(h[:r, :k], h[:r, k:], h[r:, :k], h[r:, k:])):
            act[n, :, pl.ds(d_ff // 2, k)] = t

    def product(col0, row0, rows, n):
        if n in (1, 4):
            w = wraw[0 if n == 1 else 3, pl.ds(row0, rows), :]
        else:
            w = aux[pl.ds((0, 2, 3, 5, 6).index(n) * WR + row0, rows), :]
        return _dot(act[n, :, pl.ds(col0, 2 * rows)], _w(w))

    ffn_in(0)

    def ffn_body(i, carry):
        for j in range(FH):
            g = _strassen_out(functools.partial(product, d_ff // 2, j * UP, UP))
            u = _strassen_out(functools.partial(product, d_ff // 2, (FH + j) * UP, UP))
            for n, t in enumerate(_strassen_lhs(*(_silu(a) * b for a, b in zip(g, u)))):
                act[n, :, pl.ds(j * LANE, LANE)] = t
        ffn_in(jnp.minimum(i + 1, n_blk - 1))
        for j in range(DH):
            c = _strassen_out(functools.partial(product, 0, 2 * FH * UP + j * DN, DN))
            for n in (1, 2, 3, 0):
                sg = i * SB + (n // 2) * (SB // 2)
                cols = slice((j + (n % 2) * DH) * LANE, (j + (n % 2) * DH + 1) * LANE)
                y = resid(sg, SB // 2, cols) + mod[5, 0:1, cols] * c[n]
                attn[pl.ds(sg, SB // 2), :, cols] = y.reshape(SB // 2, seg, LANE).astype(BF16)
        sl = pl.ds(i * SB, SB)
        pltpu.make_async_copy(attn.at[sl], out_hbm.at[sl], sems.at[S_OUT]).start()
        return carry

    lax.fori_loop(0, n_blk, ffn_body, 0)
    pltpu.make_async_copy(attn, out_hbm, sems.at[S_OUT]).wait()


@functools.partial(jax.jit, static_argnames=("A_seg_len",))
def pallas_adaLN_cond__memory_aug_recurrent_mem_tr__glu_gated_swiglu__prompt_kernel(
    A_x, A_mem0, A_Wq, A_Wk, A_Wv, A_Wo, A_seg_len, B_x, B_w1, B_w3, B_w2, c, w_mod,
):
    del B_x
    B, S, D = A_x.shape
    _, H, Dh = A_Wq.shape
    M = A_mem0.shape[1]
    F = B_w1.shape[1]
    seg = int(A_seg_len)
    n_seg = S // seg
    assert max(F, 2 * D) // LANE <= n_seg // 2 and AHEAD < 8
    assert B == 1 and Dh == LANE and S % seg == 0 and S % MB == 0 and MB % seg == 0
    kern = functools.partial(_kernel, seg=seg, n_seg=n_seg, n_mem=M, n_head=H, d_model=D, d_ff=F)
    hbm = pl.BlockSpec(memory_space=pl.ANY)
    vmem = pl.BlockSpec(memory_space=pltpu.VMEM)
    out = pl.pallas_call(
        kern,
        out_shape=jax.ShapeDtypeStruct((n_seg, seg, D), A_x.dtype),
        in_specs=[vmem, vmem] + [hbm] * 9,
        out_specs=hbm,
        scratch_shapes=[
            pltpu.VMEM((3 * H, D // 2, LANE), U32),
            pltpu.VMEM((D // LANE, H * Dh // 2, LANE), U32),
            pltpu.VMEM((4, 3 * D * F // (8 * LANE), LANE), U32),
            pltpu.VMEM((5 * 3 * D * F // (8 * LANE) + 3 * H * n_seg * PRE, LANE), U32),
            pltpu.VMEM((n_seg, PRE, D), BF16),
            pltpu.VMEM((7, n_seg * PRE // 2, D // 2), BF16),
            pltpu.VMEM((n_seg, seg, D), BF16),
            pltpu.VMEM((n_seg, seg, D), BF16),
            pltpu.VMEM((M + seg - PRE, D), BF16),
            pltpu.VMEM((6, 8, D), F32),
            pltpu.VMEM((7, MB // 2, (F + D) // 2), BF16),
            pltpu.SemaphoreType.DMA((6 + 8,)),
        ],
        compiler_params=pltpu.CompilerParams(vmem_limit_bytes=127 * 1024 * 1024,
                                             disable_bounds_checks=True),
    )(c, A_mem0.reshape(M, D), A_x.reshape(n_seg, seg, D),
      A_Wq.reshape(D // 2, 2 * H, Dh), A_Wk.reshape(D // 2, 2 * H, Dh),
      A_Wv.reshape(D // 2, 2 * H, Dh),
      A_Wo.reshape(H * Dh, D), B_w1, B_w3, B_w2, w_mod)
    return out.reshape(B, S, D)
```

```python
import functools

import jax
import jax.numpy as jnp
from jax import lax
import jax.experimental.pallas as pl
import jax.experimental.pallas.tpu as pltpu

F32 = jnp.float32
BF16 = jnp.bfloat16
U32 = jnp.uint32
LANE = 128
PRE = 8
HG = 4
SPLIT = 8
AHEAD = 3
RING = 4
MB = 128
PAIRS_PER_IT = 2


def _layernorm(x):
    m = jnp.mean(x, axis=-1, keepdims=True)
    d = x - m
    v = jnp.mean(d * d, axis=-1, keepdims=True)
    return d * lax.rsqrt(v + 1e-5)


def _silu(x):
    return x / (1.0 + jnp.exp(-x))


def _w(tile_u32):
    return pltpu.bitcast(tile_u32, BF16)


def _dot(a, b):
    return lax.dot_general(a, b, (((1,), (0,)), ((), ())), preferred_element_type=F32)


def _dot_nt(a, b):
    return lax.dot_general(a, b, (((1,), (1,)), ((), ())), preferred_element_type=F32)


def _add(a, b):
    return jax.tree.map(jnp.add, a, b)


def _sub(a, b):
    return jax.tree.map(jnp.subtract, a, b)


def _strassen_lhs(a11, a12, a21, a22):
    return [_add(a11, a22), _add(a21, a22), a11, a22, _add(a11, a12), _sub(a21, a11),
            _sub(a12, a22)]


def _strassen_rhs(b11, b12, b21, b22):
    return [_add(b11, b22), b11, _sub(b12, b22), _sub(b21, b11), b22, _add(b11, b12),
            _add(b21, b22)]


def _strassen_out(prod):
    m1, m3 = prod(1), prod(3)
    c21 = _add(m1, m3)
    m4 = prod(4)
    c11 = _sub(m3, m4)
    m2 = prod(2)
    c12 = _add(m2, m4)
    c22 = _sub(m2, m1)
    m0 = prod(0)
    c11, c22 = _add(c11, m0), _add(c22, m0)
    c22 = _add(c22, prod(5))
    return [_add(c11, prod(6)), c12, c21, c22]


def _two_level(operands, block):
    halves = [[block(2 * r1 + r2, 2 * c1 + c2) for r2 in range(2) for c2 in range(2)]
              for r1 in range(2) for c1 in range(2)]
    return [t for outer in operands(*halves) for t in operands(*outer)]


def _two_level_out(prod):
    c = _strassen_out(lambda n: _strassen_out(lambda m: prod(7 * n + m)))
    return {(2 * (o // 2) + i // 2, 2 * (o % 2) + i % 2): c[o][i]
            for o in (2, 1, 3, 0) for i in (2, 1, 3, 0)}


def _kernel(c_ref, mem_ref, x_hbm, wq_hbm, wk_hbm, wv_hbm, wo_hbm, w1_hbm, w3_hbm, w2_hbm,
            wmod_hbm, out_hbm,
            wqkv, wo, ring, aux, xp, hp, xs, attn, lhs, mod, act,
            sems, *, seg, n_seg, n_mem, n_head, d_model, d_ff):
    D, H, M = d_model, n_head, n_mem
    DT = D // LANE
    FT = d_ff // LANE
    L = M + seg
    CUR = seg - PRE
    PP = PAIRS_PER_IT
    n_it = 3 * H // (2 * PP)
    it_per_mat = n_it // 3
    (S_XP, S_X, S_WO, S_FF, S_OUT, S_MOD, S_ST) = range(7)

    NP = n_seg * PRE
    TR = LANE // 2
    GM = (DT // 4) * (FT // 4)
    s0 = n_seg - 3 * GM
    PR = 3 * H * PRE
    item = 16 * TR + PR

    def raw_base(g):
        return aux.shape[0] - item * (3 * GM - g)

    def pre_base(s, late):
        return raw_base(s - s0) + 16 * TR if late else s * PR

    def wmod_rows(part, j):
        return aux_rows(s0 * PR + (part * 2 * DT + j) * (D // 2), D // 2)

    def aux_rows(start, size):
        return pl.ds(start if isinstance(start, int) else pl.multiple_of(start, 8), size)

    def pair_copies(w_hbm, i):
        src = w_hbm.bitcast(U32)
        return [pltpu.make_async_copy(
            src.at[:, (i % it_per_mat) * PP + t + par * (H // 2), :],
            ring.at[i % RING, 2 * t + par], sems.at[S_ST + i % RING])
            for t in range(PP) for par in range(2)]

    def lane_tile(j):
        return pl.ds(j * LANE if isinstance(j, int) else pl.multiple_of(j * LANE, LANE), LANE)

    def wmod_copy(part, j):
        return pltpu.make_async_copy(
            wmod_hbm.bitcast(U32).at[:, lane_tile(part * 2 * DT + j)],
            aux.at[wmod_rows(part, j), :], sems.at[S_MOD])

    def wmod_copies(part):
        return [wmod_copy(part, j) for j in range(2 * DT)]

    def wo_copy(j):
        return pltpu.make_async_copy(wo_hbm.bitcast(U32).at[:, lane_tile(j)], wo.at[j],
                                     sems.at[S_WO])

    def x_copy(j):
        sl = pl.ds(j * (n_seg // it_per_mat), n_seg // it_per_mat)
        return pltpu.make_async_copy(x_hbm.at[sl], xs.at[sl], sems.at[S_X])

    def ffn_copy(m, i, nq):
        per_row = DT // 4
        kk, j = (i % per_row, i // per_row) if m < 2 else (i // per_row, i % per_row)
        return pltpu.make_async_copy(
            (w1_hbm, w3_hbm, w2_hbm)[m].bitcast(U32).at[aux_rows(kk * 4 * TR, 4 * TR),
                                                        lane_tile(4 * j + nq)],
            aux.at[aux_rows(raw_base(m * GM + i) + nq * 4 * TR, 4 * TR), :], sems.at[S_FF])

    def prefetch_ffn(s, part):
        if part < 6:
            @pl.when(s < GM)
            def _():
                for nq in range(2):
                    ffn_copy(part // 2, s, 2 * (part % 2) + nq).start()
        elif part == 6:
            @pl.when(s < 2 * DT)
            def _():
                wmod_copy(1, s).start()
                wmod_copy(2, s).start()

    def start(cps):
        for cp in cps:
            cp.start()

    def wait(cps):
        for cp in cps:
            cp.wait()

    xp_copy = pltpu.make_async_copy(x_hbm.at[:, pl.ds(CUR, PRE), :], xp, sems.at[S_XP])

    def modulation(part):
        sc = jnp.broadcast_to(_silu(c_ref[...].astype(F32)), (8, D))
        for j in range(2 * DT):
            r = _dot(sc, _w(aux[wmod_rows(part, j), :]))
            mod[2 * part + j // DT, :, pl.ds((j % DT) * LANE, LANE)] = r

    def modrow(i):
        return mod[i, 0:1, :]

    xp_copy.start()
    start(wmod_copies(0))
    start(pair_copies(wq_hbm, 0))
    xp_copy.wait()
    xn = _layernorm(xp[...].astype(F32).reshape(n_seg * PRE, D))
    wait(wmod_copies(0))
    for i in range(1, AHEAD):
        start(pair_copies(wq_hbm, i))
    modulation(0)
    hn = xn * (1.0 + modrow(1)) + modrow(0)
    r, k = NP // 2, D // 2
    for n, t in enumerate(_strassen_lhs(hn[:r, :k], hn[:r, k:], hn[r:, :k], hn[r:, k:])):
        hp[n] = t.astype(BF16)

    def pro_body(w_next, extra, i, carry):
        wait(pair_copies(wq_hbm, i))
        for t in range(PP):
            a = ring[i % RING, 2 * t]
            b = ring[i % RING, 2 * t + 1]
            heads = ((a & jnp.uint32(0xFFFF)) | (b << 16), (a >> 16) | (b & jnp.uint32(0xFFFF0000)))
            for par in range(2):
                wqkv[(i * PP + t) * 2 + par] = heads[par]
            if t == PP - 1 and w_next is not None:
                start(pair_copies(w_next, i + AHEAD))
                if extra is not None:
                    extra((i + AHEAD) % it_per_mat).start()
            blocks = [_w(heads[par][kh * (D // 4):(kh + 1) * (D // 4)])
                      for kh in range(2) for par in range(2)]
            rhs = _strassen_rhs(*(w.astype(F32) for w in blocks))
            rhs[1], rhs[4] = blocks[0], blocks[3]
            c = _strassen_out(lambda n: _dot(hp[n], rhs[n].astype(BF16)))
            for n in (2, 1, 3, 0):
                for r in range(n_seg // 2):
                    sg = (n // 2) * (n_seg // 2) + r
                    r0 = pre_base(sg, sg >= s0) + ((i * PP + t) * 2 + n % 2) * PRE
                    aux[aux_rows(r0, PRE), :] = pltpu.bitcast(c[n][r * PRE:(r + 1) * PRE], U32)
        return carry

    for m, (w_hbm, extra) in enumerate(((wq_hbm, None), (wk_hbm, wo_copy), (wv_hbm, x_copy))):
        lax.fori_loop(max(m * it_per_mat - AHEAD, 0), (m + 1) * it_per_mat - AHEAD,
                      functools.partial(pro_body, w_hbm, extra), 0)
    lax.fori_loop(n_it - AHEAD, n_it, functools.partial(pro_body, None, None), 0)
    wait([wo_copy(j) for j in range(DT)])
    wait([x_copy(j) for j in range(it_per_mat)])

    def seg_rows(s):
        xn = _layernorm(xs[s].astype(F32)[0:CUR])
        return xn * (1.0 + modrow(1)) + modrow(0)

    lhs[...] = jnp.concatenate([mem_ref[...].astype(F32), seg_rows(0)], axis=0).astype(BF16)
    scale = float(LANE) ** -0.5
    NG = H // HG

    def chain_body(combine, s, carry):
        row = lax.broadcasted_iota(jnp.int32, (L, L), 0)
        col = lax.broadcasted_iota(jnp.int32, (L, L), 1)
        mask = (row < M) | (row >= col)
        q, k, v, p, ov = {}, {}, {}, {}, {}

        def heads(g):
            return range(g * HG, (g + 1) * HG)

        def proj(m, h):
            done = aux[aux_rows(pre_base(s, combine) + (m * H + h) * PRE, PRE), :]
            return jnp.concatenate([_dot(lhs[...], _w(wqkv[m * H + h])),
                                    pltpu.bitcast(done, F32)], axis=0)

        def probs(g):
            for h in heads(g):
                z = jnp.where(mask, _dot_nt(q[h], k[h]) * scale, -1e9)
                e = jnp.exp(z - jnp.max(z, axis=-1, keepdims=True))
                p[h] = e / jnp.sum(e, axis=-1, keepdims=True)

        def values(g):
            for h in heads(g):
                ov[h] = _dot(p[h], v[h])

        def out_proj(h0, h1):
            o = jnp.concatenate([ov[h] for h in range(h0, h1)], axis=1)
            return jnp.concatenate(
                [_dot(o, _w(wo[j, pl.ds(h0 * LANE // 2, (h1 - h0) * LANE // 2), :]))
                 for j in range(DT)], axis=1)

        def combine_weights(part):
            for piece in range(part * (TR // 4) // (2 * NG), (part + 1) * (TR // 4) // (2 * NG)):
                r = piece // 2 * 8

                def block(kq, nq):
                    rows = aux_rows(raw_base(s - s0) + (nq * 4 + kq) * TR + r, 8)
                    return _w(aux[rows, :]).astype(F32)

                for n, t in enumerate(_two_level(_strassen_rhs, block)):
                    if (n // 7 in (0, 1, 2, 5)) == (piece % 2 == 0):
                        rows = aux_rows(((s - s0) * 49 + n) * TR + r, 8)
                        aux[rows, :] = pltpu.bitcast(t.astype(BF16), U32)

        for g in range(NG):
            if combine:
                combine_weights(g)
            for h in heads(g):
                q[h] = proj(0, h)
                k[h] = proj(1, h).astype(BF16)
            if g >= 1:
                probs(g - 1)
            if not combine:
                prefetch_ffn(s, g)
        for g in range(NG):
            if combine:
                combine_weights(NG + g)
            for h in heads(g):
                v[h] = proj(2, h).astype(BF16)
            if g == 0:
                probs(NG - 1)
            else:
                values(g - 1)
        nxt = seg_rows(jnp.minimum(s + 1, n_seg - 1))
        o = out_proj(0, SPLIT)
        values(NG - 1)
        o = o + out_proj(SPLIT, H)
        attn[s] = o[M:].astype(BF16)
        lhs[...] = jnp.concatenate([o[:M], nxt], axis=0).astype(BF16)
        return carry

    lax.fori_loop(0, s0, functools.partial(chain_body, False), 0)
    wait([ffn_copy(m, i, nq) for m in range(3) for i in range(GM) for nq in range(4)])
    wait(wmod_copies(1))
    wait(wmod_copies(2))
    modulation(1)
    modulation(2)
    lax.fori_loop(s0, n_seg, functools.partial(chain_body, True), 0)

    SB = MB // seg
    n_blk = n_seg // SB
    RQ = MB // 4

    def resid(sg, n, cols=slice(None)):
        sl = pl.ds(sg, n)
        r = xs[sl, :, cols].astype(F32) + mod[2, 0:1, cols] * attn[sl, :, cols].astype(F32)
        return r.reshape(n * seg, r.shape[2])

    def ffn_in(i):
        h = _layernorm(resid(i * SB, SB)) * (1.0 + modrow(4)) + modrow(3)

        def block(rq, kq):
            return jnp.concatenate([h[rq * RQ:(rq + 1) * RQ, t * LANE:(t + 1) * LANE]
                                    for t in range(kq, DT, 4)], axis=1)

        for n, t in enumerate(_two_level(_strassen_lhs, block)):
            act[n, :, pl.ds(d_ff // 4, D // 4)] = t

    def product(col0, granules, n):
        w = jnp.concatenate([aux[pl.ds((g * 49 + n) * TR, TR), :] for g in granules], axis=0)
        return _dot(act[n, :, pl.ds(col0, len(granules) * LANE)], _w(w))

    ffn_in(0)

    def ffn_body(i, carry):
        for j in range(FT // 4):
            gate, up = (_two_level_out(functools.partial(
                product, d_ff // 4, range(m * GM + j * (DT // 4), m * GM + (j + 1) * (DT // 4))))
                for m in range(2))
            hidden = {rc: _silu(gate[rc]) * up[rc] for rc in gate}
            for n, t in enumerate(_two_level(_strassen_lhs, lambda r, c: hidden[r, c])):
                act[n, :, pl.ds(j * LANE, LANE)] = t
        ffn_in(jnp.minimum(i + 1, n_blk - 1))
        for j in range(DT // 4):
            c = _two_level_out(functools.partial(product, 0, range(2 * GM + j, 3 * GM, DT // 4)))
            for (rq, nq), t in c.items():
                sg = i * SB + rq * (SB // 4)
                cols = slice((4 * j + nq) * LANE, (4 * j + nq + 1) * LANE)
                y = resid(sg, SB // 4, cols) + mod[5, 0:1, cols] * t
                attn[pl.ds(sg, SB // 4), :, cols] = y.reshape(SB // 4, seg, LANE).astype(BF16)
        sl = pl.ds(i * SB, SB)
        pltpu.make_async_copy(attn.at[sl], out_hbm.at[sl], sems.at[S_OUT]).start()
        return carry

    lax.fori_loop(0, n_blk, ffn_body, 0)
    pltpu.make_async_copy(attn, out_hbm, sems.at[S_OUT]).wait()


@functools.partial(jax.jit, static_argnames=("A_seg_len",))
def pallas_adaLN_cond__memory_aug_recurrent_mem_tr__glu_gated_swiglu__prompt_kernel(
    A_x, A_mem0, A_Wq, A_Wk, A_Wv, A_Wo, A_seg_len, B_x, B_w1, B_w3, B_w2, c, w_mod,
):
    del B_x
    B, S, D = A_x.shape
    _, H, Dh = A_Wq.shape
    M = A_mem0.shape[1]
    F = B_w1.shape[1]
    seg = int(A_seg_len)
    n_seg = S // seg
    n_gran = 3 * (D // (4 * LANE)) * (F // (4 * LANE))
    assert max(n_gran // 3, 2 * D // LANE) <= n_seg - n_gran and AHEAD < RING
    assert B == 1 and Dh == LANE and S % seg == 0 and S % MB == 0 and MB % seg == 0
    kern = functools.partial(_kernel, seg=seg, n_seg=n_seg, n_mem=M, n_head=H, d_model=D, d_ff=F)
    hbm = pl.BlockSpec(memory_space=pl.ANY)
    vmem = pl.BlockSpec(memory_space=pltpu.VMEM)
    out = pl.pallas_call(
        kern,
        out_shape=jax.ShapeDtypeStruct((n_seg, seg, D), A_x.dtype),
        in_specs=[vmem, vmem] + [hbm] * 9,
        out_specs=hbm,
        scratch_shapes=[
            pltpu.VMEM((3 * H, D // 2, LANE), U32),
            pltpu.VMEM((D // LANE, H * Dh // 2, LANE), U32),
            pltpu.VMEM((RING, 2 * PAIRS_PER_IT, D // 2, LANE), U32),
            pltpu.VMEM(((49 * n_gran + 16) * LANE // 2 + 3 * H * PRE, LANE), U32),
            pltpu.VMEM((n_seg, PRE, D), BF16),
            pltpu.VMEM((7, n_seg * PRE // 2, D // 2), BF16),
            pltpu.VMEM((n_seg, seg, D), BF16),
            pltpu.VMEM((n_seg, seg, D), BF16),
            pltpu.VMEM((M + seg - PRE, D), BF16),
            pltpu.VMEM((6, 8, D), F32),
            pltpu.VMEM((49, MB // 4, (F + D) // 4), F32),
            pltpu.SemaphoreType.DMA((6 + RING,)),
        ],
        compiler_params=pltpu.CompilerParams(vmem_limit_bytes=127 * 1024 * 1024,
                                             disable_bounds_checks=True),
    )(c, A_mem0.reshape(M, D), A_x.reshape(n_seg, seg, D),
      A_Wq.reshape(D // 2, 2 * H, Dh), A_Wk.reshape(D // 2, 2 * H, Dh),
      A_Wv.reshape(D // 2, 2 * H, Dh),
      A_Wo.reshape(H * Dh, D), B_w1, B_w3, B_w2, w_mod)
    return out.reshape(B, S, D)
```

```python
import functools

import jax
import jax.numpy as jnp
from jax import lax
import jax.experimental.pallas as pl
import jax.experimental.pallas.tpu as pltpu

F32 = jnp.float32
BF16 = jnp.bfloat16
U32 = jnp.uint32
LANE = 128
EPS = 1e-5
PRE = 8
HG = 4
SPLIT = 8
AHEAD = 3
RING = 4
CW = ((0, 2, 5), (3, 6), (1, 4))
FIRST = (10, 49)
LN_ROWS = 16
PAIRS_PER_IT = 2


def _layernorm(x):
    m = jnp.mean(x, axis=-1, keepdims=True)
    d = x - m
    v = jnp.mean(d * d, axis=-1, keepdims=True)
    return d * lax.rsqrt(v + EPS)


def _silu(x):
    return x / (1.0 + jnp.exp(-x))


def _w(tile_u32):
    return pltpu.bitcast(tile_u32, BF16)


def _dot(a, b):
    return lax.dot_general(a, b, (((1,), (0,)), ((), ())), preferred_element_type=F32)


def _dot_nt(a, b):
    return lax.dot_general(a, b, (((1,), (1,)), ((), ())), preferred_element_type=F32)


def _add(a, b):
    return jax.tree.map(jnp.add, a, b)


def _sub(a, b):
    return jax.tree.map(jnp.subtract, a, b)


def _strassen_lhs(a11, a12, a21, a22):
    return [_add(a11, a22), _add(a21, a22), a11, a22, _add(a11, a12), _sub(a21, a11),
            _sub(a12, a22)]


def _strassen_rhs(b11, b12, b21, b22):
    return [_add(b11, b22), b11, _sub(b12, b22), _sub(b21, b11), b22, _add(b11, b12),
            _add(b21, b22)]


def _strassen_out(prod):
    m1, m3 = prod(1), prod(3)
    c21 = _add(m1, m3)
    m4 = prod(4)
    c11 = _sub(m3, m4)
    m2 = prod(2)
    c12 = _add(m2, m4)
    c22 = _sub(m2, m1)
    m0 = prod(0)
    c11, c22 = _add(c11, m0), _add(c22, m0)
    c22 = _add(c22, prod(5))
    return [_add(c11, prod(6)), c12, c21, c22]


def _two_level(operands, block):
    halves = [[block(2 * r1 + r2, 2 * c1 + c2) for r2 in range(2) for c2 in range(2)]
              for r1 in range(2) for c1 in range(2)]
    return [t for outer in operands(*halves) for t in operands(*outer)]


def _two_level_out(prod):
    c = _strassen_out(lambda n: _strassen_out(lambda m: prod(7 * n + m)))
    return {(2 * (o // 2) + i // 2, 2 * (o % 2) + i % 2): c[o][i]
            for o in (2, 1, 3, 0) for i in (2, 1, 3, 0)}


def _kernel(c_ref, mem_ref, x_hbm, wq_hbm, wk_hbm, wv_hbm, wo_hbm, w1_hbm, w3_hbm, w2_hbm,
            wmod_hbm, out_hbm,
            wqkv, wo, aux, xs, attn, lhs, mod,
            sems, *, seg, n_seg, n_mem, n_head, d_model, d_ff):
    D, H, M = d_model, n_head, n_mem
    DT = D // LANE
    FT = d_ff // LANE
    L = M + seg
    CUR = seg - PRE
    PP = PAIRS_PER_IT
    n_it = 3 * H // (2 * PP)
    it_per_mat = n_it // 3
    (S_XP, S_X, S_WO, S_FF, S_OUT, S_MOD, S_ST) = range(7)

    NP = n_seg * PRE
    TR = LANE // 2
    GM = (DT // 4) * (FT // 4)
    s0 = n_seg - 3 * GM
    PR = 3 * H * PRE
    item = 16 * TR + PR

    def raw_base(g):
        return aux.shape[0] - item * (3 * GM - g)

    def pre_base(s, late):
        return raw_base(s - s0) + 16 * TR if late else s * PR

    def wmod_rows(part, j):
        return aux_rows(s0 * PR + (part * 2 * DT + j) * (D // 2), D // 2)

    def aux_rows(start, size):
        return pl.ds(start if isinstance(start, int) else pl.multiple_of(start, 8), size)

    def lane_tile(j):
        return pl.ds(j * LANE if isinstance(j, int) else pl.multiple_of(j * LANE, LANE), LANE)

    def wmod_copy(part, j):
        return pltpu.make_async_copy(
            wmod_hbm.bitcast(U32).at[:, lane_tile(part * 2 * DT + j)],
            aux.at[wmod_rows(part, j), :], sems.at[S_MOD])

    def wmod_copies(part):
        return [wmod_copy(part, j) for j in range(2 * DT)]

    def wo_copy(j):
        return pltpu.make_async_copy(wo_hbm.bitcast(U32).at[:, lane_tile(j)], wo.at[j],
                                     sems.at[S_WO])

    def x_copy(j):
        sl = pl.ds(j * (n_seg // it_per_mat), n_seg // it_per_mat)
        return pltpu.make_async_copy(x_hbm.at[sl], xs.at[sl], sems.at[S_X])

    def ffn_copy(m, i, nq):
        per_row = DT // 4
        kk, j = (i % per_row, i // per_row) if m < 2 else (i // per_row, i % per_row)
        return pltpu.make_async_copy(
            (w1_hbm, w3_hbm, w2_hbm)[m].bitcast(U32).at[aux_rows(kk * 4 * TR, 4 * TR),
                                                        lane_tile(4 * j + nq)],
            aux.at[aux_rows(raw_base(m * GM + i) + nq * 4 * TR, 4 * TR), :], sems.at[S_FF])

    def prefetch_ffn(s, part):
        if part < 6:
            @pl.when(s < GM)
            def _():
                for nq in range(2):
                    ffn_copy(part // 2, s, 2 * (part % 2) + nq).start()
        elif part == 6:
            @pl.when(s < 2 * DT)
            def _():
                wmod_copy(1, s).start()
                wmod_copy(2, s).start()

    def start(cps):
        for cp in cps:
            cp.start()

    def wait(cps):
        for cp in cps:
            cp.wait()

    def modulation(part):
        sc = jnp.broadcast_to(_silu(c_ref[...].astype(F32)), (8, D))
        for j in range(2 * DT):
            r = _dot(sc, _w(aux[wmod_rows(part, j), :]))
            mod[2 * part + j // DT, :, pl.ds((j % DT) * LANE, LANE)] = r

    def modrow(i):
        return mod[i, 0:1, :]

    def prologue(ring, xp, hp):
        def pair_copies(w_hbm, i):
            src = w_hbm.bitcast(U32)
            return [pltpu.make_async_copy(
                src.at[:, (i % it_per_mat) * PP + t + par * (H // 2), :],
                ring.at[i % RING, 2 * t + par], sems.at[S_ST + i % RING])
                for t in range(PP) for par in range(2)]

        xp_copy = pltpu.make_async_copy(x_hbm.at[:, pl.ds(CUR, PRE), :], xp, sems.at[S_XP])
        xp_copy.start()
        start(wmod_copies(0))
        start(pair_copies(wq_hbm, 0))
        xp_copy.wait()
        xn = _layernorm(xp[...].astype(F32).reshape(n_seg * PRE, D))
        wait(wmod_copies(0))
        for i in range(1, AHEAD):
            start(pair_copies(wq_hbm, i))
        modulation(0)
        hn = xn * (1.0 + modrow(1)) + modrow(0)
        r, k = NP // 2, D // 2
        for n, t in enumerate(_strassen_lhs(hn[:r, :k], hn[:r, k:], hn[r:, :k], hn[r:, k:])):
            hp[n] = t.astype(BF16)

        def pro_body(w_next, extra, i, carry):
            wait(pair_copies(wq_hbm, i))
            for t in range(PP):
                a = ring[i % RING, 2 * t]
                b = ring[i % RING, 2 * t + 1]
                heads = ((a & jnp.uint32(0xFFFF)) | (b << 16), (a >> 16) | (b & jnp.uint32(0xFFFF0000)))
                for par in range(2):
                    wqkv[(i * PP + t) * 2 + par] = heads[par]
                if t == PP - 1 and w_next is not None:
                    start(pair_copies(w_next, i + AHEAD))
                    if extra is not None:
                        extra((i + AHEAD) % it_per_mat).start()
                blocks = [_w(heads[par][kh * (D // 4):(kh + 1) * (D // 4)])
                          for kh in range(2) for par in range(2)]
                rhs = _strassen_rhs(*(w.astype(F32) for w in blocks))
                rhs[1], rhs[4] = blocks[0], blocks[3]
                c = _strassen_out(lambda n: _dot(hp[n], rhs[n].astype(BF16)))
                for n in (2, 1, 3, 0):
                    for r in range(n_seg // 2):
                        sg = (n // 2) * (n_seg // 2) + r
                        r0 = pre_base(sg, sg >= s0) + ((i * PP + t) * 2 + n % 2) * PRE
                        aux[aux_rows(r0, PRE), :] = pltpu.bitcast(c[n][r * PRE:(r + 1) * PRE], U32)
            return carry

        for m, (w_hbm, extra) in enumerate(((wq_hbm, None), (wk_hbm, wo_copy), (wv_hbm, x_copy))):
            lax.fori_loop(max(m * it_per_mat - AHEAD, 0), (m + 1) * it_per_mat - AHEAD,
                          functools.partial(pro_body, w_hbm, extra), 0)
        lax.fori_loop(n_it - AHEAD, n_it, functools.partial(pro_body, None, None), 0)

    pl.run_scoped(prologue, pltpu.VMEM((RING, 2 * PP, D // 2, LANE), U32),
                  pltpu.VMEM((n_seg, PRE, D), BF16), pltpu.VMEM((7, NP // 2, D // 2), BF16))
    wait([wo_copy(j) for j in range(DT)])
    wait([x_copy(j) for j in range(it_per_mat)])

    def seg_rows(s):
        xn = _layernorm(xs[s].astype(F32)[0:CUR])
        return xn * (1.0 + modrow(1)) + modrow(0)

    lhs[...] = jnp.concatenate([mem_ref[...].astype(F32), seg_rows(0)], axis=0).astype(BF16)
    scale = float(LANE) ** -0.5
    NG = H // HG

    def chain_body(combine, s, carry):
        row = lax.broadcasted_iota(jnp.int32, (L, L), 0)
        col = lax.broadcasted_iota(jnp.int32, (L, L), 1)
        mask = (row < M) | (row >= col)
        q, k, v, p, ov = {}, {}, {}, {}, {}

        def heads(g):
            return range(g * HG, (g + 1) * HG)

        def proj(m, h):
            done = aux[aux_rows(pre_base(s, combine) + (m * H + h) * PRE, PRE), :]
            return jnp.concatenate([_dot(lhs[...], _w(wqkv[m * H + h])),
                                    pltpu.bitcast(done, F32)], axis=0)

        def probs(g):
            for h in heads(g):
                z = jnp.where(mask, _dot_nt(q[h], k[h]) * scale, -1e9)
                e = jnp.exp(z - jnp.max(z, axis=-1, keepdims=True))
                p[h] = e / jnp.sum(e, axis=-1, keepdims=True)

        def values(g):
            for h in heads(g):
                ov[h] = _dot(p[h], v[h])

        def out_proj(h0, h1):
            o = jnp.concatenate([ov[h] for h in range(h0, h1)], axis=1)
            return jnp.concatenate(
                [_dot(o, _w(wo[j, pl.ds(h0 * LANE // 2, (h1 - h0) * LANE // 2), :]))
                 for j in range(DT)], axis=1)

        def combine_weights(g, outer):
            for r in range(g * TR // NG // 8 * 8, (g + 1) * TR // NG // 8 * 8, 8) if combine else ():
                def block(kq, nq):
                    rows = aux_rows(raw_base(s - s0) + (nq * 4 + kq) * TR + r, 8)
                    return _w(aux[rows, :]).astype(F32)

                for n, t in enumerate(_two_level(_strassen_rhs, block)):
                    if n // 7 in outer:
                        rows = aux_rows(((s - s0) * 49 + n) * TR + r, 8)
                        aux[rows, :] = pltpu.bitcast(t.astype(BF16), U32)

        for g in range(NG):
            combine_weights(g, CW[0])
            for h in heads(g):
                k[h] = proj(1, h).astype(BF16)
            combine_weights(g, CW[1])
            for h in heads(g):
                q[h] = proj(0, h)
            if g >= 1:
                probs(g - 1)
            if not combine:
                prefetch_ffn(s, g)
        for g in range(NG):
            combine_weights(g, CW[2])
            for h in heads(g):
                v[h] = proj(2, h).astype(BF16)
            if g == 0:
                probs(NG - 1)
            else:
                values(g - 1)
        nxt = seg_rows(jnp.minimum(s + 1, n_seg - 1))
        o = out_proj(0, SPLIT)
        values(NG - 1)
        o = o + out_proj(SPLIT, H)
        attn[s] = o[M:].astype(BF16)
        lhs[...] = jnp.concatenate([o[:M], nxt], axis=0).astype(BF16)
        return carry

    lax.fori_loop(0, s0, functools.partial(chain_body, False), 0)
    wait([ffn_copy(m, i, nq) for m in range(3) for i in range(GM) for nq in range(4)])
    wait(wmod_copies(1))
    wait(wmod_copies(2))
    modulation(1)
    modulation(2)
    lax.fori_loop(s0, n_seg, functools.partial(chain_body, True), 0)

    SB = 4
    n_blk = n_seg // SB

    def resid(sg, rows=slice(None), cols=slice(None)):
        return (xs[sg, rows, cols].astype(F32)
                + mod[2, 0:1, cols] * attn[sg, rows, cols].astype(F32))

    def ffn(act, upin, hbuf):
        KT = DT // 4

        def norm_steps(i, zero):
            def center(sg, rows):
                x1 = resid(i * SB + sg, rows=rows)
                hbuf[sg + zero, rows] = x1 - jnp.mean(x1, axis=-1, keepdims=True)

            def normalize(sg, rows):
                d = hbuf[sg, rows]
                rstd = lax.rsqrt(jnp.mean(d * d, axis=-1, keepdims=True) + EPS)
                hbuf[sg + zero, rows] = d * rstd * (1.0 + modrow(4)) + modrow(3)

            return [functools.partial(f, sg, slice(r, r + LN_ROWS)) for f in (center, normalize)
                    for sg in range(SB) for r in range(0, seg, LN_ROWS)]

        def operand_steps(zero):
            def operands(outer, t):
                ops = _two_level(_strassen_lhs,
                                 lambda rq, kq: hbuf[rq, :, lane_tile(4 * t + kq)])
                for n in range(7 * outer, 7 * outer + 7):
                    upin[n + zero, :, pl.ds(t * LANE, LANE)] = ops[n]

            return [functools.partial(operands, n, t) for n in range(7) for t in range(KT)]

        def products(a_ref, n_calls, first, steps, zero):
            calls = iter(range(n_calls))
            when = {first + k * (n_calls - first) // len(steps): f for k, f in enumerate(steps)}
            assert len(when) == len(steps)

            def product(granules, n):
                w = jnp.concatenate([aux[pl.ds((g * 49 + n) * TR, TR), :] for g in granules],
                                    axis=0)
                r = _dot(a_ref[n], _w(w))
                step = when.get(next(calls))
                if step is not None:
                    hbuf[SB + zero, 0:8, 0:LANE] = r[0:8]
                    step()
                return r

            return product

        for step in norm_steps(0, 0) + operand_steps(0):
            step()

        def ffn_body(i, carry):
            zero = i // n_blk
            product = products(upin, 2 * 49 * (FT // 4), FIRST[0],
                               norm_steps(jnp.minimum(i + 1, n_blk - 1), zero), zero)
            for j in range(FT // 4):
                gate, up = (_two_level_out(functools.partial(
                    product, range(m * GM + j * KT, m * GM + (j + 1) * KT))) for m in range(2))
                hidden = {rc: _silu(gate[rc]) * up[rc] for rc in gate}
                for n, t in enumerate(_two_level(_strassen_lhs, lambda r, c: hidden[r, c])):
                    act[n, :, lane_tile(j)] = t
            product = products(act, 49 * KT, FIRST[1], operand_steps(zero), zero)
            for j in range(KT):
                c = _two_level_out(functools.partial(product, range(2 * GM + j, 3 * GM, KT)))
                for (rq, nq), t in c.items():
                    cols = slice((4 * j + nq) * LANE, (4 * j + nq + 1) * LANE)
                    y = resid(i * SB + rq, cols=cols) + mod[5, 0:1, cols] * t
                    attn[i * SB + rq, :, cols] = y.astype(BF16)
            sl = pl.ds(i * SB, SB)
            pltpu.make_async_copy(attn.at[sl], out_hbm.at[sl], sems.at[S_OUT]).start()
            return carry

        lax.fori_loop(0, n_blk, ffn_body, 0)

    pl.run_scoped(ffn, pltpu.VMEM((49, seg, d_ff // 4), F32),
                  pltpu.VMEM((49, seg, D // 4), F32), pltpu.VMEM((SB + 1, seg, D), F32))
    pltpu.make_async_copy(attn, out_hbm, sems.at[S_OUT]).wait()


@functools.partial(jax.jit, static_argnames=("A_seg_len",))
def pallas_adaLN_cond__memory_aug_recurrent_mem_tr__glu_gated_swiglu__prompt_kernel(
    A_x, A_mem0, A_Wq, A_Wk, A_Wv, A_Wo, A_seg_len, B_x, B_w1, B_w3, B_w2, c, w_mod,
):
    del B_x
    B, S, D = A_x.shape
    _, H, Dh = A_Wq.shape
    M = A_mem0.shape[1]
    F = B_w1.shape[1]
    seg = int(A_seg_len)
    n_seg = S // seg
    n_gran = 3 * (D // (4 * LANE)) * (F // (4 * LANE))
    assert max(n_gran // 3, 2 * D // LANE) <= n_seg - n_gran and AHEAD < RING
    assert B == 1 and Dh == LANE and S % seg == 0 and n_seg % 4 == 0
    kern = functools.partial(_kernel, seg=seg, n_seg=n_seg, n_mem=M, n_head=H, d_model=D, d_ff=F)
    hbm = pl.BlockSpec(memory_space=pl.ANY)
    vmem = pl.BlockSpec(memory_space=pltpu.VMEM)
    out = pl.pallas_call(
        kern,
        out_shape=jax.ShapeDtypeStruct((n_seg, seg, D), A_x.dtype),
        in_specs=[vmem, vmem] + [hbm] * 9,
        out_specs=hbm,
        scratch_shapes=[
            pltpu.VMEM((3 * H, D // 2, LANE), U32),
            pltpu.VMEM((D // LANE, H * Dh // 2, LANE), U32),
            pltpu.VMEM(((49 * n_gran + 16) * LANE // 2 + 3 * H * PRE, LANE), U32),
            pltpu.VMEM((n_seg, seg, D), BF16),
            pltpu.VMEM((n_seg, seg, D), BF16),
            pltpu.VMEM((M + seg - PRE, D), BF16),
            pltpu.VMEM((6, 8, D), F32),
            pltpu.SemaphoreType.DMA((6 + RING,)),
        ],
        compiler_params=pltpu.CompilerParams(vmem_limit_bytes=127 * 1024 * 1024,
                                             disable_bounds_checks=True),
    )(c, A_mem0.reshape(M, D), A_x.reshape(n_seg, seg, D),
      A_Wq.reshape(D // 2, 2 * H, Dh), A_Wk.reshape(D // 2, 2 * H, Dh),
      A_Wv.reshape(D // 2, 2 * H, Dh),
      A_Wo.reshape(H * Dh, D), B_w1, B_w3, B_w2, w_mod)
    return out.reshape(B, S, D)
```

```python
import functools

import jax
import jax.numpy as jnp
from jax import lax
import jax.experimental.pallas as pl
import jax.experimental.pallas.tpu as pltpu

F32 = jnp.float32
BF16 = jnp.bfloat16
U32 = jnp.uint32
LANE = 128
EPS = 1e-5
PRE = 8
HG = 4
SPLIT = 8
AHEAD = 3
RING = 4
CW = ((2, 5), (3, 6), (1,), (0, 4))
FIRST = (10, 49)
LN_ROWS = 16
PAIRS_PER_IT = 2


def _layernorm(x):
    m = jnp.mean(x, axis=-1, keepdims=True)
    d = x - m
    v = jnp.mean(d * d, axis=-1, keepdims=True)
    return d * lax.rsqrt(v + EPS)


def _silu(x):
    return x / (1.0 + jnp.exp(-x))


def _w(tile_u32):
    return pltpu.bitcast(tile_u32, BF16)


def _dot(a, b):
    return lax.dot_general(a, b, (((1,), (0,)), ((), ())), preferred_element_type=F32)


def _dot_nt(a, b):
    return lax.dot_general(a, b, (((1,), (1,)), ((), ())), preferred_element_type=F32)


def _add(a, b):
    return jax.tree.map(jnp.add, a, b)


def _sub(a, b):
    return jax.tree.map(jnp.subtract, a, b)


def _strassen_lhs(a11, a12, a21, a22):
    return [_add(a11, a22), _add(a21, a22), a11, a22, _add(a11, a12), _sub(a21, a11),
            _sub(a12, a22)]


def _strassen_rhs(b11, b12, b21, b22):
    return [_add(b11, b22), b11, _sub(b12, b22), _sub(b21, b11), b22, _add(b11, b12),
            _add(b21, b22)]


def _strassen_out(prod):
    m1, m3 = prod(1), prod(3)
    c21 = _add(m1, m3)
    m4 = prod(4)
    c11 = _sub(m3, m4)
    m2 = prod(2)
    c12 = _add(m2, m4)
    c22 = _sub(m2, m1)
    m0 = prod(0)
    c11, c22 = _add(c11, m0), _add(c22, m0)
    c22 = _add(c22, prod(5))
    return [_add(c11, prod(6)), c12, c21, c22]


def _two_level(operands, block):
    halves = [[block(2 * r1 + r2, 2 * c1 + c2) for r2 in range(2) for c2 in range(2)]
              for r1 in range(2) for c1 in range(2)]
    return [t for outer in operands(*halves) for t in operands(*outer)]


def _two_level_out(prod):
    c = _strassen_out(lambda n: _strassen_out(lambda m: prod(7 * n + m)))
    return {(2 * (o // 2) + i // 2, 2 * (o % 2) + i % 2): c[o][i]
            for o in (2, 1, 3, 0) for i in (2, 1, 3, 0)}


def _kernel(c_ref, mem_ref, x_hbm, wq_hbm, wk_hbm, wv_hbm, wo_hbm, w1_hbm, w3_hbm, w2_hbm,
            wmod_hbm, out_hbm,
            wqkv, wo, aux, xs, attn, lhs, mod,
            sems, *, seg, n_seg, n_mem, n_head, d_model, d_ff):
    D, H, M = d_model, n_head, n_mem
    DT = D // LANE
    FT = d_ff // LANE
    L = M + seg
    CUR = seg - PRE
    PP = PAIRS_PER_IT
    n_it = 3 * H // (2 * PP)
    it_per_mat = n_it // 3
    (S_XP, S_X, S_WO, S_FF, S_OUT, S_MOD, S_ST) = range(7)

    NP = n_seg * PRE
    TR = LANE // 2
    GM = (DT // 4) * (FT // 4)
    s0 = n_seg - 3 * GM
    PR = 3 * H * PRE
    item = 16 * TR + PR

    def raw_base(g):
        return aux.shape[0] - item * (3 * GM - g)

    def pre_base(s, late):
        return raw_base(s - s0) + 16 * TR if late else s * PR

    def wmod_rows(part, j):
        return aux_rows(s0 * PR + (part * 2 * DT + j) * (D // 2), D // 2)

    def aux_rows(start, size):
        return pl.ds(start if isinstance(start, int) else pl.multiple_of(start, 8), size)

    def lane_tile(j):
        return pl.ds(j * LANE if isinstance(j, int) else pl.multiple_of(j * LANE, LANE), LANE)

    def wmod_copy(part, j):
        return pltpu.make_async_copy(
            wmod_hbm.bitcast(U32).at[:, lane_tile(part * 2 * DT + j)],
            aux.at[wmod_rows(part, j), :], sems.at[S_MOD])

    def wmod_copies(part):
        return [wmod_copy(part, j) for j in range(2 * DT)]

    def wo_copy(j):
        return pltpu.make_async_copy(wo_hbm.bitcast(U32).at[:, lane_tile(j)], wo.at[j],
                                     sems.at[S_WO])

    def x_copy(j):
        sl = pl.ds(j * (n_seg // it_per_mat), n_seg // it_per_mat)
        return pltpu.make_async_copy(x_hbm.at[sl], xs.at[sl], sems.at[S_X])

    def ffn_copy(m, i, nq):
        per_row = DT // 4
        kk, j = (i % per_row, i // per_row) if m < 2 else (i // per_row, i % per_row)
        return pltpu.make_async_copy(
            (w1_hbm, w3_hbm, w2_hbm)[m].bitcast(U32).at[aux_rows(kk * 4 * TR, 4 * TR),
                                                        lane_tile(4 * j + nq)],
            aux.at[aux_rows(raw_base(m * GM + i) + nq * 4 * TR, 4 * TR), :], sems.at[S_FF])

    def prefetch_ffn(s, part):
        if part < 6:
            @pl.when(s < GM)
            def _():
                for nq in range(2):
                    ffn_copy(part // 2, s, 2 * (part % 2) + nq).start()
        elif part == 6:
            @pl.when(s < 2 * DT)
            def _():
                wmod_copy(1, s).start()
                wmod_copy(2, s).start()

    def start(cps):
        for cp in cps:
            cp.start()

    def wait(cps):
        for cp in cps:
            cp.wait()

    def modulation(part):
        sc = jnp.broadcast_to(_silu(c_ref[...].astype(F32)), (8, D))
        for j in range(2 * DT):
            r = _dot(sc, _w(aux[wmod_rows(part, j), :]))
            mod[2 * part + j // DT, :, pl.ds((j % DT) * LANE, LANE)] = r

    def modrow(i):
        return mod[i, 0:1, :]

    def prologue(ring, xp, hp):
        def pair_copies(w_hbm, i):
            src = w_hbm.bitcast(U32)
            return [pltpu.make_async_copy(
                src.at[:, (i % it_per_mat) * PP + t + par * (H // 2), :],
                ring.at[i % RING, 2 * t + par], sems.at[S_ST + i % RING])
                for t in range(PP) for par in range(2)]

        xp_copy = pltpu.make_async_copy(x_hbm.at[:, pl.ds(CUR, PRE), :], xp, sems.at[S_XP])
        xp_copy.start()
        start(wmod_copies(0))
        start(pair_copies(wq_hbm, 0))
        xp_copy.wait()
        xn = _layernorm(xp[...].astype(F32).reshape(n_seg * PRE, D))
        wait(wmod_copies(0))
        for i in range(1, AHEAD):
            start(pair_copies(wq_hbm, i))
        modulation(0)
        hn = xn * (1.0 + modrow(1)) + modrow(0)
        r, k = NP // 2, D // 2
        for n, t in enumerate(_strassen_lhs(hn[:r, :k], hn[:r, k:], hn[r:, :k], hn[r:, k:])):
            hp[n] = t.astype(BF16)

        def pro_body(w_next, extra, i, carry):
            wait(pair_copies(wq_hbm, i))
            for t in range(PP):
                a = ring[i % RING, 2 * t]
                b = ring[i % RING, 2 * t + 1]
                heads = ((a & jnp.uint32(0xFFFF)) | (b << 16), (a >> 16) | (b & jnp.uint32(0xFFFF0000)))
                for par in range(2):
                    wqkv[(i * PP + t) * 2 + par] = heads[par]
                if t == PP - 1 and w_next is not None:
                    start(pair_copies(w_next, i + AHEAD))
                    if extra is not None:
                        extra((i + AHEAD) % it_per_mat).start()
                blocks = [_w(heads[par][kh * (D // 4):(kh + 1) * (D // 4)])
                          for kh in range(2) for par in range(2)]
                rhs = _strassen_rhs(*(w.astype(F32) for w in blocks))
                rhs[1], rhs[4] = blocks[0], blocks[3]
                c = _strassen_out(lambda n: _dot(hp[n], rhs[n].astype(BF16)))
                for n in (2, 1, 3, 0):
                    for r in range(n_seg // 2):
                        sg = (n // 2) * (n_seg // 2) + r
                        r0 = pre_base(sg, sg >= s0) + ((i * PP + t) * 2 + n % 2) * PRE
                        aux[aux_rows(r0, PRE), :] = pltpu.bitcast(c[n][r * PRE:(r + 1) * PRE], U32)
            return carry

        for m, (w_hbm, extra) in enumerate(((wq_hbm, None), (wk_hbm, wo_copy), (wv_hbm, x_copy))):
            lax.fori_loop(max(m * it_per_mat - AHEAD, 0), (m + 1) * it_per_mat - AHEAD,
                          functools.partial(pro_body, w_hbm, extra), 0)
        lax.fori_loop(n_it - AHEAD, n_it, functools.partial(pro_body, None, None), 0)

    pl.run_scoped(prologue, pltpu.VMEM((RING, 2 * PP, D // 2, LANE), U32),
                  pltpu.VMEM((n_seg, PRE, D), BF16), pltpu.VMEM((7, NP // 2, D // 2), BF16))
    wait([wo_copy(j) for j in range(DT)])
    wait([x_copy(j) for j in range(it_per_mat)])

    def seg_rows(s):
        xn = _layernorm(xs[s].astype(F32)[0:CUR])
        return xn * (1.0 + modrow(1)) + modrow(0)

    lhs[...] = jnp.concatenate([mem_ref[...].astype(F32), seg_rows(0)], axis=0).astype(BF16)
    scale = float(LANE) ** -0.5
    NG = H // HG

    def chain_body(combine, s, carry):
        row = lax.broadcasted_iota(jnp.int32, (L, L), 0)
        col = lax.broadcasted_iota(jnp.int32, (L, L), 1)
        mask = (row < M) | (row >= col)
        q, k, v, p, ov = {}, {}, {}, {}, {}

        def heads(g):
            return range(g * HG, (g + 1) * HG)

        def proj(m, h):
            done = aux[aux_rows(pre_base(s, combine) + (m * H + h) * PRE, PRE), :]
            return jnp.concatenate([_dot(lhs[...], _w(wqkv[m * H + h])),
                                    pltpu.bitcast(done, F32)], axis=0)

        def probs(g):
            for h in heads(g):
                z = jnp.where(mask, _dot_nt(q[h], k[h]) * scale, -1e9)
                e = jnp.exp(z - jnp.max(z, axis=-1, keepdims=True))
                p[h] = e / jnp.sum(e, axis=-1, keepdims=True)

        def values(g):
            for h in heads(g):
                ov[h] = _dot(p[h], v[h])

        def out_proj(h0, h1, marks):
            o = jnp.concatenate([ov[h] for h in range(h0, h1)], axis=1)
            cols = []
            for j in range(DT):
                cols.append(_dot(o, _w(wo[j, pl.ds(h0 * TR, (h1 - h0) * TR), :])))
                if combine and j in marks:
                    aux[aux_rows(pre_base(s, True), 8), :] = pltpu.bitcast(cols[-1][0:8], U32)
                    combine_weights(marks[j], CW[3])
            return jnp.concatenate(cols, axis=1)

        def combine_weights(g, outer):
            for r in range(g * TR // NG // 8 * 8, (g + 1) * TR // NG // 8 * 8, 8) if combine else ():
                def block(kq, nq):
                    rows = aux_rows(raw_base(s - s0) + (nq * 4 + kq) * TR + r, 8)
                    return _w(aux[rows, :]).astype(F32)

                for n, t in enumerate(_two_level(_strassen_rhs, block)):
                    if n // 7 in outer:
                        rows = aux_rows(((s - s0) * 49 + n) * TR + r, 8)
                        aux[rows, :] = pltpu.bitcast(t.astype(BF16), U32)

        for g in range(NG):
            combine_weights(g, CW[0])
            for h in heads(g):
                k[h] = proj(1, h).astype(BF16)
            combine_weights(g, CW[1])
            for h in heads(g):
                q[h] = proj(0, h)
            if g >= 1:
                probs(g - 1)
            if not combine:
                prefetch_ffn(s, g)
        for g in range(NG):
            combine_weights(g, CW[2])
            for h in heads(g):
                v[h] = proj(2, h).astype(BF16)
            if g == 0:
                probs(NG - 1)
            else:
                values(g - 1)
        nxt = seg_rows(jnp.minimum(s + 1, n_seg - 1))
        o = out_proj(0, SPLIT, {DT // 2 - 1: 0, DT - 1: 1})
        values(NG - 1)
        o = o + out_proj(SPLIT, H, {j: j + 2 for j in range(NG - 2)})
        attn[s] = o[M:].astype(BF16)
        lhs[...] = jnp.concatenate([o[:M], nxt], axis=0).astype(BF16)
        return carry

    lax.fori_loop(0, s0, functools.partial(chain_body, False), 0)
    wait([ffn_copy(m, i, nq) for m in range(3) for i in range(GM) for nq in range(4)])
    wait(wmod_copies(1))
    wait(wmod_copies(2))
    modulation(1)
    modulation(2)
    lax.fori_loop(s0, n_seg, functools.partial(chain_body, True), 0)

    SB = 4
    n_blk = n_seg // SB

    def resid(sg, rows=slice(None), cols=slice(None)):
        return (xs[sg, rows, cols].astype(F32)
                + mod[2, 0:1, cols] * attn[sg, rows, cols].astype(F32))

    def ffn(act, upin, hbuf):
        KT = DT // 4

        def norm_steps(i, zero):
            def center(sg, rows):
                x1 = resid(i * SB + sg, rows=rows)
                hbuf[sg + zero, rows] = x1 - jnp.mean(x1, axis=-1, keepdims=True)

            def normalize(sg, rows):
                d = hbuf[sg, rows]
                rstd = lax.rsqrt(jnp.mean(d * d, axis=-1, keepdims=True) + EPS)
                hbuf[sg + zero, rows] = d * rstd * (1.0 + modrow(4)) + modrow(3)

            return [functools.partial(f, sg, slice(r, r + LN_ROWS)) for f in (center, normalize)
                    for sg in range(SB) for r in range(0, seg, LN_ROWS)]

        def operand_steps(zero):
            def operands(outer, t):
                ops = _two_level(_strassen_lhs,
                                 lambda rq, kq: hbuf[rq, :, lane_tile(4 * t + kq)])
                for n in range(7 * outer, 7 * outer + 7):
                    upin[n + zero, :, pl.ds(t * LANE, LANE)] = ops[n]

            return [functools.partial(operands, n, t) for n in range(7) for t in range(KT)]

        def products(a_ref, n_calls, first, steps, zero):
            calls = iter(range(n_calls))
            when = {first + k * (n_calls - first) // len(steps): f for k, f in enumerate(steps)}
            assert len(when) == len(steps)

            def product(granules, n):
                w = jnp.concatenate([aux[pl.ds((g * 49 + n) * TR, TR), :] for g in granules],
                                    axis=0)
                r = _dot(a_ref[n], _w(w))
                step = when.get(next(calls))
                if step is not None:
                    hbuf[SB + zero, 0:8, 0:LANE] = r[0:8]
                    step()
                return r

            return product

        for step in norm_steps(0, 0) + operand_steps(0):
            step()

        def ffn_body(i, carry):
            zero = i // n_blk
            product = products(upin, 2 * 49 * (FT // 4), FIRST[0],
                               norm_steps(jnp.minimum(i + 1, n_blk - 1), zero), zero)
            for j in range(FT // 4):
                gate, up = (_two_level_out(functools.partial(
                    product, range(m * GM + j * KT, m * GM + (j + 1) * KT))) for m in range(2))
                hidden = {rc: _silu(gate[rc]) * up[rc] for rc in gate}
                for n, t in enumerate(_two_level(_strassen_lhs, lambda r, c: hidden[r, c])):
                    act[n, :, lane_tile(j)] = t
            product = products(act, 49 * KT, FIRST[1], operand_steps(zero), zero)
            for j in range(KT):
                c = _two_level_out(functools.partial(product, range(2 * GM + j, 3 * GM, KT)))
                for (rq, nq), t in c.items():
                    cols = slice((4 * j + nq) * LANE, (4 * j + nq + 1) * LANE)
                    y = resid(i * SB + rq, cols=cols) + mod[5, 0:1, cols] * t
                    attn[i * SB + rq, :, cols] = y.astype(BF16)
            sl = pl.ds(i * SB, SB)
            pltpu.make_async_copy(attn.at[sl], out_hbm.at[sl], sems.at[S_OUT]).start()
            return carry

        lax.fori_loop(0, n_blk, ffn_body, 0)

    pl.run_scoped(ffn, pltpu.VMEM((49, seg, d_ff // 4), F32),
                  pltpu.VMEM((49, seg, D // 4), F32), pltpu.VMEM((SB + 1, seg, D), F32))
    pltpu.make_async_copy(attn, out_hbm, sems.at[S_OUT]).wait()


@functools.partial(jax.jit, static_argnames=("A_seg_len",))
def pallas_adaLN_cond__memory_aug_recurrent_mem_tr__glu_gated_swiglu__prompt_kernel(
    A_x, A_mem0, A_Wq, A_Wk, A_Wv, A_Wo, A_seg_len, B_x, B_w1, B_w3, B_w2, c, w_mod,
):
    del B_x
    B, S, D = A_x.shape
    _, H, Dh = A_Wq.shape
    M = A_mem0.shape[1]
    F = B_w1.shape[1]
    seg = int(A_seg_len)
    n_seg = S // seg
    n_gran = 3 * (D // (4 * LANE)) * (F // (4 * LANE))
    assert max(n_gran // 3, 2 * D // LANE) <= n_seg - n_gran and AHEAD < RING
    assert B == 1 and Dh == LANE and S % seg == 0 and n_seg % 4 == 0
    kern = functools.partial(_kernel, seg=seg, n_seg=n_seg, n_mem=M, n_head=H, d_model=D, d_ff=F)
    hbm = pl.BlockSpec(memory_space=pl.ANY)
    vmem = pl.BlockSpec(memory_space=pltpu.VMEM)
    out = pl.pallas_call(
        kern,
        out_shape=jax.ShapeDtypeStruct((n_seg, seg, D), A_x.dtype),
        in_specs=[vmem, vmem] + [hbm] * 9,
        out_specs=hbm,
        scratch_shapes=[
            pltpu.VMEM((3 * H, D // 2, LANE), U32),
            pltpu.VMEM((D // LANE, H * Dh // 2, LANE), U32),
            pltpu.VMEM(((49 * n_gran + 16) * LANE // 2 + 3 * H * PRE, LANE), U32),
            pltpu.VMEM((n_seg, seg, D), BF16),
            pltpu.VMEM((n_seg, seg, D), BF16),
            pltpu.VMEM((M + seg - PRE, D), BF16),
            pltpu.VMEM((6, 8, D), F32),
            pltpu.SemaphoreType.DMA((6 + RING,)),
        ],
        compiler_params=pltpu.CompilerParams(vmem_limit_bytes=127 * 1024 * 1024,
                                             disable_bounds_checks=True),
    )(c, A_mem0.reshape(M, D), A_x.reshape(n_seg, seg, D),
      A_Wq.reshape(D // 2, 2 * H, Dh), A_Wk.reshape(D // 2, 2 * H, Dh),
      A_Wv.reshape(D // 2, 2 * H, Dh),
      A_Wo.reshape(H * Dh, D), B_w1, B_w3, B_w2, w_mod)
    return out.reshape(B, S, D)
```

```python
import functools

import jax
import jax.numpy as jnp
from jax import lax
import jax.experimental.pallas as pl
import jax.experimental.pallas.tpu as pltpu

F32 = jnp.float32
BF16 = jnp.bfloat16
U32 = jnp.uint32
LANE = 128
EPS = 1e-5
PRE = 8
HG = 4
SPLIT = 8
AHEAD = 3
RING = 4
CW = ((2, 5), (3, 6), (1,), (0, 4))
FIRST = (60, 56)
LN_ROWS = 16
PAIRS_PER_IT = 2


def _layernorm(x):
    m = jnp.mean(x, axis=-1, keepdims=True)
    d = x - m
    v = jnp.mean(d * d, axis=-1, keepdims=True)
    return d * lax.rsqrt(v + EPS)


def _silu(x):
    h = 0.5 * x
    return h + h * jnp.tanh(h)


def _w(tile_u32):
    return pltpu.bitcast(tile_u32, BF16)


def _dot(a, b):
    return lax.dot_general(a, b, (((1,), (0,)), ((), ())), preferred_element_type=F32)


def _dot_nt(a, b):
    return lax.dot_general(a, b, (((1,), (1,)), ((), ())), preferred_element_type=F32)


def _add(a, b):
    return jax.tree.map(jnp.add, a, b)


def _sub(a, b):
    return jax.tree.map(jnp.subtract, a, b)


def _strassen_lhs(a11, a12, a21, a22):
    return [_add(a11, a22), _add(a21, a22), a11, a22, _add(a11, a12), _sub(a21, a11),
            _sub(a12, a22)]


def _strassen_rhs(b11, b12, b21, b22):
    return [_add(b11, b22), b11, _sub(b12, b22), _sub(b21, b11), b22, _add(b11, b12),
            _add(b21, b22)]


def _strassen_out(prod):
    m1, m3 = prod(1), prod(3)
    c21 = _add(m1, m3)
    m4 = prod(4)
    c11 = _sub(m3, m4)
    m2 = prod(2)
    c12 = _add(m2, m4)
    c22 = _sub(m2, m1)
    m0 = prod(0)
    c11, c22 = _add(c11, m0), _add(c22, m0)
    c22 = _add(c22, prod(5))
    return [_add(c11, prod(6)), c12, c21, c22]


def _two_level(operands, block):
    halves = [[block(2 * r1 + r2, 2 * c1 + c2) for r2 in range(2) for c2 in range(2)]
              for r1 in range(2) for c1 in range(2)]
    return [t for outer in operands(*halves) for t in operands(*outer)]


def _two_level_out(prod):
    c = _strassen_out(lambda n: _strassen_out(lambda m: prod(7 * n + m)))
    return {(2 * (o // 2) + i // 2, 2 * (o % 2) + i % 2): c[o][i]
            for o in (2, 1, 3, 0) for i in (2, 1, 3, 0)}


def _kernel(c_ref, mem_ref, x_hbm, wq_hbm, wk_hbm, wv_hbm, wo_hbm, w1_hbm, w3_hbm, w2_hbm,
            wmod_hbm, out_hbm,
            wqkv, wo, aux, xs, attn, lhs, mod,
            sems, *, seg, n_seg, n_mem, n_head, d_model, d_ff):
    D, H, M = d_model, n_head, n_mem
    DT = D // LANE
    FT = d_ff // LANE
    L = M + seg
    CUR = seg - PRE
    PP = PAIRS_PER_IT
    n_it = 3 * H // (2 * PP)
    it_per_mat = n_it // 3
    (S_XP, S_X, S_WO, S_FF, S_OUT, S_MOD, S_ST) = range(7)

    NP = n_seg * PRE
    TR = LANE // 2
    GM = (DT // 4) * (FT // 4)
    s0 = n_seg - 3 * GM
    PR = 3 * H * PRE
    item = 16 * TR + PR

    def raw_base(g):
        return aux.shape[0] - item * (3 * GM - g)

    def pre_base(s, late):
        return raw_base(s - s0) + 16 * TR if late else s * PR

    def wmod_rows(part, j):
        return aux_rows(s0 * PR + (part * 2 * DT + j) * (D // 2), D // 2)

    def aux_rows(start, size):
        return pl.ds(start if isinstance(start, int) else pl.multiple_of(start, 8), size)

    def lane_tile(j):
        return pl.ds(j * LANE if isinstance(j, int) else pl.multiple_of(j * LANE, LANE), LANE)

    def wmod_copy(part, j):
        return pltpu.make_async_copy(
            wmod_hbm.bitcast(U32).at[:, lane_tile(part * 2 * DT + j)],
            aux.at[wmod_rows(part, j), :], sems.at[S_MOD])

    def wmod_copies(part):
        return [wmod_copy(part, j) for j in range(2 * DT)]

    def wo_copy(half, j):
        rows = pl.ds(half * (H // 2) * TR, (H // 2) * TR)
        return pltpu.make_async_copy(wo_hbm.bitcast(U32).at[rows, lane_tile(j)], wo.at[j, rows],
                                     sems.at[S_WO])

    x_copy = pltpu.make_async_copy(x_hbm, xs, sems.at[S_X])

    def ffn_copy(m, i, nq):
        per_row = DT // 4
        kk, j = (i % per_row, i // per_row) if m < 2 else (i // per_row, i % per_row)
        return pltpu.make_async_copy(
            (w1_hbm, w3_hbm, w2_hbm)[m].bitcast(U32).at[aux_rows(kk * 4 * TR, 4 * TR),
                                                        lane_tile(4 * j + nq)],
            aux.at[aux_rows(raw_base(m * GM + i) + nq * 4 * TR, 4 * TR), :], sems.at[S_FF])

    def prefetch_ffn(s, part):
        if part < 6:
            @pl.when(s < GM)
            def _():
                for nq in range(2):
                    ffn_copy(part // 2, s, 2 * (part % 2) + nq).start()
        elif part == 6:
            @pl.when(s < 2 * DT)
            def _():
                wmod_copy(1, s).start()
                wmod_copy(2, s).start()

    def start(cps):
        for cp in cps:
            cp.start()

    def wait(cps):
        for cp in cps:
            cp.wait()

    def modulation(part):
        sc = jnp.broadcast_to(_silu(c_ref[...].astype(F32)), (8, D))
        for j in range(2 * DT):
            r = _dot(sc, _w(aux[wmod_rows(part, j), :]))
            mod[2 * part + j // DT, :, pl.ds((j % DT) * LANE, LANE)] = r

    def modrow(i):
        return mod[i, 0:1, :]

    def prologue(ring, xp, hp):
        def pair_copies(w_hbm, i):
            src = w_hbm.bitcast(U32)
            return [pltpu.make_async_copy(
                src.at[:, (i % it_per_mat) * PP + t + par * (H // 2), :],
                ring.at[i % RING, 2 * t + par], sems.at[S_ST + i % RING])
                for t in range(PP) for par in range(2)]

        xp_copy = pltpu.make_async_copy(x_hbm.at[:, pl.ds(CUR, PRE), :], xp, sems.at[S_XP])
        xp_copy.start()
        start(wmod_copies(0))
        xp_copy.wait()
        xn = _layernorm(xp[...].astype(F32).reshape(n_seg * PRE, D))
        wait(wmod_copies(0))
        for i in range(AHEAD):
            start(pair_copies(wq_hbm, i))
        modulation(0)
        hn = xn * (1.0 + modrow(1)) + modrow(0)
        r, k = NP // 4, D // 4
        ops = _two_level(_strassen_lhs, lambda rq, kq: hn[rq * r:(rq + 1) * r, kq * k:(kq + 1) * k])
        for n, t in enumerate(ops):
            hp[n] = t.astype(BF16)

        def pro_body(w_next, wo_half, i, carry):
            wait(pair_copies(wq_hbm, i))
            heads = []
            for t in range(PP):
                a = ring[i % RING, 2 * t]
                b = ring[i % RING, 2 * t + 1]
                heads += [(a & jnp.uint32(0xFFFF)) | (b << 16),
                          (a >> 16) | (b & jnp.uint32(0xFFFF0000))]
            for n, w in enumerate(heads):
                wqkv[i * 2 * PP + n] = w
            if w_next is not None:
                start(pair_copies(w_next, i + AHEAD))
            if wo_half is not None:
                wo_copy(wo_half, (i + AHEAD) % it_per_mat).start()
            rhs = _two_level(_strassen_rhs, lambda kq, nq: _w(
                heads[nq][kq * (D // 8):(kq + 1) * (D // 8)]).astype(F32))
            c = _two_level_out(lambda n: _dot(hp[n], rhs[n].astype(BF16)))
            for (rq, nq), val in c.items():
                for j in range(n_seg // 4):
                    sg = rq * (n_seg // 4) + j
                    r0 = pre_base(sg, sg >= s0) + (i * 2 * PP + nq) * PRE
                    aux[aux_rows(r0, PRE), :] = pltpu.bitcast(val[j * PRE:(j + 1) * PRE], U32)
            return carry

        for m, (w_hbm, wo_half) in enumerate(((wq_hbm, None), (wk_hbm, 0), (wv_hbm, 1))):
            lax.fori_loop(max(m * it_per_mat - AHEAD, 0), (m + 1) * it_per_mat - AHEAD,
                          functools.partial(pro_body, w_hbm, wo_half), 0)
        x_copy.start()
        lax.fori_loop(n_it - AHEAD, n_it, functools.partial(pro_body, None, None), 0)

    pl.run_scoped(prologue, pltpu.VMEM((RING, 2 * PP, D // 2, LANE), U32),
                  pltpu.VMEM((n_seg, PRE, D), BF16), pltpu.VMEM((49, NP // 4, D // 4), BF16))
    wait([wo_copy(half, j) for half in range(2) for j in range(DT)])
    x_copy.wait()

    def seg_rows(s):
        xn = _layernorm(xs[s].astype(F32)[0:CUR])
        return xn * (1.0 + modrow(1)) + modrow(0)

    lhs[...] = jnp.concatenate([mem_ref[...].astype(F32), seg_rows(0)], axis=0).astype(BF16)
    scale = float(LANE) ** -0.5
    NG = H // HG

    def chain_body(combine, s, carry):
        row = lax.broadcasted_iota(jnp.int32, (L, L), 0)
        col = lax.broadcasted_iota(jnp.int32, (L, L), 1)
        mask = (row < M) | (row >= col)
        q, k, v, p, ov = {}, {}, {}, {}, {}

        def heads(g):
            return range(g * HG, (g + 1) * HG)

        def proj(m, h):
            done = aux[aux_rows(pre_base(s, combine) + (m * H + h) * PRE, PRE), :]
            return jnp.concatenate([_dot(lhs[...], _w(wqkv[m * H + h])),
                                    pltpu.bitcast(done, F32)], axis=0)

        def probs(g):
            for h in heads(g):
                z = jnp.where(mask, _dot_nt(q[h], k[h]) * scale, -1e9)
                e = jnp.exp(z - jnp.max(z, axis=-1, keepdims=True))
                p[h] = e / jnp.sum(e, axis=-1, keepdims=True)

        def values(g):
            for h in heads(g):
                ov[h] = _dot(p[h], v[h])

        def out_proj(h0, h1, marks):
            o = jnp.concatenate([ov[h] for h in range(h0, h1)], axis=1)
            cols = []
            for j in range(DT):
                cols.append(_dot(o, _w(wo[j, pl.ds(h0 * TR, (h1 - h0) * TR), :])))
                if combine and j in marks:
                    aux[aux_rows(pre_base(s, True), 8), :] = pltpu.bitcast(cols[-1][0:8], U32)
                    combine_weights(marks[j], CW[3])
            return jnp.concatenate(cols, axis=1)

        def combine_weights(g, outer):
            for r in range(g * TR // NG // 8 * 8, (g + 1) * TR // NG // 8 * 8, 8) if combine else ():
                def block(kq, nq):
                    rows = aux_rows(raw_base(s - s0) + (nq * 4 + kq) * TR + r, 8)
                    return _w(aux[rows, :]).astype(F32)

                for n, t in enumerate(_two_level(_strassen_rhs, block)):
                    if n // 7 in outer:
                        rows = aux_rows(((s - s0) * 49 + n) * TR + r, 8)
                        aux[rows, :] = pltpu.bitcast(t.astype(BF16), U32)

        for g in range(NG):
            combine_weights(g, CW[0])
            for h in heads(g):
                k[h] = proj(1, h).astype(BF16)
            combine_weights(g, CW[1])
            for h in heads(g):
                q[h] = proj(0, h)
            if g >= 1:
                probs(g - 1)
            if not combine:
                prefetch_ffn(s, g)
        for g in range(NG):
            combine_weights(g, CW[2])
            for h in heads(g):
                v[h] = proj(2, h).astype(BF16)
            if g == 0:
                probs(NG - 1)
            else:
                values(g - 1)
        nxt = seg_rows(jnp.minimum(s + 1, n_seg - 1))
        o = out_proj(0, SPLIT, {DT // 2 - 1: 0, DT - 1: 1})
        values(NG - 1)
        o = o + out_proj(SPLIT, H, {j: j + 2 for j in range(NG - 2)})
        attn[s] = o[M:].astype(BF16)
        lhs[...] = jnp.concatenate([o[:M], nxt], axis=0).astype(BF16)
        return carry

    lax.fori_loop(0, s0, functools.partial(chain_body, False), 0)
    wait([ffn_copy(m, i, nq) for m in range(3) for i in range(GM) for nq in range(4)])
    wait(wmod_copies(1))
    wait(wmod_copies(2))
    modulation(1)
    modulation(2)
    lax.fori_loop(s0, n_seg, functools.partial(chain_body, True), 0)

    SB = 4
    n_blk = n_seg // SB

    def resid(sg, rows=slice(None), cols=slice(None)):
        return (xs[sg, rows, cols].astype(F32)
                + mod[2, 0:1, cols] * attn[sg, rows, cols].astype(F32))

    def ffn(act, upin, hbuf):
        KT = DT // 4

        def norm_steps(i, zero):
            def center(sg, rows):
                x1 = resid(i * SB + sg, rows=rows)
                hbuf[sg + zero, rows] = x1 - jnp.mean(x1, axis=-1, keepdims=True)

            def normalize(sg, rows):
                d = hbuf[sg, rows]
                rstd = lax.rsqrt(jnp.mean(d * d, axis=-1, keepdims=True) + EPS)
                hbuf[sg + zero, rows] = d * rstd * (1.0 + modrow(4)) + modrow(3)

            return [functools.partial(f, sg, slice(r, r + LN_ROWS)) for f in (center, normalize)
                    for sg in range(SB) for r in range(0, seg, LN_ROWS)]

        def operand_steps(zero):
            def operands(outer, t):
                ops = _two_level(_strassen_lhs,
                                 lambda rq, kq: hbuf[rq, :, lane_tile(4 * t + kq)])
                for n in range(7 * outer, 7 * outer + 7):
                    upin[n + zero, :, pl.ds(t * LANE, LANE)] = ops[n]

            return [functools.partial(operands, n, t) for n in range(7) for t in range(KT)]

        def products(a_ref, n_calls, first, steps, zero):
            calls = iter(range(n_calls))
            when = {first + k * (n_calls - first) // len(steps): f for k, f in enumerate(steps)}
            assert len(when) == len(steps)

            def product(granules, n):
                w = jnp.concatenate([aux[pl.ds((g * 49 + n) * TR, TR), :] for g in granules],
                                    axis=0)
                r = _dot(a_ref[n], _w(w))
                step = when.get(next(calls))
                if step is not None:
                    hbuf[SB + zero, 0:8, 0:LANE] = r[0:8]
                    step()
                return r

            return product

        for step in norm_steps(0, 0) + operand_steps(0):
            step()

        def ffn_body(i, carry):
            zero = i // n_blk
            product = products(upin, 2 * 49 * (FT // 4), FIRST[0],
                               norm_steps(jnp.minimum(i + 1, n_blk - 1), zero), zero)
            for j in range(FT // 4):
                gate, up = (_two_level_out(functools.partial(
                    product, range(m * GM + j * KT, m * GM + (j + 1) * KT))) for m in range(2))
                hidden = {rc: _silu(gate[rc]) * up[rc] for rc in gate}
                for n, t in enumerate(_two_level(_strassen_lhs, lambda r, c: hidden[r, c])):
                    act[n, :, lane_tile(j)] = t
            product = products(act, 49 * KT, FIRST[1], operand_steps(zero), zero)
            for j in range(KT):
                c = _two_level_out(functools.partial(product, range(2 * GM + j, 3 * GM, KT)))
                for (rq, nq), t in c.items():
                    cols = slice((4 * j + nq) * LANE, (4 * j + nq + 1) * LANE)
                    y = resid(i * SB + rq, cols=cols) + mod[5, 0:1, cols] * t
                    attn[i * SB + rq, :, cols] = y.astype(BF16)
            sl = pl.ds(i * SB, SB)
            pltpu.make_async_copy(attn.at[sl], out_hbm.at[sl], sems.at[S_OUT]).start()
            return carry

        lax.fori_loop(0, n_blk, ffn_body, 0)

    pl.run_scoped(ffn, pltpu.VMEM((49, seg, d_ff // 4), F32),
                  pltpu.VMEM((49, seg, D // 4), F32), pltpu.VMEM((SB + 1, seg, D), F32))
    pltpu.make_async_copy(attn, out_hbm, sems.at[S_OUT]).wait()


@functools.partial(jax.jit, static_argnames=("A_seg_len",))
def pallas_adaLN_cond__memory_aug_recurrent_mem_tr__glu_gated_swiglu__prompt_kernel(
    A_x, A_mem0, A_Wq, A_Wk, A_Wv, A_Wo, A_seg_len, B_x, B_w1, B_w3, B_w2, c, w_mod,
):
    del B_x
    B, S, D = A_x.shape
    _, H, Dh = A_Wq.shape
    M = A_mem0.shape[1]
    F = B_w1.shape[1]
    seg = int(A_seg_len)
    n_seg = S // seg
    n_gran = 3 * (D // (4 * LANE)) * (F // (4 * LANE))
    assert max(n_gran // 3, 2 * D // LANE) <= n_seg - n_gran and AHEAD < RING
    assert B == 1 and Dh == LANE and S % seg == 0 and n_seg % 4 == 0
    kern = functools.partial(_kernel, seg=seg, n_seg=n_seg, n_mem=M, n_head=H, d_model=D, d_ff=F)
    hbm = pl.BlockSpec(memory_space=pl.ANY)
    vmem = pl.BlockSpec(memory_space=pltpu.VMEM)
    out = pl.pallas_call(
        kern,
        out_shape=jax.ShapeDtypeStruct((n_seg, seg, D), A_x.dtype),
        in_specs=[vmem, vmem] + [hbm] * 9,
        out_specs=hbm,
        scratch_shapes=[
            pltpu.VMEM((3 * H, D // 2, LANE), U32),
            pltpu.VMEM((D // LANE, H * Dh // 2, LANE), U32),
            pltpu.VMEM(((49 * n_gran + 16) * LANE // 2 + 3 * H * PRE, LANE), U32),
            pltpu.VMEM((n_seg, seg, D), BF16),
            pltpu.VMEM((n_seg, seg, D), BF16),
            pltpu.VMEM((M + seg - PRE, D), BF16),
            pltpu.VMEM((6, 8, D), F32),
            pltpu.SemaphoreType.DMA((6 + RING,)),
        ],
        compiler_params=pltpu.CompilerParams(vmem_limit_bytes=127 * 1024 * 1024,
                                             disable_bounds_checks=True),
    )(c, A_mem0.reshape(M, D), A_x.reshape(n_seg, seg, D),
      A_Wq.reshape(D // 2, 2 * H, Dh), A_Wk.reshape(D // 2, 2 * H, Dh),
      A_Wv.reshape(D // 2, 2 * H, Dh),
      A_Wo.reshape(H * Dh, D), B_w1, B_w3, B_w2, w_mod)
    return out.reshape(B, S, D)
```

```python
import functools

import jax
import jax.numpy as jnp
from jax import lax
import jax.experimental.pallas as pl
import jax.experimental.pallas.tpu as pltpu

F32 = jnp.float32
BF16 = jnp.bfloat16
U32 = jnp.uint32
LANE = 128
EPS = 1e-5
PRE = 8
HG = 4
SPLIT = 8
AHEAD = 3
RING = 4
CW = ((2, 5), (3, 6), (1,), (0, 4))
FIRST = (60, 56)
LN_ROWS = 16
PAIRS_PER_IT = 2


def _layernorm(x):
    m = jnp.mean(x, axis=-1, keepdims=True)
    d = x - m
    v = jnp.mean(d * d, axis=-1, keepdims=True)
    return d * lax.rsqrt(v + EPS)


def _silu(x):
    h = 0.5 * x
    return h + h * jnp.tanh(h)


def _w(tile_u32):
    return pltpu.bitcast(tile_u32, BF16)


def _dot(a, b):
    return lax.dot_general(a, b, (((1,), (0,)), ((), ())), preferred_element_type=F32)


def _dot_nt(a, b):
    return lax.dot_general(a, b, (((1,), (1,)), ((), ())), preferred_element_type=F32)


def _add(a, b):
    return jax.tree.map(jnp.add, a, b)


def _sub(a, b):
    return jax.tree.map(jnp.subtract, a, b)


def _strassen_lhs(a11, a12, a21, a22):
    return [_add(a11, a22), _add(a21, a22), a11, a22, _add(a11, a12), _sub(a21, a11),
            _sub(a12, a22)]


def _strassen_rhs(b11, b12, b21, b22):
    return [_add(b11, b22), b11, _sub(b12, b22), _sub(b21, b11), b22, _add(b11, b12),
            _add(b21, b22)]


def _strassen_out(prod):
    m1, m3 = prod(1), prod(3)
    c21 = _add(m1, m3)
    m4 = prod(4)
    c11 = _sub(m3, m4)
    m2 = prod(2)
    c12 = _add(m2, m4)
    c22 = _sub(m2, m1)
    m0 = prod(0)
    c11, c22 = _add(c11, m0), _add(c22, m0)
    c22 = _add(c22, prod(5))
    return [_add(c11, prod(6)), c12, c21, c22]


def _two_level(operands, block):
    halves = [[block(2 * r1 + r2, 2 * c1 + c2) for r2 in range(2) for c2 in range(2)]
              for r1 in range(2) for c1 in range(2)]
    return [t for outer in operands(*halves) for t in operands(*outer)]


def _two_level_out(prod):
    c = _strassen_out(lambda n: _strassen_out(lambda m: prod(7 * n + m)))
    return {(2 * (o // 2) + i // 2, 2 * (o % 2) + i % 2): c[o][i]
            for o in (2, 1, 3, 0) for i in (2, 1, 3, 0)}


def _kernel(c_ref, mem_ref, x_hbm, wq_hbm, wk_hbm, wv_hbm, wo_hbm, w1_hbm, w3_hbm, w2_hbm,
            wmod_hbm, out_hbm,
            wqkv, wo, aux, xs, attn, lhs, mod,
            sems, *, seg, n_seg, n_mem, n_head, d_model, d_ff):
    D, H, M = d_model, n_head, n_mem
    DT = D // LANE
    FT = d_ff // LANE
    L = M + seg
    CUR = seg - PRE
    PP = PAIRS_PER_IT
    n_it = 3 * H // (2 * PP)
    it_per_mat = n_it // 3
    (S_XP, S_X, S_WO, S_FF, S_OUT, S_MOD, S_ST) = range(7)

    NP = n_seg * PRE
    TR = LANE // 2
    GM = (DT // 4) * (FT // 4)
    s0 = n_seg - 3 * GM
    PR = 3 * H * PRE
    item = 16 * TR + PR

    def raw_base(g):
        return aux.shape[0] - item * (3 * GM - g)

    def pre_base(s, late):
        return raw_base(s - s0) + 16 * TR if late else s * PR

    def wmod_rows(part, j):
        return aux_rows(s0 * PR + (part * 2 * DT + j) * (D // 2), D // 2)

    def aux_rows(start, size):
        return pl.ds(start if isinstance(start, int) else pl.multiple_of(start, 8), size)

    def lane_tile(j):
        return pl.ds(j * LANE if isinstance(j, int) else pl.multiple_of(j * LANE, LANE), LANE)

    def wmod_copy(part, j, sem=S_MOD):
        return pltpu.make_async_copy(
            wmod_hbm.bitcast(U32).at[:, lane_tile(part * 2 * DT + j)],
            aux.at[wmod_rows(part, j), :], sems.at[sem])

    def wo_copy(half, j):
        rows = pl.ds(half * (H // 2) * TR, (H // 2) * TR)
        return pltpu.make_async_copy(wo_hbm.bitcast(U32).at[rows, lane_tile(j)], wo.at[j, rows],
                                     sems.at[S_WO])

    x_copy = pltpu.make_async_copy(x_hbm, xs, sems.at[S_X])

    def ffn_copy(m, i, nq):
        per_row = DT // 4
        kk, j = (i % per_row, i // per_row) if m < 2 else (i // per_row, i % per_row)
        return pltpu.make_async_copy(
            (w1_hbm, w3_hbm, w2_hbm)[m].bitcast(U32).at[aux_rows(kk * 4 * TR, 4 * TR),
                                                        lane_tile(4 * j + nq)],
            aux.at[aux_rows(raw_base(m * GM + i) + nq * 4 * TR, 4 * TR), :], sems.at[S_FF])

    def prefetch_ffn(s, part):
        if part < 6:
            @pl.when(s < GM)
            def _():
                for nq in range(2):
                    ffn_copy(part // 2, s, 2 * (part % 2) + nq).start()
        elif part == 6:
            @pl.when(s < 2 * DT)
            def _():
                wmod_copy(1, s).start()
                wmod_copy(2, s).start()

    def start(cps):
        for cp in cps:
            cp.start()

    def wait(cps):
        for cp in cps:
            cp.wait()

    def modulation(part, tiles):
        sc = jnp.broadcast_to(_silu(c_ref[...].astype(F32)), (8, D))
        for j in tiles:
            r = _dot(sc, _w(aux[wmod_rows(part, j), :]))
            mod[2 * part + j // DT, :, pl.ds((j % DT) * LANE, LANE)] = r

    def modrow(i):
        return mod[i, 0:1, :]

    def prologue(ring, xp, hp):
        def pair_copies(w_hbm, i):
            src = w_hbm.bitcast(U32)
            return [pltpu.make_async_copy(
                src.at[:, (i % it_per_mat) * PP + t + par * (H // 2), :],
                ring.at[i % RING, 2 * t + par], sems.at[S_ST + i % RING])
                for t in range(PP) for par in range(2)]

        xp_copy = pltpu.make_async_copy(x_hbm.at[:, pl.ds(CUR, PRE), :], xp, sems.at[S_XP])
        xp_copy.start()
        tiles = [range(t, 2 * DT, 2) for t in range(2)]
        halves = [[wmod_copy(0, j, sem) for j in tiles[t]] for t, sem in enumerate((S_MOD, S_FF))]
        start(halves[0])
        xp_copy.wait()
        start(halves[1])
        xn = _layernorm(xp[...].astype(F32).reshape(NP, D))
        for t in range(2):
            wait(halves[t])
            for i in range(t, AHEAD if t else 1):
                start(pair_copies(wq_hbm, i))
            modulation(0, tiles[t])
            for u in range(t, DT // 4, 2):
                def block(rq, kq):
                    cols = slice((kq * (DT // 4) + u) * LANE, (kq * (DT // 4) + u + 1) * LANE)
                    return (xn[rq * (NP // 4):(rq + 1) * (NP // 4), cols]
                            * (1.0 + mod[1, 0:1, cols]) + mod[0, 0:1, cols])

                for n, a in enumerate(_two_level(_strassen_lhs, block)):
                    hp[n, :, lane_tile(u)] = a.astype(BF16)

        def pro_body(w_next, wo_half, i, carry):
            wait(pair_copies(wq_hbm, i))
            heads = []
            for t in range(PP):
                a = ring[i % RING, 2 * t]
                b = ring[i % RING, 2 * t + 1]
                heads += [(a & jnp.uint32(0xFFFF)) | (b << 16),
                          (a >> 16) | (b & jnp.uint32(0xFFFF0000))]
            for n, w in enumerate(heads):
                wqkv[i * 2 * PP + n] = w
            if w_next is not None:
                start(pair_copies(w_next, i + AHEAD))
            if wo_half is not None:
                wo_copy(wo_half, (i + AHEAD) % it_per_mat).start()
            rhs = _two_level(_strassen_rhs, lambda kq, nq: _w(
                heads[nq][kq * (D // 8):(kq + 1) * (D // 8)]).astype(F32))
            c = _two_level_out(lambda n: _dot(hp[n], rhs[n].astype(BF16)))
            for (rq, nq), val in c.items():
                for j in range(n_seg // 4):
                    sg = rq * (n_seg // 4) + j
                    r0 = pre_base(sg, sg >= s0) + (i * 2 * PP + nq) * PRE
                    aux[aux_rows(r0, PRE), :] = pltpu.bitcast(val[j * PRE:(j + 1) * PRE], U32)
            return carry

        for m, (w_hbm, wo_half) in enumerate(((wq_hbm, None), (wk_hbm, 0), (wv_hbm, 1))):
            lax.fori_loop(max(m * it_per_mat - AHEAD, 0), (m + 1) * it_per_mat - AHEAD,
                          functools.partial(pro_body, w_hbm, wo_half), 0)
        x_copy.start()
        lax.fori_loop(n_it - AHEAD, n_it, functools.partial(pro_body, None, None), 0)

    pl.run_scoped(prologue, pltpu.VMEM((RING, 2 * PP, D // 2, LANE), U32),
                  pltpu.VMEM((n_seg, PRE, D), BF16), pltpu.VMEM((49, NP // 4, D // 4), BF16))
    wait([wo_copy(half, j) for half in range(2) for j in range(DT)])
    x_copy.wait()

    def seg_rows(s):
        xn = _layernorm(xs[s].astype(F32)[0:CUR])
        return xn * (1.0 + modrow(1)) + modrow(0)

    lhs[...] = jnp.concatenate([mem_ref[...].astype(F32), seg_rows(0)], axis=0).astype(BF16)
    scale = float(LANE) ** -0.5
    NG = H // HG

    def chain_body(combine, s, carry):
        row = lax.broadcasted_iota(jnp.int32, (L, L), 0)
        col = lax.broadcasted_iota(jnp.int32, (L, L), 1)
        mask = (row < M) | (row >= col)
        q, k, v, p, ov = {}, {}, {}, {}, {}

        def heads(g):
            return range(g * HG, (g + 1) * HG)

        def proj(m, h):
            done = aux[aux_rows(pre_base(s, combine) + (m * H + h) * PRE, PRE), :]
            return jnp.concatenate([_dot(lhs[...], _w(wqkv[m * H + h])),
                                    pltpu.bitcast(done, F32)], axis=0)

        def probs(g):
            for h in heads(g):
                z = jnp.where(mask, _dot_nt(q[h], k[h]) * scale, -1e9)
                e = jnp.exp(z - jnp.max(z, axis=-1, keepdims=True))
                p[h] = e / jnp.sum(e, axis=-1, keepdims=True)

        def values(g):
            for h in heads(g):
                ov[h] = _dot(p[h], v[h])

        def out_proj(h0, h1, marks):
            o = jnp.concatenate([ov[h] for h in range(h0, h1)], axis=1)
            cols = []
            for j in range(DT):
                cols.append(_dot(o, _w(wo[j, pl.ds(h0 * TR, (h1 - h0) * TR), :])))
                if combine and j in marks:
                    aux[aux_rows(pre_base(s, True), 8), :] = pltpu.bitcast(cols[-1][0:8], U32)
                    combine_weights(marks[j], CW[3])
            return jnp.concatenate(cols, axis=1)

        def combine_weights(g, outer):
            for r in range(g * TR // NG // 8 * 8, (g + 1) * TR // NG // 8 * 8, 8) if combine else ():
                def block(kq, nq):
                    rows = aux_rows(raw_base(s - s0) + (nq * 4 + kq) * TR + r, 8)
                    return _w(aux[rows, :]).astype(F32)

                for n, t in enumerate(_two_level(_strassen_rhs, block)):
                    if n // 7 in outer:
                        rows = aux_rows(((s - s0) * 49 + n) * TR + r, 8)
                        aux[rows, :] = pltpu.bitcast(t.astype(BF16), U32)

        for g in range(NG):
            combine_weights(g, CW[0])
            for h in heads(g):
                k[h] = proj(1, h).astype(BF16)
            combine_weights(g, CW[1])
            for h in heads(g):
                q[h] = proj(0, h)
            if g >= 1:
                probs(g - 1)
            if not combine:
                prefetch_ffn(s, g)
        for g in range(NG):
            combine_weights(g, CW[2])
            for h in heads(g):
                v[h] = proj(2, h).astype(BF16)
            if g == 0:
                probs(NG - 1)
            else:
                values(g - 1)
        nxt = seg_rows(jnp.minimum(s + 1, n_seg - 1))
        o = out_proj(0, SPLIT, {DT // 2 - 1: 0, DT - 1: 1})
        values(NG - 1)
        o = o + out_proj(SPLIT, H, {j: j + 2 for j in range(NG - 2)})
        attn[s] = o[M:].astype(BF16)
        lhs[...] = jnp.concatenate([o[:M], nxt], axis=0).astype(BF16)
        return carry

    lax.fori_loop(0, s0, functools.partial(chain_body, False), 0)
    wait([ffn_copy(m, i, nq) for m in range(3) for i in range(GM) for nq in range(4)])
    wait([wmod_copy(part, j) for part in (1, 2) for j in range(2 * DT)])
    modulation(1, range(2 * DT))
    modulation(2, range(2 * DT))
    lax.fori_loop(s0, n_seg, functools.partial(chain_body, True), 0)

    SB = 4
    n_blk = n_seg // SB

    def resid(sg, rows=slice(None), cols=slice(None)):
        return (xs[sg, rows, cols].astype(F32)
                + mod[2, 0:1, cols] * attn[sg, rows, cols].astype(F32))

    def ffn(act, upin, hbuf):
        KT = DT // 4

        def norm_steps(i, zero):
            def center(sg, rows):
                x1 = resid(i * SB + sg, rows=rows)
                hbuf[sg + zero, rows] = x1 - jnp.mean(x1, axis=-1, keepdims=True)

            def normalize(sg, rows):
                d = hbuf[sg, rows]
                rstd = lax.rsqrt(jnp.mean(d * d, axis=-1, keepdims=True) + EPS)
                hbuf[sg + zero, rows] = d * rstd * (1.0 + modrow(4)) + modrow(3)

            return [functools.partial(f, sg, slice(r, r + LN_ROWS)) for f in (center, normalize)
                    for sg in range(SB) for r in range(0, seg, LN_ROWS)]

        def operand_steps(zero):
            def operands(outer, t):
                ops = _two_level(_strassen_lhs,
                                 lambda rq, kq: hbuf[rq, :, lane_tile(4 * t + kq)])
                for n in range(7 * outer, 7 * outer + 7):
                    upin[n + zero, :, pl.ds(t * LANE, LANE)] = ops[n]

            return [functools.partial(operands, n, t) for n in range(7) for t in range(KT)]

        def products(a_ref, n_calls, first, steps, zero):
            calls = iter(range(n_calls))
            when = {first + k * (n_calls - first) // len(steps): f for k, f in enumerate(steps)}
            assert len(when) == len(steps)

            def product(granules, n):
                w = jnp.concatenate([aux[pl.ds((g * 49 + n) * TR, TR), :] for g in granules],
                                    axis=0)
                r = _dot(a_ref[n], _w(w))
                step = when.get(next(calls))
                if step is not None:
                    hbuf[SB + zero, 0:8, 0:LANE] = r[0:8]
                    step()
                return r

            return product

        for step in norm_steps(0, 0) + operand_steps(0):
            step()

        def ffn_body(i, carry):
            zero = i // n_blk
            product = products(upin, 2 * 49 * (FT // 4), FIRST[0],
                               norm_steps(jnp.minimum(i + 1, n_blk - 1), zero), zero)
            for j in range(FT // 4):
                gate, up = (_two_level_out(functools.partial(
                    product, range(m * GM + j * KT, m * GM + (j + 1) * KT))) for m in range(2))
                hidden = {rc: _silu(gate[rc]) * up[rc] for rc in gate}
                for n, t in enumerate(_two_level(_strassen_lhs, lambda r, c: hidden[r, c])):
                    act[n, :, lane_tile(j)] = t
            product = products(act, 49 * KT, FIRST[1], operand_steps(zero), zero)
            for j in range(KT):
                c = _two_level_out(functools.partial(product, range(2 * GM + j, 3 * GM, KT)))
                for (rq, nq), t in c.items():
                    cols = slice((4 * j + nq) * LANE, (4 * j + nq + 1) * LANE)
                    y = resid(i * SB + rq, cols=cols) + mod[5, 0:1, cols] * t
                    attn[i * SB + rq, :, cols] = y.astype(BF16)
            sl = pl.ds(i * SB, SB)
            pltpu.make_async_copy(attn.at[sl], out_hbm.at[sl], sems.at[S_OUT]).start()
            return carry

        lax.fori_loop(0, n_blk, ffn_body, 0)

    pl.run_scoped(ffn, pltpu.VMEM((49, seg, d_ff // 4), F32),
                  pltpu.VMEM((49, seg, D // 4), F32), pltpu.VMEM((SB + 1, seg, D), F32))
    pltpu.make_async_copy(attn, out_hbm, sems.at[S_OUT]).wait()


@functools.partial(jax.jit, static_argnames=("A_seg_len",))
def pallas_adaLN_cond__memory_aug_recurrent_mem_tr__glu_gated_swiglu__prompt_kernel(
    A_x, A_mem0, A_Wq, A_Wk, A_Wv, A_Wo, A_seg_len, B_x, B_w1, B_w3, B_w2, c, w_mod,
):
    del B_x
    B, S, D = A_x.shape
    _, H, Dh = A_Wq.shape
    M = A_mem0.shape[1]
    F = B_w1.shape[1]
    seg = int(A_seg_len)
    n_seg = S // seg
    n_gran = 3 * (D // (4 * LANE)) * (F // (4 * LANE))
    assert max(n_gran // 3, 2 * D // LANE) <= n_seg - n_gran and AHEAD < RING
    assert B == 1 and Dh == LANE and S % seg == 0 and n_seg % 4 == 0
    kern = functools.partial(_kernel, seg=seg, n_seg=n_seg, n_mem=M, n_head=H, d_model=D, d_ff=F)
    hbm = pl.BlockSpec(memory_space=pl.ANY)
    vmem = pl.BlockSpec(memory_space=pltpu.VMEM)
    out = pl.pallas_call(
        kern,
        out_shape=jax.ShapeDtypeStruct((n_seg, seg, D), A_x.dtype),
        in_specs=[vmem, vmem] + [hbm] * 9,
        out_specs=hbm,
        scratch_shapes=[
            pltpu.VMEM((3 * H, D // 2, LANE), U32),
            pltpu.VMEM((D // LANE, H * Dh // 2, LANE), U32),
            pltpu.VMEM(((49 * n_gran + 16) * LANE // 2 + 3 * H * PRE, LANE), U32),
            pltpu.VMEM((n_seg, seg, D), BF16),
            pltpu.VMEM((n_seg, seg, D), BF16),
            pltpu.VMEM((M + seg - PRE, D), BF16),
            pltpu.VMEM((6, 8, D), F32),
            pltpu.SemaphoreType.DMA((6 + RING,)),
        ],
        compiler_params=pltpu.CompilerParams(vmem_limit_bytes=127 * 1024 * 1024,
                                             disable_bounds_checks=True),
    )(c, A_mem0.reshape(M, D), A_x.reshape(n_seg, seg, D),
      A_Wq.reshape(D // 2, 2 * H, Dh), A_Wk.reshape(D // 2, 2 * H, Dh),
      A_Wv.reshape(D // 2, 2 * H, Dh),
      A_Wo.reshape(H * Dh, D), B_w1, B_w3, B_w2, w_mod)
    return out.reshape(B, S, D)
```

```python
import functools

import jax
import jax.numpy as jnp
from jax import lax
import jax.experimental.pallas as pl
import jax.experimental.pallas.tpu as pltpu

F32 = jnp.float32
BF16 = jnp.bfloat16
U32 = jnp.uint32
LANE = 128
EPS = 1e-5
PRE = 8
HG = 4
SPLIT = 8
AHEAD = 3
RING = 4
CW = ((2, 5), (3, 6), (0, 4), (1,))
FIRST = (60, 56)
LN_ROWS = 16


def _layernorm(x):
    m = jnp.mean(x, axis=-1, keepdims=True)
    d = x - m
    v = jnp.mean(d * d, axis=-1, keepdims=True)
    return d * lax.rsqrt(v + EPS)


def _silu(x):
    h = 0.5 * x
    return h + h * jnp.tanh(h)


def _w(tile_u32):
    return pltpu.bitcast(tile_u32, BF16)


def _dot(a, b):
    return lax.dot_general(a, b, (((1,), (0,)), ((), ())), preferred_element_type=F32)


def _dot_nt(a, b):
    return lax.dot_general(a, b, (((1,), (1,)), ((), ())), preferred_element_type=F32)


def _add(a, b):
    return jax.tree.map(jnp.add, a, b)


def _sub(a, b):
    return jax.tree.map(jnp.subtract, a, b)


def _strassen_lhs(a11, a12, a21, a22):
    return [_add(a11, a22), _add(a21, a22), a11, a22, _add(a11, a12), _sub(a21, a11),
            _sub(a12, a22)]


def _strassen_rhs(b11, b12, b21, b22):
    return [_add(b11, b22), b11, _sub(b12, b22), _sub(b21, b11), b22, _add(b11, b12),
            _add(b21, b22)]


def _strassen_out(prod):
    m1, m3 = prod(1), prod(3)
    c21 = _add(m1, m3)
    m4 = prod(4)
    c11 = _sub(m3, m4)
    m2 = prod(2)
    c12 = _add(m2, m4)
    c22 = _sub(m2, m1)
    m0 = prod(0)
    c11, c22 = _add(c11, m0), _add(c22, m0)
    c22 = _add(c22, prod(5))
    return [_add(c11, prod(6)), c12, c21, c22]


def _two_level(operands, block):
    halves = [[block(2 * r1 + r2, 2 * c1 + c2) for r2 in range(2) for c2 in range(2)]
              for r1 in range(2) for c1 in range(2)]
    return [t for outer in operands(*halves) for t in operands(*outer)]


def _two_level_out(prod):
    c = _strassen_out(lambda n: _strassen_out(lambda m: prod(7 * n + m)))
    return {(2 * (o // 2) + i // 2, 2 * (o % 2) + i % 2): c[o][i]
            for o in (2, 1, 3, 0) for i in (2, 1, 3, 0)}


def _kernel(c_ref, mem_ref, x_hbm, wq_hbm, wk_hbm, wv_hbm, wo_hbm, w1_hbm, w3_hbm, w2_hbm,
            wmod_hbm, out_hbm,
            wqkv, wo, aux, xs, attn, lhs, mod,
            sems, *, seg, n_seg, n_mem, n_head, d_model, d_ff):
    D, H, M = d_model, n_head, n_mem
    DT = D // LANE
    FT = d_ff // LANE
    L = M + seg
    CUR = seg - PRE
    PP = 2
    n_it = 3 * H // (2 * PP)
    it_per_mat = n_it // 3
    (S_XP, S_X, S_WO, S_FF, S_OUT, S_MOD, S_ST) = range(7)

    NP = n_seg * PRE
    TR = LANE // 2
    GM = (DT // 4) * (FT // 4)
    s0 = n_seg - 3 * GM
    PR = 3 * H * PRE
    item = 16 * TR + PR

    def raw_base(g):
        return aux.shape[0] - item * (3 * GM - g)

    def pre_base(s, late):
        return raw_base(s - s0) + 16 * TR if late else s * PR

    def wmod_rows(part, j):
        return aux_rows(s0 * PR + (part * 2 * DT + j) * (D // 2), D // 2)

    def aux_rows(start, size):
        return pl.ds(start if isinstance(start, int) else pl.multiple_of(start, 8), size)

    def lane_tile(j):
        return pl.ds(j * LANE if isinstance(j, int) else pl.multiple_of(j * LANE, LANE), LANE)

    def wmod_copy(part, j, sem=S_MOD):
        return pltpu.make_async_copy(
            wmod_hbm.bitcast(U32).at[:, lane_tile(part * 2 * DT + j)],
            aux.at[wmod_rows(part, j), :], sems.at[sem])

    def wo_copy(half, j):
        rows = pl.ds(half * (H // 2) * TR, (H // 2) * TR)
        return pltpu.make_async_copy(wo_hbm.bitcast(U32).at[rows, lane_tile(j)], wo.at[j, rows],
                                     sems.at[S_WO])

    x_copy = pltpu.make_async_copy(x_hbm, xs, sems.at[S_X])

    def ffn_copy(m, i, nq):
        per_row = DT // 4
        kk, j = (i % per_row, i // per_row) if m < 2 else (i // per_row, i % per_row)
        return pltpu.make_async_copy(
            (w1_hbm, w3_hbm, w2_hbm)[m].bitcast(U32).at[aux_rows(kk * 4 * TR, 4 * TR),
                                                        lane_tile(4 * j + nq)],
            aux.at[aux_rows(raw_base(m * GM + i) + nq * 4 * TR, 4 * TR), :], sems.at[S_FF])

    def prefetch_ffn(s, part):
        if part < 6:
            @pl.when(s < GM)
            def _():
                for nq in range(2):
                    ffn_copy(part // 2, s, 2 * (part % 2) + nq).start()
        elif part == 6:
            @pl.when(s < 2 * DT)
            def _():
                wmod_copy(1, s).start()
                wmod_copy(2, s).start()

    def start(cps):
        for cp in cps:
            cp.start()

    def wait(cps):
        for cp in cps:
            cp.wait()

    def modulation(part, tiles):
        sc = jnp.broadcast_to(_silu(c_ref[...].astype(F32)), (8, D))
        for j in tiles:
            r = _dot(sc, _w(aux[wmod_rows(part, j), :]))
            mod[2 * part + j // DT, :, pl.ds((j % DT) * LANE, LANE)] = r

    def modrow(i):
        return mod[i, 0:1, :]

    def prologue(ring, xp, hp):
        def pair_copies(w_hbm, i):
            src = w_hbm.bitcast(U32)
            return [pltpu.make_async_copy(
                src.at[:, (i % it_per_mat) * PP + t + par * (H // 2), :],
                ring.at[i % RING, 2 * t + par], sems.at[S_ST + i % RING])
                for t in range(PP) for par in range(2)]

        xp_copy = pltpu.make_async_copy(x_hbm.at[:, pl.ds(CUR, PRE), :], xp, sems.at[S_XP])
        xp_copy.start()
        tiles = [range(t, 2 * DT, 2) for t in range(2)]
        halves = [[wmod_copy(0, j, sem) for j in tiles[t]] for t, sem in enumerate((S_MOD, S_FF))]
        start(halves[0])
        xp_copy.wait()
        start(halves[1])
        xn = _layernorm(xp[...].astype(F32).reshape(NP, D))
        for t in range(2):
            wait(halves[t])
            for i in range(t, AHEAD if t else 1):
                start(pair_copies(wq_hbm, i))
            modulation(0, tiles[t])
            for u in range(t, DT // 4, 2):
                def block(rq, kq):
                    cols = slice((kq * (DT // 4) + u) * LANE, (kq * (DT // 4) + u + 1) * LANE)
                    return (xn[rq * (NP // 4):(rq + 1) * (NP // 4), cols]
                            * (1.0 + mod[1, 0:1, cols]) + mod[0, 0:1, cols])

                for n, a in enumerate(_two_level(_strassen_lhs, block)):
                    hp[n, :, lane_tile(u)] = a.astype(BF16)

        def pro_body(w_next, wo_half, i, carry):
            wait(pair_copies(wq_hbm, i))
            heads = []
            for t in range(PP):
                a = ring[i % RING, 2 * t]
                b = ring[i % RING, 2 * t + 1]
                heads += [(a & jnp.uint32(0xFFFF)) | (b << 16),
                          (a >> 16) | (b & jnp.uint32(0xFFFF0000))]
            for n, w in enumerate(heads):
                wqkv[i * 2 * PP + n] = w
            if w_next is not None:
                start(pair_copies(w_next, i + AHEAD))
            if wo_half is not None:
                wo_copy(wo_half, (i + AHEAD) % it_per_mat).start()
            rhs = _two_level(_strassen_rhs, lambda kq, nq: _w(
                heads[nq][kq * (D // 8):(kq + 1) * (D // 8)]).astype(F32))
            c = _two_level_out(lambda n: _dot(hp[n], rhs[n].astype(BF16)))
            for (rq, nq), val in c.items():
                for j in range(n_seg // 4):
                    sg = rq * (n_seg // 4) + j
                    r0 = pre_base(sg, sg >= s0) + (i * 2 * PP + nq) * PRE
                    aux[aux_rows(r0, PRE), :] = pltpu.bitcast(val[j * PRE:(j + 1) * PRE], U32)
            return carry

        for m, (w_hbm, wo_half) in enumerate(((wq_hbm, None), (wk_hbm, 0), (wv_hbm, 1))):
            lax.fori_loop(max(m * it_per_mat - AHEAD, 0), (m + 1) * it_per_mat - AHEAD,
                          functools.partial(pro_body, w_hbm, wo_half), 0)
        x_copy.start()
        lax.fori_loop(n_it - AHEAD, n_it, functools.partial(pro_body, None, None), 0)

    pl.run_scoped(prologue, pltpu.VMEM((RING, 2 * PP, D // 2, LANE), U32),
                  pltpu.VMEM((n_seg, PRE, D), BF16), pltpu.VMEM((49, NP // 4, D // 4), BF16))
    wait([wo_copy(half, j) for half in range(2) for j in range(DT)])
    x_copy.wait()

    def seg_rows(s):
        xn = _layernorm(xs[s].astype(F32)[0:CUR])
        return xn * (1.0 + modrow(1)) + modrow(0)

    lhs[...] = jnp.concatenate([mem_ref[...].astype(F32), seg_rows(0)], axis=0).astype(BF16)
    scale = float(LANE) ** -0.5
    NG = H // HG

    def chain_body(combine, s, carry):
        row = lax.broadcasted_iota(jnp.int32, (L, L), 0)
        col = lax.broadcasted_iota(jnp.int32, (L, L), 1)
        mask = (row < M) | (row >= col)
        q, k, v, p, ov = {}, {}, {}, {}, {}

        def heads(g):
            return range(g * HG, (g + 1) * HG)

        def proj(m, h):
            done = aux[aux_rows(pre_base(s, combine) + (m * H + h) * PRE, PRE), :]
            return jnp.concatenate([_dot(lhs[...], _w(wqkv[m * H + h])),
                                    pltpu.bitcast(done, F32)], axis=0)

        def probs(g):
            for h in heads(g):
                z = jnp.where(mask, _dot_nt(q[h], k[h]) * scale, -1e9)
                e = jnp.exp(z - jnp.max(z, axis=-1, keepdims=True))
                p[h] = e * pl.reciprocal(jnp.sum(e, axis=-1, keepdims=True), full_range=False)

        def values(g):
            for h in heads(g):
                ov[h] = _dot(p[h], v[h])

        def out_proj(h0, h1, marks):
            o = jnp.concatenate([ov[h] for h in range(h0, h1)], axis=1)
            cols = []
            for j in range(DT):
                cols.append(_dot(o, _w(wo[j, pl.ds(h0 * TR, (h1 - h0) * TR), :])))
                if combine and j in marks:
                    aux[aux_rows(pre_base(s, True), 8), :] = pltpu.bitcast(cols[-1][0:8], U32)
                    combine_weights(marks[j], CW[3])
            return jnp.concatenate(cols, axis=1)

        def combine_weights(g, outer):
            for r in range(g * TR // NG // 8 * 8, (g + 1) * TR // NG // 8 * 8, 8) if combine else ():
                def block(kq, nq):
                    rows = aux_rows(raw_base(s - s0) + (nq * 4 + kq) * TR + r, 8)
                    return _w(aux[rows, :]).astype(F32)

                for n, t in enumerate(_two_level(_strassen_rhs, block)):
                    if n // 7 in outer:
                        rows = aux_rows(((s - s0) * 49 + n) * TR + r, 8)
                        aux[rows, :] = pltpu.bitcast(t.astype(BF16), U32)

        for g in range(NG):
            combine_weights(g, CW[0])
            for h in heads(g):
                k[h] = proj(1, h).astype(BF16)
            combine_weights(g, CW[1])
            for h in heads(g):
                q[h] = proj(0, h)
            if g >= 1:
                probs(g - 1)
            if not combine:
                prefetch_ffn(s, g)
        for g in range(NG):
            combine_weights(g, CW[2])
            for h in heads(g):
                v[h] = proj(2, h).astype(BF16)
            if g == 0:
                probs(NG - 1)
            else:
                values(g - 1)
        nxt = seg_rows(jnp.minimum(s + 1, n_seg - 1))
        o = out_proj(0, SPLIT, {DT // 2 - 1: 0, DT - 1: 1})
        values(NG - 1)
        o = o + out_proj(SPLIT, H, {j: j + 2 for j in range(NG - 2)})
        attn[s] = o[M:].astype(BF16)
        lhs[...] = jnp.concatenate([o[:M], nxt], axis=0).astype(BF16)
        return carry

    lax.fori_loop(0, s0, functools.partial(chain_body, False), 0)
    wait([ffn_copy(m, i, nq) for m in range(3) for i in range(GM) for nq in range(4)])
    wait([wmod_copy(part, j) for part in (1, 2) for j in range(2 * DT)])
    modulation(1, range(2 * DT))
    modulation(2, range(2 * DT))
    lax.fori_loop(s0, n_seg, functools.partial(chain_body, True), 0)

    SB = 4
    n_blk = n_seg // SB

    def resid(sg, rows=slice(None), cols=slice(None)):
        return (xs[sg, rows, cols].astype(F32)
                + mod[2, 0:1, cols] * attn[sg, rows, cols].astype(F32))

    def ffn(act, upin, hbuf):
        KT = DT // 4

        def norm_steps(i, zero):
            def center(sg, rows):
                x1 = resid(i * SB + sg, rows=rows)
                hbuf[sg + zero, rows] = x1 - jnp.mean(x1, axis=-1, keepdims=True)

            def normalize(sg, rows):
                d = hbuf[sg, rows]
                rstd = lax.rsqrt(jnp.mean(d * d, axis=-1, keepdims=True) + EPS)
                hbuf[sg + zero, rows] = d * rstd * (1.0 + modrow(4)) + modrow(3)

            return [functools.partial(f, sg, slice(r, r + LN_ROWS)) for sg in range(SB)
                    for r in range(0, seg, LN_ROWS) for f in (center, normalize)]

        def operand_steps(zero):
            def operands(outer, t):
                ops = _two_level(_strassen_lhs,
                                 lambda rq, kq: hbuf[rq, :, lane_tile(4 * t + kq)])
                for n in range(7 * outer, 7 * outer + 7):
                    upin[n + zero, :, pl.ds(t * LANE, LANE)] = ops[n]

            return [functools.partial(operands, n, t) for n in range(7) for t in range(KT)]

        def products(a_ref, n_calls, first, steps, zero):
            calls = iter(range(n_calls))
            when = {first + k * (n_calls - first) // len(steps): f for k, f in enumerate(steps)}
            assert len(when) == len(steps)

            def product(granules, n):
                w = jnp.concatenate([aux[pl.ds((g * 49 + n) * TR, TR), :] for g in granules],
                                    axis=0)
                r = _dot(a_ref[n], _w(w))
                step = when.get(next(calls))
                if step is not None:
                    hbuf[SB + zero, 0:8, 0:LANE] = r[0:8]
                    step()
                return r

            return product

        for step in norm_steps(0, 0) + operand_steps(0):
            step()

        def ffn_body(i, carry):
            zero = i // n_blk
            product = products(upin, 2 * 49 * (FT // 4), FIRST[0],
                               norm_steps(jnp.minimum(i + 1, n_blk - 1), zero), zero)
            for j in range(FT // 4):
                gate, up = (_two_level_out(functools.partial(
                    product, range(m * GM + j * KT, m * GM + (j + 1) * KT))) for m in range(2))
                hidden = {rc: _silu(gate[rc]) * up[rc] for rc in gate}
                for n, t in enumerate(_two_level(_strassen_lhs, lambda r, c: hidden[r, c])):
                    act[n, :, lane_tile(j)] = t
            product = products(act, 49 * KT, FIRST[1], operand_steps(zero), zero)
            for j in range(KT):
                c = _two_level_out(functools.partial(product, range(2 * GM + j, 3 * GM, KT)))
                for (rq, nq), t in c.items():
                    cols = slice((4 * j + nq) * LANE, (4 * j + nq + 1) * LANE)
                    y = resid(i * SB + rq, cols=cols) + mod[5, 0:1, cols] * t
                    attn[i * SB + rq, :, cols] = y.astype(BF16)
            sl = pl.ds(i * SB, SB)
            pltpu.make_async_copy(attn.at[sl], out_hbm.at[sl], sems.at[S_OUT]).start()
            return carry

        lax.fori_loop(0, n_blk, ffn_body, 0)

    pl.run_scoped(ffn, pltpu.VMEM((49, seg, d_ff // 4), F32),
                  pltpu.VMEM((49, seg, D // 4), F32), pltpu.VMEM((SB + 1, seg, D), F32))
    pltpu.make_async_copy(attn, out_hbm, sems.at[S_OUT]).wait()


@functools.partial(jax.jit, static_argnames=("A_seg_len",))
def pallas_adaLN_cond__memory_aug_recurrent_mem_tr__glu_gated_swiglu__prompt_kernel(
    A_x, A_mem0, A_Wq, A_Wk, A_Wv, A_Wo, A_seg_len, B_x, B_w1, B_w3, B_w2, c, w_mod,
):
    del B_x
    B, S, D = A_x.shape
    _, H, Dh = A_Wq.shape
    M = A_mem0.shape[1]
    F = B_w1.shape[1]
    seg = int(A_seg_len)
    n_seg = S // seg
    n_gran = 3 * (D // (4 * LANE)) * (F // (4 * LANE))
    assert B == 1 and Dh == LANE and S % seg == 0 and n_seg % 4 == 0 and F % (4 * LANE) == 0
    assert max(n_gran // 3, 2 * D // LANE) <= n_seg - n_gran and AHEAD < RING
    assert H // 4 == D // LANE == H // HG == 8 and M == PRE == 8
    kern = functools.partial(_kernel, seg=seg, n_seg=n_seg, n_mem=M, n_head=H, d_model=D, d_ff=F)
    hbm = pl.BlockSpec(memory_space=pl.ANY)
    vmem = pl.BlockSpec(memory_space=pltpu.VMEM)
    out = pl.pallas_call(
        kern,
        out_shape=jax.ShapeDtypeStruct((n_seg, seg, D), A_x.dtype),
        in_specs=[vmem, vmem] + [hbm] * 9,
        out_specs=hbm,
        scratch_shapes=[
            pltpu.VMEM((3 * H, D // 2, LANE), U32),
            pltpu.VMEM((D // LANE, H * Dh // 2, LANE), U32),
            pltpu.VMEM(((49 * n_gran + 16) * LANE // 2 + 3 * H * PRE, LANE), U32),
            pltpu.VMEM((n_seg, seg, D), BF16),
            pltpu.VMEM((n_seg, seg, D), BF16),
            pltpu.VMEM((M + seg - PRE, D), BF16),
            pltpu.VMEM((6, 8, D), F32),
            pltpu.SemaphoreType.DMA((6 + RING,)),
        ],
        compiler_params=pltpu.CompilerParams(vmem_limit_bytes=127 * 1024 * 1024,
                                             disable_bounds_checks=True),
    )(c, A_mem0.reshape(M, D), A_x.reshape(n_seg, seg, D),
      A_Wq.reshape(D // 2, 2 * H, Dh), A_Wk.reshape(D // 2, 2 * H, Dh),
      A_Wv.reshape(D // 2, 2 * H, Dh),
      A_Wo.reshape(H * Dh, D), B_w1, B_w3, B_w2, w_mod)
    return out.reshape(B, S, D)
```

```python
import functools

import jax
import jax.numpy as jnp
from jax import lax
import jax.experimental.pallas as pl
import jax.experimental.pallas.tpu as pltpu

F32 = jnp.float32
BF16 = jnp.bfloat16
U32 = jnp.uint32
LANE = 128
EPS = 1e-5
PRE = 8
HG = 4
SPLIT = 8
AHEAD = 3
RING = 4
CW = ((2, 5), (3, 6), (0, 4), (1,))
FIRST = (60, 56)
LN_ROWS = 16


def _layernorm(x):
    m = jnp.mean(x, axis=-1, keepdims=True)
    d = x - m
    v = jnp.mean(d * d, axis=-1, keepdims=True)
    return d * lax.rsqrt(v + EPS)


def _silu(x):
    h = 0.5 * x
    return h + h * jnp.tanh(h)


def _w(tile_u32):
    return pltpu.bitcast(tile_u32, BF16)


def _dot(a, b):
    return lax.dot_general(a, b, (((1,), (0,)), ((), ())), preferred_element_type=F32)


def _dot_nt(a, b):
    return lax.dot_general(a, b, (((1,), (1,)), ((), ())), preferred_element_type=F32)


def _add(a, b):
    return jax.tree.map(jnp.add, a, b)


def _sub(a, b):
    return jax.tree.map(jnp.subtract, a, b)


def _strassen_lhs(a11, a12, a21, a22):
    return [_add(a11, a22), _add(a21, a22), a11, a22, _add(a11, a12), _sub(a21, a11),
            _sub(a12, a22)]


def _strassen_rhs(b11, b12, b21, b22):
    return [_add(b11, b22), b11, _sub(b12, b22), _sub(b21, b11), b22, _add(b11, b12),
            _add(b21, b22)]


def _strassen_out(prod):
    m1, m3 = prod(1), prod(3)
    c21 = _add(m1, m3)
    m4 = prod(4)
    c11 = _sub(m3, m4)
    m2 = prod(2)
    c12 = _add(m2, m4)
    c22 = _sub(m2, m1)
    m0 = prod(0)
    c11, c22 = _add(c11, m0), _add(c22, m0)
    c22 = _add(c22, prod(5))
    return [_add(c11, prod(6)), c12, c21, c22]


def _two_level(operands, block):
    halves = [[block(2 * r1 + r2, 2 * c1 + c2) for r2 in range(2) for c2 in range(2)]
              for r1 in range(2) for c1 in range(2)]
    return [t for outer in operands(*halves) for t in operands(*outer)]


def _two_level_out(prod):
    c = _strassen_out(lambda n: _strassen_out(lambda m: prod(7 * n + m)))
    return {(2 * (o // 2) + i // 2, 2 * (o % 2) + i % 2): c[o][i]
            for o in (2, 1, 3, 0) for i in (2, 1, 3, 0)}


def _kernel(c_ref, mem_ref, x_hbm, wq_hbm, wk_hbm, wv_hbm, wo_hbm, w1_hbm, w3_hbm, w2_hbm,
            wmod_hbm, out_hbm,
            wqkv, wo, aux, xs, attn, lhs, mod,
            sems, *, seg, n_seg, n_mem, n_head, d_model, d_ff):
    D, H, M = d_model, n_head, n_mem
    DT = D // LANE
    FT = d_ff // LANE
    L = M + seg
    CUR = seg - PRE
    PP = 2
    n_it = 3 * H // (2 * PP)
    it_per_mat = n_it // 3
    (S_XP, S_X, S_WO, S_FF, S_OUT, S_MOD, S_ST) = range(7)

    NP = n_seg * PRE
    TR = LANE // 2
    GM = (DT // 4) * (FT // 4)
    s0 = n_seg - 3 * GM
    PR = 3 * H * PRE
    item = 16 * TR + PR

    def raw_base(g):
        return aux.shape[0] - item * (3 * GM - g)

    def pre_base(s, late):
        return raw_base(s - s0) + 16 * TR if late else s * PR

    def wmod_rows(part, j):
        return aux_rows(s0 * PR + (part * 2 * DT + j) * (D // 2), D // 2)

    def aux_rows(start, size):
        return pl.ds(start if isinstance(start, int) else pl.multiple_of(start, 8), size)

    def lane_tile(j):
        return pl.ds(j * LANE if isinstance(j, int) else pl.multiple_of(j * LANE, LANE), LANE)

    def wmod_copy(part, j, sem=S_MOD):
        return pltpu.make_async_copy(
            wmod_hbm.bitcast(U32).at[:, lane_tile(part * 2 * DT + j)],
            aux.at[wmod_rows(part, j), :], sems.at[sem])

    def wo_copy(half, j):
        rows = pl.ds(half * (H // 2) * TR, (H // 2) * TR)
        return pltpu.make_async_copy(wo_hbm.bitcast(U32).at[rows, lane_tile(j)], wo.at[j, rows],
                                     sems.at[S_WO])

    x_copy = pltpu.make_async_copy(x_hbm, xs, sems.at[S_X])

    def ffn_copy(m, i, nq):
        per_row = DT // 4
        kk, j = (i % per_row, i // per_row) if m < 2 else (i // per_row, i % per_row)
        return pltpu.make_async_copy(
            (w1_hbm, w3_hbm, w2_hbm)[m].bitcast(U32).at[aux_rows(kk * 4 * TR, 4 * TR),
                                                        lane_tile(4 * j + nq)],
            aux.at[aux_rows(raw_base(m * GM + i) + nq * 4 * TR, 4 * TR), :], sems.at[S_FF])

    def prefetch_ffn(s, part):
        if part < 6:
            @pl.when(s < GM)
            def _():
                for nq in range(2):
                    ffn_copy(part // 2, s, 2 * (part % 2) + nq).start()
        elif part == 6:
            @pl.when(s < 2 * DT)
            def _():
                wmod_copy(1, s).start()
                wmod_copy(2, s).start()

    def start(cps):
        for cp in cps:
            cp.start()

    def wait(cps):
        for cp in cps:
            cp.wait()

    def modulation(part, tiles):
        sc = jnp.broadcast_to(_silu(c_ref[...].astype(F32)), (8, D))
        for j in tiles:
            r = _dot(sc, _w(aux[wmod_rows(part, j), :]))
            mod[2 * part + j // DT, :, pl.ds((j % DT) * LANE, LANE)] = r

    def modrow(i):
        return mod[i, 0:1, :]

    def prologue(ring, xp, hp):
        def pair_copies(w_hbm, i):
            src = w_hbm.bitcast(U32)
            return [pltpu.make_async_copy(
                src.at[:, (i % it_per_mat) * PP + t + par * (H // 2), :],
                ring.at[i % RING, 2 * t + par], sems.at[S_ST + i % RING])
                for t in range(PP) for par in range(2)]

        xp_copy = pltpu.make_async_copy(x_hbm.at[:, pl.ds(CUR, PRE), :], xp, sems.at[S_XP])
        xp_copy.start()
        tiles = [range(t, 2 * DT, 2) for t in range(2)]
        halves = [[wmod_copy(0, j, sem) for j in tiles[t]] for t, sem in enumerate((S_MOD, S_FF))]
        start(halves[0])
        xp_copy.wait()
        start(halves[1])
        xn = _layernorm(xp[...].astype(F32).reshape(NP, D))
        for t in range(2):
            wait(halves[t])
            for i in range(t, AHEAD if t else 1):
                start(pair_copies(wq_hbm, i))
            modulation(0, tiles[t])
            for u in range(t, DT // 4, 2):
                def block(rq, kq):
                    cols = slice((kq * (DT // 4) + u) * LANE, (kq * (DT // 4) + u + 1) * LANE)
                    return (xn[rq * (NP // 4):(rq + 1) * (NP // 4), cols]
                            * (1.0 + mod[1, 0:1, cols]) + mod[0, 0:1, cols])

                for n, a in enumerate(_two_level(_strassen_lhs, block)):
                    hp[n, :, lane_tile(u)] = a.astype(BF16)

        def pro_body(i, carry):
            wait(pair_copies(wq_hbm, i))
            heads = []
            for t in range(PP):
                a = ring[i % RING, 2 * t]
                b = ring[i % RING, 2 * t + 1]
                heads += [(a & jnp.uint32(0xFFFF)) | (b << 16),
                          (a >> 16) | (b & jnp.uint32(0xFFFF0000))]
            for n, w in enumerate(heads):
                wqkv[i * 2 * PP + n] = w
            nxt = i + AHEAD
            for m, w_hbm in enumerate((wq_hbm, wk_hbm, wv_hbm)):
                @pl.when((nxt >= m * it_per_mat) & (nxt < (m + 1) * it_per_mat))
                def _():
                    start(pair_copies(w_hbm, nxt))
                    if m > 0:
                        wo_copy(m - 1, nxt - m * it_per_mat).start()

            @pl.when(nxt == n_it)
            def _():
                x_copy.start()

            rhs = _two_level(_strassen_rhs, lambda kq, nq: _w(
                heads[nq][kq * (D // 8):(kq + 1) * (D // 8)]).astype(F32))
            c = _two_level_out(lambda n: _dot(hp[n], rhs[n].astype(BF16)))
            for (rq, nq), val in c.items():
                for j in range(n_seg // 4):
                    sg = rq * (n_seg // 4) + j
                    r0 = pre_base(sg, sg >= s0) + (i * 2 * PP + nq) * PRE
                    aux[aux_rows(r0, PRE), :] = pltpu.bitcast(val[j * PRE:(j + 1) * PRE], U32)
            return carry

        lax.fori_loop(0, n_it, pro_body, 0)

    pl.run_scoped(prologue, pltpu.VMEM((RING, 2 * PP, D // 2, LANE), U32),
                  pltpu.VMEM((n_seg, PRE, D), BF16), pltpu.VMEM((49, NP // 4, D // 4), BF16))
    wait([wo_copy(half, j) for half in range(2) for j in range(DT)])
    x_copy.wait()

    def seg_rows(s):
        xn = _layernorm(xs[s].astype(F32)[0:CUR])
        return xn * (1.0 + modrow(1)) + modrow(0)

    lhs[...] = jnp.concatenate([mem_ref[...].astype(F32), seg_rows(0)], axis=0).astype(BF16)
    scale = float(LANE) ** -0.5
    NG = H // HG

    def chain_body(combine, s, carry):
        row = lax.broadcasted_iota(jnp.int32, (L, L), 0)
        col = lax.broadcasted_iota(jnp.int32, (L, L), 1)
        mask = (row < M) | (row >= col)
        q, k, v, p, ov = {}, {}, {}, {}, {}

        def heads(g):
            return range(g * HG, (g + 1) * HG)

        def proj(m, h):
            done = aux[aux_rows(pre_base(s, combine) + (m * H + h) * PRE, PRE), :]
            return jnp.concatenate([_dot(lhs[...], _w(wqkv[m * H + h])),
                                    pltpu.bitcast(done, F32)], axis=0)

        def probs(g):
            for h in heads(g):
                z = jnp.where(mask, _dot_nt(q[h], k[h]) * scale, -1e9)
                e = jnp.exp(z - jnp.max(z, axis=-1, keepdims=True))
                p[h] = e * pl.reciprocal(jnp.sum(e, axis=-1, keepdims=True), full_range=False)

        def values(g):
            for h in heads(g):
                ov[h] = _dot(p[h], v[h])

        def out_proj(h0, h1, marks):
            o = jnp.concatenate([ov[h] for h in range(h0, h1)], axis=1)
            cols = []
            for j in range(DT):
                cols.append(_dot(o, _w(wo[j, pl.ds(h0 * TR, (h1 - h0) * TR), :])))
                if combine and j in marks:
                    aux[aux_rows(pre_base(s, True), 8), :] = pltpu.bitcast(cols[-1][0:8], U32)
                    combine_weights(marks[j], CW[3])
            return jnp.concatenate(cols, axis=1)

        def combine_weights(g, outer):
            for r in range(g * TR // NG // 8 * 8, (g + 1) * TR // NG // 8 * 8, 8) if combine else ():
                def block(kq, nq):
                    rows = aux_rows(raw_base(s - s0) + (nq * 4 + kq) * TR + r, 8)
                    return _w(aux[rows, :]).astype(F32)

                for n, t in enumerate(_two_level(_strassen_rhs, block)):
                    if n // 7 in outer:
                        rows = aux_rows(((s - s0) * 49 + n) * TR + r, 8)
                        aux[rows, :] = pltpu.bitcast(t.astype(BF16), U32)

        for g in range(NG):
            combine_weights(g, CW[0])
            for h in heads(g):
                k[h] = proj(1, h).astype(BF16)
            combine_weights(g, CW[1])
            for h in heads(g):
                q[h] = proj(0, h)
            if g >= 1:
                probs(g - 1)
            if not combine:
                prefetch_ffn(s, g)
        for g in range(NG):
            combine_weights(g, CW[2])
            for h in heads(g):
                v[h] = proj(2, h).astype(BF16)
            if g == 0:
                probs(NG - 1)
            else:
                values(g - 1)
        nxt = seg_rows(jnp.minimum(s + 1, n_seg - 1))
        o = out_proj(0, SPLIT, {DT // 2 - 1: 0, DT - 1: 1})
        values(NG - 1)
        o = o + out_proj(SPLIT, H, {j: j + 2 for j in range(NG - 2)})
        attn[s] = o[M:].astype(BF16)
        lhs[...] = jnp.concatenate([o[:M], nxt], axis=0).astype(BF16)
        return carry

    lax.fori_loop(0, s0, functools.partial(chain_body, False), 0)
    wait([ffn_copy(m, i, nq) for m in range(3) for i in range(GM) for nq in range(4)])
    wait([wmod_copy(part, j) for part in (1, 2) for j in range(2 * DT)])
    modulation(1, range(2 * DT))
    modulation(2, range(2 * DT))
    lax.fori_loop(s0, n_seg, functools.partial(chain_body, True), 0)

    SB = 4
    n_blk = n_seg // SB

    def resid(sg, rows=slice(None), cols=slice(None)):
        return (xs[sg, rows, cols].astype(F32)
                + mod[2, 0:1, cols] * attn[sg, rows, cols].astype(F32))

    def ffn(act, upin, hbuf):
        KT = DT // 4

        def norm_steps(i, zero):
            def center(sg, rows):
                x1 = resid(i * SB + sg, rows=rows)
                hbuf[sg + zero, rows] = x1 - jnp.mean(x1, axis=-1, keepdims=True)

            def normalize(sg, rows):
                d = hbuf[sg, rows]
                rstd = lax.rsqrt(jnp.mean(d * d, axis=-1, keepdims=True) + EPS)
                hbuf[sg + zero, rows] = d * rstd * (1.0 + modrow(4)) + modrow(3)

            return [functools.partial(f, sg, slice(r, r + LN_ROWS)) for sg in range(SB)
                    for r in range(0, seg, LN_ROWS) for f in (center, normalize)]

        def operand_steps(zero):
            def operands(outer, t):
                ops = _two_level(_strassen_lhs,
                                 lambda rq, kq: hbuf[rq, :, lane_tile(4 * t + kq)])
                for n in range(7 * outer, 7 * outer + 7):
                    upin[n + zero, :, pl.ds(t * LANE, LANE)] = ops[n]

            return [functools.partial(operands, n, t) for n in range(7) for t in range(KT)]

        def products(a_ref, n_calls, first, steps, zero):
            calls = iter(range(n_calls))
            when = {first + k * (n_calls - first) // len(steps): f for k, f in enumerate(steps)}
            assert len(when) == len(steps)

            def product(granules, n):
                w = jnp.concatenate([aux[pl.ds((g * 49 + n) * TR, TR), :] for g in granules],
                                    axis=0)
                r = _dot(a_ref[n], _w(w))
                step = when.get(next(calls))
                if step is not None:
                    hbuf[SB + zero, 0:8, 0:LANE] = r[0:8]
                    step()
                return r

            return product

        for step in norm_steps(0, 0) + operand_steps(0):
            step()

        def ffn_body(i, carry):
            zero = i // n_blk
            product = products(upin, 2 * 49 * (FT // 4), FIRST[0],
                               norm_steps(jnp.minimum(i + 1, n_blk - 1), zero), zero)
            for j in range(FT // 4):
                gate, up = (_two_level_out(functools.partial(
                    product, range(m * GM + j * KT, m * GM + (j + 1) * KT))) for m in range(2))
                hidden = {rc: _silu(gate[rc]) * up[rc] for rc in gate}
                for n, t in enumerate(_two_level(_strassen_lhs, lambda r, c: hidden[r, c])):
                    act[n, :, lane_tile(j)] = t
            product = products(act, 49 * KT, FIRST[1], operand_steps(zero), zero)
            for j in range(KT):
                c = _two_level_out(functools.partial(product, range(2 * GM + j, 3 * GM, KT)))
                for (rq, nq), t in c.items():
                    cols = slice((4 * j + nq) * LANE, (4 * j + nq + 1) * LANE)
                    y = resid(i * SB + rq, cols=cols) + mod[5, 0:1, cols] * t
                    attn[i * SB + rq, :, cols] = y.astype(BF16)
            sl = pl.ds(i * SB, SB)
            pltpu.make_async_copy(attn.at[sl], out_hbm.at[sl], sems.at[S_OUT]).start()
            return carry

        lax.fori_loop(0, n_blk, ffn_body, 0)

    pl.run_scoped(ffn, pltpu.VMEM((49, seg, d_ff // 4), F32),
                  pltpu.VMEM((49, seg, D // 4), F32), pltpu.VMEM((SB + 1, seg, D), F32))
    pltpu.make_async_copy(attn, out_hbm, sems.at[S_OUT]).wait()


@functools.partial(jax.jit, static_argnames=("A_seg_len",))
def pallas_adaLN_cond__memory_aug_recurrent_mem_tr__glu_gated_swiglu__prompt_kernel(
    A_x, A_mem0, A_Wq, A_Wk, A_Wv, A_Wo, A_seg_len, B_x, B_w1, B_w3, B_w2, c, w_mod,
):
    del B_x
    B, S, D = A_x.shape
    _, H, Dh = A_Wq.shape
    M = A_mem0.shape[1]
    F = B_w1.shape[1]
    seg = int(A_seg_len)
    n_seg = S // seg
    n_gran = 3 * (D // (4 * LANE)) * (F // (4 * LANE))
    assert B == 1 and Dh == LANE and S % seg == 0 and n_seg % 4 == 0 and F % (4 * LANE) == 0
    assert max(n_gran // 3, 2 * D // LANE) <= n_seg - n_gran and AHEAD < RING
    assert H // 4 == D // LANE == H // HG == 8 and M == PRE == 8
    kern = functools.partial(_kernel, seg=seg, n_seg=n_seg, n_mem=M, n_head=H, d_model=D, d_ff=F)
    hbm = pl.BlockSpec(memory_space=pl.ANY)
    vmem = pl.BlockSpec(memory_space=pltpu.VMEM)
    out = pl.pallas_call(
        kern,
        out_shape=jax.ShapeDtypeStruct((n_seg, seg, D), A_x.dtype),
        in_specs=[vmem, vmem] + [hbm] * 9,
        out_specs=hbm,
        scratch_shapes=[
            pltpu.VMEM((3 * H, D // 2, LANE), U32),
            pltpu.VMEM((D // LANE, H * Dh // 2, LANE), U32),
            pltpu.VMEM(((49 * n_gran + 16) * LANE // 2 + 3 * H * PRE, LANE), U32),
            pltpu.VMEM((n_seg, seg, D), BF16),
            pltpu.VMEM((n_seg, seg, D), BF16),
            pltpu.VMEM((M + seg - PRE, D), BF16),
            pltpu.VMEM((6, 8, D), F32),
            pltpu.SemaphoreType.DMA((6 + RING,)),
        ],
        compiler_params=pltpu.CompilerParams(vmem_limit_bytes=127 * 1024 * 1024,
                                             disable_bounds_checks=True),
    )(c, A_mem0.reshape(M, D), A_x.reshape(n_seg, seg, D),
      A_Wq.reshape(D // 2, 2 * H, Dh), A_Wk.reshape(D // 2, 2 * H, Dh),
      A_Wv.reshape(D // 2, 2 * H, Dh),
      A_Wo.reshape(H * Dh, D), B_w1, B_w3, B_w2, w_mod)
    return out.reshape(B, S, D)
```

```python
import functools

import jax
import jax.numpy as jnp
from jax import lax
import jax.experimental.pallas as pl
import jax.experimental.pallas.tpu as pltpu

F32 = jnp.float32
BF16 = jnp.bfloat16
U32 = jnp.uint32
LANE = 128
EPS = 1e-5
PRE = 8
HG = 4
SPLIT = 8
AHEAD = 3
RING = 4
CW = ((2, 5), (3, 6), (0, 4), (1,))
FIRST = (60, 14)
LN_ROWS = 8


def _layernorm(x):
    m = jnp.mean(x, axis=-1, keepdims=True)
    d = x - m
    v = jnp.mean(d * d, axis=-1, keepdims=True)
    return d * lax.rsqrt(v + EPS)


def _silu(x):
    h = 0.5 * x
    return h + h * jnp.tanh(h)


def _w(tile_u32):
    return pltpu.bitcast(tile_u32, BF16)


def _dot(a, b):
    return lax.dot_general(a, b, (((1,), (0,)), ((), ())), preferred_element_type=F32)


def _dot_nt(a, b):
    return lax.dot_general(a, b, (((1,), (1,)), ((), ())), preferred_element_type=F32)


def _add(a, b):
    return jax.tree.map(jnp.add, a, b)


def _sub(a, b):
    return jax.tree.map(jnp.subtract, a, b)


def _strassen_lhs(a11, a12, a21, a22):
    return [_add(a11, a22), _add(a21, a22), a11, a22, _add(a11, a12), _sub(a21, a11),
            _sub(a12, a22)]


def _strassen_rhs(b11, b12, b21, b22):
    return [_add(b11, b22), b11, _sub(b12, b22), _sub(b21, b11), b22, _add(b11, b12),
            _add(b21, b22)]


def _strassen_out(prod):
    m1, m3 = prod(1), prod(3)
    c21 = _add(m1, m3)
    m4 = prod(4)
    c11 = _sub(m3, m4)
    m2 = prod(2)
    c12 = _add(m2, m4)
    c22 = _sub(m2, m1)
    m0 = prod(0)
    c11, c22 = _add(c11, m0), _add(c22, m0)
    c22 = _add(c22, prod(5))
    return [_add(c11, prod(6)), c12, c21, c22]


def _two_level(operands, block):
    halves = [[block(2 * r1 + r2, 2 * c1 + c2) for r2 in range(2) for c2 in range(2)]
              for r1 in range(2) for c1 in range(2)]
    return [t for outer in operands(*halves) for t in operands(*outer)]


def _two_level_out(prod):
    c = _strassen_out(lambda n: _strassen_out(lambda m: prod(7 * n + m)))
    return {(2 * (o // 2) + i // 2, 2 * (o % 2) + i % 2): c[o][i]
            for o in (2, 1, 3, 0) for i in (2, 1, 3, 0)}


def _kernel(c_ref, mem_ref, x_hbm, wq_hbm, wk_hbm, wv_hbm, wo_hbm, w1_hbm, w3_hbm, w2_hbm,
            wmod_hbm, out_hbm,
            wqkv, wo, aux, xs, attn, lhs, mod,
            sems, *, seg, n_seg, n_mem, n_head, d_model, d_ff):
    D, H, M = d_model, n_head, n_mem
    DT = D // LANE
    FT = d_ff // LANE
    L = M + seg
    CUR = seg - PRE
    PP = 2
    n_it = 3 * H // (2 * PP)
    it_per_mat = n_it // 3
    (S_XP, S_X, S_WO, S_FF, S_OUT, S_MOD, S_ST) = range(7)

    NP = n_seg * PRE
    TR = LANE // 2
    GM = (DT // 4) * (FT // 4)
    s0 = n_seg - 3 * GM
    PR = 3 * H * PRE
    item = 16 * TR + PR

    def raw_base(g):
        return aux.shape[0] - item * (3 * GM - g)

    def pre_base(s, late):
        return raw_base(s - s0) + 16 * TR if late else s * PR

    def wmod_rows(part, j):
        return aux_rows(s0 * PR + (part * 2 * DT + j) * (D // 2), D // 2)

    def aux_rows(start, size):
        return pl.ds(start if isinstance(start, int) else pl.multiple_of(start, 8), size)

    def lane_tile(j):
        return pl.ds(j * LANE if isinstance(j, int) else pl.multiple_of(j * LANE, LANE), LANE)

    def wmod_copy(part, j, sem=S_MOD):
        return pltpu.make_async_copy(
            wmod_hbm.bitcast(U32).at[:, lane_tile(part * 2 * DT + j)],
            aux.at[wmod_rows(part, j), :], sems.at[sem])

    def wo_copy(half, j):
        rows = pl.ds(half * (H // 2) * TR, (H // 2) * TR)
        return pltpu.make_async_copy(wo_hbm.bitcast(U32).at[rows, lane_tile(j)], wo.at[j, rows],
                                     sems.at[S_WO])

    x_copy = pltpu.make_async_copy(x_hbm, xs, sems.at[S_X])

    def ffn_copy(m, i, nq):
        per_row = DT // 4
        kk, j = (i % per_row, i // per_row) if m < 2 else (i // per_row, i % per_row)
        return pltpu.make_async_copy(
            (w1_hbm, w3_hbm, w2_hbm)[m].bitcast(U32).at[aux_rows(kk * 4 * TR, 4 * TR),
                                                        lane_tile(4 * j + nq)],
            aux.at[aux_rows(raw_base(m * GM + i) + nq * 4 * TR, 4 * TR), :], sems.at[S_FF])

    def prefetch_ffn(s, part):
        if part < 6:
            @pl.when(s < GM)
            def _():
                for nq in range(2):
                    ffn_copy(part // 2, s, 2 * (part % 2) + nq).start()
        elif part == 6:
            @pl.when(s < 2 * DT)
            def _():
                wmod_copy(1, s).start()
                wmod_copy(2, s).start()

    def start(cps):
        for cp in cps:
            cp.start()

    def wait(cps):
        for cp in cps:
            cp.wait()

    def modulation(part, tiles):
        sc = jnp.broadcast_to(_silu(c_ref[...].astype(F32)), (8, D))
        for j in tiles:
            r = _dot(sc, _w(aux[wmod_rows(part, j), :]))
            mod[2 * part + j // DT, :, pl.ds((j % DT) * LANE, LANE)] = r

    def modrow(i):
        return mod[i, 0:1, :]

    def prologue(ring, xp, hp):
        def pair_copies(w_hbm, i):
            src = w_hbm.bitcast(U32)
            return [pltpu.make_async_copy(
                src.at[:, (i % it_per_mat) * PP + t + par * (H // 2), :],
                ring.at[i % RING, 2 * t + par], sems.at[S_ST + i % RING])
                for t in range(PP) for par in range(2)]

        xp_copy = pltpu.make_async_copy(x_hbm.at[:, pl.ds(CUR, PRE), :], xp, sems.at[S_XP])
        xp_copy.start()
        tiles = [range(t, 2 * DT, 2) for t in range(2)]
        halves = [[wmod_copy(0, j, sem) for j in tiles[t]] for t, sem in enumerate((S_MOD, S_FF))]
        start(halves[0])
        xp_copy.wait()
        start(halves[1])
        xn = _layernorm(xp[...].astype(F32).reshape(NP, D))
        for t in range(2):
            wait(halves[t])
            for i in range(t, AHEAD if t else 1):
                start(pair_copies(wq_hbm, i))
            modulation(0, tiles[t])
            for u in range(t, DT // 4, 2):
                def block(rq, kq):
                    cols = slice((kq * (DT // 4) + u) * LANE, (kq * (DT // 4) + u + 1) * LANE)
                    return (xn[rq * (NP // 4):(rq + 1) * (NP // 4), cols]
                            * (1.0 + mod[1, 0:1, cols]) + mod[0, 0:1, cols])

                for n, a in enumerate(_two_level(_strassen_lhs, block)):
                    hp[n, :, lane_tile(u)] = a.astype(BF16)

        def pro_body(i, carry):
            wait(pair_copies(wq_hbm, i))
            heads = []
            for t in range(PP):
                a = ring[i % RING, 2 * t]
                b = ring[i % RING, 2 * t + 1]
                heads += [(a & jnp.uint32(0xFFFF)) | (b << 16),
                          (a >> 16) | (b & jnp.uint32(0xFFFF0000))]
            for n, w in enumerate(heads):
                wqkv[i * 2 * PP + n] = w
            nxt = i + AHEAD
            for m, w_hbm in enumerate((wq_hbm, wk_hbm, wv_hbm)):
                @pl.when((nxt >= m * it_per_mat) & (nxt < (m + 1) * it_per_mat))
                def _():
                    start(pair_copies(w_hbm, nxt))
                    if m > 0:
                        wo_copy(m - 1, nxt - m * it_per_mat).start()

            @pl.when(nxt == n_it)
            def _():
                x_copy.start()

            rhs = _two_level(_strassen_rhs, lambda kq, nq: _w(
                heads[nq][kq * (D // 8):(kq + 1) * (D // 8)]).astype(F32))
            c = _two_level_out(lambda n: _dot(hp[n], rhs[n].astype(BF16)))
            for (rq, nq), val in c.items():
                for j in range(n_seg // 4):
                    sg = rq * (n_seg // 4) + j
                    r0 = pre_base(sg, sg >= s0) + (i * 2 * PP + nq) * PRE
                    aux[aux_rows(r0, PRE), :] = pltpu.bitcast(val[j * PRE:(j + 1) * PRE], U32)
            return carry

        lax.fori_loop(0, n_it, pro_body, 0)

    pl.run_scoped(prologue, pltpu.VMEM((RING, 2 * PP, D // 2, LANE), U32),
                  pltpu.VMEM((n_seg, PRE, D), BF16), pltpu.VMEM((49, NP // 4, D // 4), BF16))
    wait([wo_copy(half, j) for half in range(2) for j in range(DT)])
    x_copy.wait()

    def seg_rows(s):
        xn = _layernorm(xs[s].astype(F32)[0:CUR])
        return xn * (1.0 + modrow(1)) + modrow(0)

    lhs[...] = jnp.concatenate([mem_ref[...].astype(F32), seg_rows(0)], axis=0).astype(BF16)
    scale = float(LANE) ** -0.5
    NG = H // HG

    def chain_body(combine, s, carry):
        row = lax.broadcasted_iota(jnp.int32, (L, L), 0)
        col = lax.broadcasted_iota(jnp.int32, (L, L), 1)
        mask = (row < M) | (row >= col)
        q, k, v, p, ov = {}, {}, {}, {}, {}

        def heads(g):
            return range(g * HG, (g + 1) * HG)

        def proj(m, h):
            done = aux[aux_rows(pre_base(s, combine) + (m * H + h) * PRE, PRE), :]
            return jnp.concatenate([_dot(lhs[...], _w(wqkv[m * H + h])),
                                    pltpu.bitcast(done, F32)], axis=0)

        def probs(g):
            for h in heads(g):
                z = jnp.where(mask, _dot_nt(q[h], k[h]) * scale, -1e9)
                e = jnp.exp(z - jnp.max(z, axis=-1, keepdims=True))
                p[h] = e * pl.reciprocal(jnp.sum(e, axis=-1, keepdims=True), full_range=False)

        def values(g):
            for h in heads(g):
                ov[h] = _dot(p[h], v[h])

        def out_proj(h0, h1, marks):
            o = jnp.concatenate([ov[h] for h in range(h0, h1)], axis=1)
            cols = []
            for j in range(DT):
                cols.append(_dot(o, _w(wo[j, pl.ds(h0 * TR, (h1 - h0) * TR), :])))
                if combine and j in marks:
                    aux[aux_rows(pre_base(s, True), 8), :] = pltpu.bitcast(cols[-1][0:8], U32)
                    combine_weights(marks[j], CW[3])
            return jnp.concatenate(cols, axis=1)

        def combine_weights(g, outer):
            for r in range(g * TR // NG // 8 * 8, (g + 1) * TR // NG // 8 * 8, 8) if combine else ():
                def block(kq, nq):
                    rows = aux_rows(raw_base(s - s0) + (nq * 4 + kq) * TR + r, 8)
                    return _w(aux[rows, :]).astype(F32)

                for n, t in enumerate(_two_level(_strassen_rhs, block)):
                    if n // 7 in outer:
                        rows = aux_rows(((s - s0) * 49 + n) * TR + r, 8)
                        aux[rows, :] = pltpu.bitcast(t.astype(BF16), U32)

        for g in range(NG):
            combine_weights(g, CW[0])
            for h in heads(g):
                k[h] = proj(1, h).astype(BF16)
            combine_weights(g, CW[1])
            for h in heads(g):
                q[h] = proj(0, h)
            if g >= 1:
                probs(g - 1)
            if not combine:
                prefetch_ffn(s, g)
        for g in range(NG):
            combine_weights(g, CW[2])
            for h in heads(g):
                v[h] = proj(2, h).astype(BF16)
            if g == 0:
                probs(NG - 1)
            else:
                values(g - 1)
        nxt = seg_rows(jnp.minimum(s + 1, n_seg - 1))
        o = out_proj(0, SPLIT, {DT // 2 - 1: 0, DT - 1: 1})
        values(NG - 1)
        o = o + out_proj(SPLIT, H, {j: j + 2 for j in range(NG - 2)})
        attn[s] = o[M:].astype(BF16)
        lhs[...] = jnp.concatenate([o[:M], nxt], axis=0).astype(BF16)
        return carry

    lax.fori_loop(0, s0, functools.partial(chain_body, False), 0)
    wait([ffn_copy(m, i, nq) for m in range(3) for i in range(GM) for nq in range(4)])
    wait([wmod_copy(part, j) for part in (1, 2) for j in range(2 * DT)])
    modulation(1, range(2 * DT))
    modulation(2, range(2 * DT))
    lax.fori_loop(s0, n_seg, functools.partial(chain_body, True), 0, unroll=2)

    SB = 4
    n_blk = n_seg // SB

    def resid(sg, rows=slice(None), cols=slice(None)):
        return (xs[sg, rows, cols].astype(F32)
                + mod[2, 0:1, cols] * attn[sg, rows, cols].astype(F32))

    def ffn(act, upin, hbuf):
        KT = DT // 4

        def norm_steps(i, zero):
            def center(sg, rows):
                x1 = resid(i * SB + sg, rows=rows)
                hbuf[sg + zero, rows] = x1 - jnp.mean(x1, axis=-1, keepdims=True)

            def normalize(sg, rows):
                d = hbuf[sg, rows]
                rstd = lax.rsqrt(jnp.mean(d * d, axis=-1, keepdims=True) + EPS)
                hbuf[sg + zero, rows] = d * rstd * (1.0 + modrow(4)) + modrow(3)

            return [functools.partial(f, sg, slice(r, r + LN_ROWS)) for sg in range(SB)
                    for r in range(0, seg, LN_ROWS) for f in (center, normalize)]

        def operand_steps(zero):
            def operands(outer, t):
                ops = _two_level(_strassen_lhs,
                                 lambda rq, kq: hbuf[rq, :, lane_tile(4 * t + kq)])
                for n in range(7 * outer, 7 * outer + 7):
                    upin[n + zero, :, pl.ds(t * LANE, LANE)] = ops[n]

            return [functools.partial(operands, n, t) for n in range(7) for t in range(KT)]

        def products(a_ref, n_calls, first, steps, zero):
            calls = iter(range(n_calls))
            when = {first + k * (n_calls - first) // len(steps): f for k, f in enumerate(steps)}
            assert len(when) == len(steps)

            def product(granules, n):
                w = jnp.concatenate([aux[pl.ds((g * 49 + n) * TR, TR), :] for g in granules],
                                    axis=0)
                r = _dot(a_ref[n], _w(w))
                step = when.get(next(calls))
                if step is not None:
                    hbuf[SB + zero, 0:8, 0:LANE] = r[0:8]
                    step()
                return r

            return product

        for step in norm_steps(0, 0) + operand_steps(0):
            step()

        def ffn_body(i, carry):
            zero = i // n_blk
            product = products(upin, 2 * 49 * (FT // 4), FIRST[0],
                               norm_steps(jnp.minimum(i + 1, n_blk - 1), zero), zero)
            for j in range(FT // 4):
                gate, up = (_two_level_out(functools.partial(
                    product, range(m * GM + j * KT, m * GM + (j + 1) * KT))) for m in range(2))
                hidden = {rc: _silu(gate[rc]) * up[rc] for rc in gate}
                for n, t in enumerate(_two_level(_strassen_lhs, lambda r, c: hidden[r, c])):
                    act[n, :, lane_tile(j)] = t
            product = products(act, 49 * KT, FIRST[1], operand_steps(zero), zero)
            c = _two_level_out(lambda n: [product(range(2 * GM + j, 3 * GM, KT), n)
                                          for j in range(KT)])
            for (rq, nq), tiles in c.items():
                for j, t in enumerate(tiles):
                    cols = slice((4 * j + nq) * LANE, (4 * j + nq + 1) * LANE)
                    y = resid(i * SB + rq, cols=cols) + mod[5, 0:1, cols] * t
                    attn[i * SB + rq, :, cols] = y.astype(BF16)
            sl = pl.ds(i * SB, SB)
            pltpu.make_async_copy(attn.at[sl], out_hbm.at[sl], sems.at[S_OUT]).start()
            return carry

        lax.fori_loop(0, n_blk, ffn_body, 0)

    pl.run_scoped(ffn, pltpu.VMEM((49, seg, d_ff // 4), F32),
                  pltpu.VMEM((49, seg, D // 4), F32), pltpu.VMEM((SB + 1, seg, D), F32))
    pltpu.make_async_copy(attn, out_hbm, sems.at[S_OUT]).wait()


@functools.partial(jax.jit, static_argnames=("A_seg_len",))
def pallas_adaLN_cond__memory_aug_recurrent_mem_tr__glu_gated_swiglu__prompt_kernel(
    A_x, A_mem0, A_Wq, A_Wk, A_Wv, A_Wo, A_seg_len, B_x, B_w1, B_w3, B_w2, c, w_mod,
):
    del B_x
    B, S, D = A_x.shape
    _, H, Dh = A_Wq.shape
    M = A_mem0.shape[1]
    F = B_w1.shape[1]
    seg = int(A_seg_len)
    n_seg = S // seg
    n_gran = 3 * (D // (4 * LANE)) * (F // (4 * LANE))
    assert B == 1 and Dh == LANE and S % seg == 0 and n_seg % 4 == 0 and F % (4 * LANE) == 0
    assert max(n_gran // 3, 2 * D // LANE) <= n_seg - n_gran and AHEAD < RING
    assert H // 4 == D // LANE == H // HG == 8 and M == PRE == 8
    aux_rows = max((49 * n_gran + 16) * LANE // 2 + 3 * H * PRE,
                   n_seg * 3 * H * PRE + 3 * D * D // LANE + n_gran * 8 * LANE)
    kern = functools.partial(_kernel, seg=seg, n_seg=n_seg, n_mem=M, n_head=H, d_model=D, d_ff=F)
    hbm = pl.BlockSpec(memory_space=pl.ANY)
    vmem = pl.BlockSpec(memory_space=pltpu.VMEM)
    out = pl.pallas_call(
        kern,
        out_shape=jax.ShapeDtypeStruct((n_seg, seg, D), A_x.dtype),
        in_specs=[vmem, vmem] + [hbm] * 9,
        out_specs=hbm,
        scratch_shapes=[
            pltpu.VMEM((3 * H, D // 2, LANE), U32),
            pltpu.VMEM((D // LANE, H * Dh // 2, LANE), U32),
            pltpu.VMEM((aux_rows, LANE), U32),
            pltpu.VMEM((n_seg, seg, D), BF16),
            pltpu.VMEM((n_seg, seg, D), BF16),
            pltpu.VMEM((M + seg - PRE, D), BF16),
            pltpu.VMEM((6, 8, D), F32),
            pltpu.SemaphoreType.DMA((6 + RING,)),
        ],
        compiler_params=pltpu.CompilerParams(vmem_limit_bytes=127 * 1024 * 1024,
                                             disable_bounds_checks=True),
    )(c, A_mem0.reshape(M, D), A_x.reshape(n_seg, seg, D),
      A_Wq.reshape(D // 2, 2 * H, Dh), A_Wk.reshape(D // 2, 2 * H, Dh),
      A_Wv.reshape(D // 2, 2 * H, Dh),
      A_Wo.reshape(H * Dh, D), B_w1, B_w3, B_w2, w_mod)
    return out.reshape(B, S, D)
```
